```python
import jax
import jax.numpy as jnp

def _softmax(x, axis=-1):
    return jax.nn.softmax(x, axis=axis)
def _gelu(x):
    return jax.nn.gelu(x, approximate=True)
def _silu(x):
    return jax.nn.silu(x)
def _sigmoid(x):
    return jax.nn.sigmoid(x)
def _layernorm(x, axis=-1, eps=1e-5):
    m = jnp.mean(x, axis=axis, keepdims=True)
    v = jnp.var(x, axis=axis, keepdims=True)
    return (x - m) / jnp.sqrt(v + eps)
def _scatter_add(tgt, idx, src, axis=0):
    return tgt.at[idx].add(src)
def _segment_sum(src, seg, n):
    return jax.ops.segment_sum(src, seg, n)
class _Rng:
    def __init__(self, key):
        self._k = key
    def _next(self):
        self._k, sub = jax.random.split(self._k)
        return sub
    def normal(self, shape):
        return jax.random.normal(self._next(), shape, dtype=jnp.bfloat16)
    def randint(self, lo, hi, shape):
        return jax.random.randint(self._next(), shape, lo, hi, dtype=jnp.int32)
    def uniform(self, shape, lo=0.0, hi=1.0):
        return jax.random.uniform(self._next(), shape, jnp.bfloat16, lo, hi)
    def permutation(self, n):
        return jax.random.permutation(self._next(), n)


kernel_name = 'standalone__dcn_v2_cross__recsys'

def setup_inputs():
    _rng = _Rng(jax.random.key(int.from_bytes(__import__("os").urandom(4), "little")))
    _w = (lambda a: (lambda t: t.astype(jnp.bfloat16) if jnp.issubdtype(t.dtype, jnp.floating) else t)(jnp.asarray(a)))
    B, F, D, L = 16384, 26, 128, 6
    Din = min(F * D, 1024)
    return {
        "x0": _w((lambda *s: _rng.normal(s) * 0.05)(B, Din)),
        "ws": _w((lambda *s: _rng.normal(s) * 0.05)(L, Din, Din)),
        "bs": _w((lambda *s: _rng.normal(s) * 0.05)(L, Din)),
    }

def reference(x0, ws, bs):
    x = x0
    for l in range(ws.shape[0]):
        x = x0 * (x @ ws[l] + bs[l]) + x
    return x
```

```python
import functools

import jax
import jax.numpy as jnp
import jax.experimental.pallas as pl
import jax.experimental.pallas.tpu as pltpu


def _kernel(x0_ref, w_ref, b_ref, o_ref, *, num_layers):
    x0b = x0_ref[...]
    x0 = x0b.astype(jnp.float32)
    x = x0
    xb = x0b
    for l in range(num_layers):
        y = jnp.dot(xb, w_ref[l], preferred_element_type=jnp.float32)
        y = y + b_ref[l : l + 1, :].astype(jnp.float32)
        x = x0 * y + x
        xb = x.astype(jnp.bfloat16)
    o_ref[...] = xb


@jax.jit
def pallas_standalone__dcn_v2_cross__recsys_kernel(
    x0: jax.Array,
    ws: jax.Array,
    bs: jax.Array,
):
    B, D = x0.shape
    L = ws.shape[0]
    tm = 512
    return pl.pallas_call(
        functools.partial(_kernel, num_layers=L),
        grid=(B // tm,),
        in_specs=[
            pl.BlockSpec((tm, D), lambda i: (i, 0)),
            pl.BlockSpec((L, D, D), lambda i: (0, 0, 0), pipeline_mode=pl.Buffered(1)),
            pl.BlockSpec((L, D), lambda i: (0, 0), pipeline_mode=pl.Buffered(1)),
        ],
        out_specs=pl.BlockSpec((tm, D), lambda i: (i, 0)),
        out_shape=jax.ShapeDtypeStruct((B, D), x0.dtype),
        compiler_params=pltpu.CompilerParams(
            dimension_semantics=("arbitrary",),
            vmem_limit_bytes=100 * 1024 * 1024,
        ),
    )(x0, ws, bs)
```

```python
import functools

import jax
import jax.numpy as jnp
from jax import lax
import jax.experimental.pallas as pl
import jax.experimental.pallas.tpu as pltpu

_A = {1: [(0, 1), (3, 1)], 2: [(2, 1), (3, 1)], 3: [(0, 1)], 4: [(3, 1)],
      5: [(0, 1), (1, 1)], 6: [(2, 1), (0, -1)], 7: [(1, 1), (3, -1)]}
_B = {1: [(0, 1), (3, 1)], 2: [(0, 1)], 3: [(1, 1), (3, -1)], 4: [(2, 1), (0, -1)],
      5: [(3, 1)], 6: [(0, 1), (1, 1)], 7: [(2, 1), (3, 1)]}
_C = {0: [(1, 1), (4, 1), (5, -1), (7, 1)], 1: [(3, 1), (5, 1)],
      2: [(2, 1), (4, 1)], 3: [(1, 1), (2, -1), (3, 1), (6, 1)]}
_ORD_E = (4, 2, 7, 1, 5, 3, 6)
_ORD_O = (3, 5, 6, 1, 2, 4, 7)


def _lincomb(terms):
    terms = sorted(terms, key=lambda t: -t[1])
    acc = terms[0][0]
    for v, s in terms[1:]:
        acc = acc + v if s > 0 else acc - v
    return acc


def _rc(o, i):
    return (o // 2) * 2 + (i // 2), (o % 2) * 2 + (i % 2)


def _kernel(x0_ref, w_hbm, b_ref, o_ref, wraw, wexp, sems, x0f, xa, xb, ma, mb, *, L, rs):
    tm, D = x0_ref.shape
    R = tm // 4
    Cw = D // 4

    @pl.when(pl.program_id(0) == 0)
    def _():
        def cp(l):
            return pltpu.make_async_copy(w_hbm.at[l], wraw.at[l], sems.at[l])

        for l in range(L):
            cp(l).start()

        def per_layer(l, carry):
            cp(l).wait()

            def per_rows(t, c2):
                r0 = pl.multiple_of(t * 16, 16)
                for c0 in range(0, Cw, 128):
                    blk = {}
                    for o in range(4):
                        for i in range(4):
                            r, c = _rc(o, i)
                            blk[o, i] = wraw[
                                l, pl.ds(r * Cw + r0, 16), c * Cw + c0 : c * Cw + c0 + 128
                            ].astype(jnp.float32)
                    for p in range(1, 8):
                        op = [_lincomb([(blk[o, i], s) for o, s in _B[p]]) for i in range(4)]
                        for q in range(1, 8):
                            v = _lincomb([(op[i], s) for i, s in _B[q]])
                            wexp[
                                l, (p - 1) * 7 + (q - 1),
                                pl.ds(pl.multiple_of(t * 8, 8), 8), c0 : c0 + 128,
                            ] = pltpu.bitcast(v.astype(jnp.bfloat16), jnp.uint32)
                return c2

            lax.fori_loop(0, Cw // 16, per_rows, 0)
            return carry

        lax.fori_loop(0, L, per_layer, 0)

    for o in (3, 2, 1, 0):
        for i in range(4):
            r, c = _rc(o, i)
            x0f[o * 4 + i] = x0_ref[r * R : (r + 1) * R, c * Cw : (c + 1) * Cw].astype(jnp.float32)
    xs = [xa, xb]
    ms = [ma, mb]
    for l in range(L):
        xin = x0f if l == 0 else xs[(l - 1) % 2]
        xout = xs[l % 2]
        m_ref = ms[l % 2]
        order = _ORD_E if l % 2 == 0 else _ORD_O
        done = set()
        for p in order:
            for q in _ORD_O:
                idx = (p - 1) * 7 + (q - 1)
                terms = [(xin[o * 4 + i], so * si) for (o, so) in _A[p] for (i, si) in _A[q]]
                a = _lincomb(terms).astype(jnp.bfloat16)
                m = jnp.dot(
                    a, pltpu.bitcast(wexp[l, idx], jnp.bfloat16),
                    preferred_element_type=jnp.float32,
                )
                if p in (3, 4) and q in (3, 4):
                    cc = (0 if p == 4 else 2) + (0 if q == 4 else 1)
                    m = m + b_ref[l : l + 1, cc * Cw : (cc + 1) * Cw].astype(jnp.float32)
                m_ref[idx] = m
            done.add(p)
            for o in range(4):
                if p in [t[0] for t in _C[o]] and all(t[0] in done for t in _C[o]):
                    for r0 in range(0, R, rs):
                        sl = slice(r0, r0 + rs)
                        mm = {
                            q: _lincomb([(m_ref[(pp - 1) * 7 + (q - 1), sl, :], s) for pp, s in _C[o]])
                            for q in range(1, 8)
                        }
                        for i in range(4):
                            y = _lincomb([(mm[q], s) for q, s in _C[i]])
                            xn = x0f[o * 4 + i, sl, :] * y + xin[o * 4 + i, sl, :]
                            if l == L - 1:
                                r, c = _rc(o, i)
                                o_ref[r * R + r0 : r * R + r0 + rs, c * Cw : (c + 1) * Cw] = (
                                    xn.astype(o_ref.dtype)
                                )
                            else:
                                xout[o * 4 + i, sl, :] = xn


@jax.jit
def pallas_standalone__dcn_v2_cross__recsys_kernel(
    x0: jax.Array,
    ws: jax.Array,
    bs: jax.Array,
):
    B, D = x0.shape
    L = ws.shape[0]
    tm = 512
    R = tm // 4
    Cw = D // 4
    return pl.pallas_call(
        functools.partial(_kernel, L=L, rs=16),
        grid=(B // tm,),
        in_specs=[
            pl.BlockSpec((tm, D), lambda i: (i, 0)),
            pl.BlockSpec(memory_space=pl.ANY),
            pl.BlockSpec((L, D), lambda i: (0, 0), pipeline_mode=pl.Buffered(1)),
        ],
        out_specs=pl.BlockSpec((tm, D), lambda i: (i, 0)),
        out_shape=jax.ShapeDtypeStruct((B, D), x0.dtype),
        scratch_shapes=[
            pltpu.VMEM((L, D, D), jnp.bfloat16),
            pltpu.VMEM((L, 49, Cw // 2, Cw), jnp.uint32),
            pltpu.SemaphoreType.DMA((L,)),
        ]
        + [pltpu.VMEM((16, R, Cw), jnp.float32)] * 3
        + [pltpu.VMEM((49, R, Cw), jnp.float32)] * 2,
        compiler_params=pltpu.CompilerParams(
            dimension_semantics=("arbitrary",),
            vmem_limit_bytes=120 * 1024 * 1024,
        ),
    )(x0, ws, bs)
```

```python
import functools

import numpy as np
import jax
import jax.numpy as jnp
from jax import lax
import jax.experimental.pallas as pl
import jax.experimental.pallas.tpu as pltpu

f32 = jnp.float32
bf16 = jnp.bfloat16

_D = float(np.sqrt(3.0))
_PH = (3, 5, 4, 7, 1, 2, 6)
_MIDB = {1: [(0, 1)], 2: [(1, 1)], 3: [(2, 1)], 5: [(3, 1)],
         4: [(0, 1), (2, -1)], 6: [(1, 1), (0, -1)], 7: [(3, 1), (0, -1)]}
_CVEC = {1: [1, 0, 0, 1], 2: [0, 0, 1, -1], 3: [1, 1, 1, 1], 4: [1, 0, 1, 0],
         5: [-1, 1, 1, -1], 6: [0, 0, 1, 1], 7: [1, 0, -1, 0]}
_BSET = (3, 4, 7, 1)
_NZ = 14
_TM = 512
_H = _TM // 8
_BS = _H // 8 + 1


def _kappa():
    m = np.array([_CVEC[p] for p in _BSET], np.float64).T
    pats = [np.array([1, 0, _D, 0]), np.array([0, 1 / _D, 0, 1])]
    return [dict(zip(_BSET, np.linalg.solve(m, t))) for t in pats]


def _lin(terms):
    terms = sorted(terms, key=lambda t: -t[1])
    acc = terms[0][0]
    for v, s in terms[1:]:
        acc = acc + v if s > 0 else acc - v
    return acc


def _comb7(m):
    s = m[3] + m[5]
    e = (m[3] - m[5]) + m[1]
    return [(e + m[4]) + m[7], s, (((s + m[4]) - m[7]) + m[2]) + m[6], (e - m[2]) + m[6]]


def _fwd(x):
    a1 = x[0] + x[3]
    return [a1, ((x[1] + x[2]) + a1) * 0.5, x[0] - x[1], x[0] + x[1]]


def _bexp(b, dbl):
    b1 = b[0] + b[3]
    u = b[1] + b[2]
    o = {1: b1, 2: b[0] - b[1], 3: b[1] - b[3], 4: u - b1, 5: b[1] + b[3], 6: b[0] + b[1], 7: u + b1}
    for p in dbl:
        o[p] = o[p] + o[p]
    return o


def _rowcol(o, i, t):
    r = (o // 2) * 4 + (i // 2) * 2 + t // 2
    c = (o % 2) * 4 + (i % 2) * 2 + t % 2
    e = (o // 2 - o % 2) + (i // 2 - i % 2) + (t // 2 - t % 2)
    return r, c, e


def _plan(l3set):
    order = []
    for p in _PH:
        ks = [q for q in range(1, 8) if (p, q) not in l3set]
        ls = [q for q in (3, 5, 2, 4, 7, 6, 1) if (p, q) in l3set]
        order += [(p, q) for q in ((ks + ls) if p in (3, 4, 2) else (ls + ks))]
    tile0 = {}
    n = 0
    for pq in order:
        tile0[pq] = n
        n += 7 if pq in l3set else 4
    return order, tile0, n


_NAMES = ([(f"u{p}", 7) for p in (3, 4, 7, 5, 1, 2, 6)]
          + [(f"a{p}", 4) for p in (3, 4, 5, 7, 2, 6)]
          + [(f"{s}{k}", 4) for s in ("fx", "H", "G", "U", "V") for k in range(2)]
          + [(f"x0{o}", 4) for o in range(4)])


def _kernel(x_hbm, w_hbm, b_ref, o_hbm, zs, ring, stage, wraw, wexp, beta,
            xsem, wsem, tsem, bsem, *bufs, L, nsteps, l3set, win):
    H = _H
    NG = H // 8
    HT = _TM // 2
    step = pl.program_id(0)
    order, tile0, _ = _plan(l3set)
    buf = dict(zip([(n, t) for n, _ in _NAMES for t in range(4)], bufs))
    skew = {n: k % 4 for k, (n, _) in enumerate(_NAMES)}
    ctx = {}

    def x_copy(i):
        return pltpu.make_async_copy(
            x_hbm.at[pl.ds(pl.multiple_of(i * _TM, _TM), _TM)], ring.at[i % 4], xsem.at[i % 4])

    def w_copy(l):
        return pltpu.make_async_copy(w_hbm.at[l], wraw.at[l], wsem.at[l])

    def top_copy(i):
        return pltpu.make_async_copy(
            stage.at[i % 2, pl.ds(HT, HT)],
            o_hbm.at[pl.ds(pl.multiple_of(i * _TM, HT), HT)], tsem.at[i % 2])

    def bot_copy(i):
        return pltpu.make_async_copy(
            stage.at[i % 2, pl.ds(0, HT)],
            o_hbm.at[pl.ds(pl.multiple_of(i * _TM - HT, HT), HT)], bsem.at[i % 2])

    def off(n, b, t):
        return ((skew[n] + t) % 4 + b * _BS) * 8

    def ld(n, b, t):
        o = off(n, b, t)
        return buf[n, t][ctx["z"], o:o + H, :]

    def st(n, b, t, v):
        o = off(n, b, t)
        buf[n, t][0, o:o + H, :] = v

    def anc(v, a):
        return v if a is None else jnp.where(ctx["mask"], a, v)

    def xin(slot, o, i, t):
        r, c, _ = _rowcol(o, i, t)
        return ring[slot, r * H:(r + 1) * H, c * 128:(c + 1) * 128].astype(f32)

    def finish(l, o, g, t, a):
        if l < L - 1:
            return [ld(f"x0{o}", i, t) * g[i] for i in range(4)]
        top = o < 2
        if g is not None:
            for i in range(4):
                r, c, e = _rowcol(o, i, t)
                y = xin(ctx["old_top"] if top else ctx["old_bot"], o, i, t) * g[i]
                if e:
                    y = y * (_D ** -e)
                r0 = (r * H + HT) % _TM
                stage[ctx["oslot"], r0:r0 + H, c * 128:(c + 1) * 128] = y.astype(bf16)
        slot = ctx["new_top"] if top else ctx["new_bot"]
        if slot is None:
            return None
        xs = []
        for i in range(4):
            e = _rowcol(o, i, t)[2]
            v = xin(slot, o, i, t)
            if i == 0:
                v = anc(v, a)
            st(f"x0{o}", i, t, v)
            xs.append(v * (_D ** e) if e else v)
        return xs

    def upd(l, u, s, t, a):
        m = {q: ld(u, q - 1, t) for q in range(1, 8)}
        m[3] = anc(m[3], a)
        y = _comb7(m)
        if l > 0:
            y = [y[i] + ld(f"{s}{(l - 1) % 2}", i, t) for i in range(4)]
        for i in range(4):
            st(f"{s}{l % 2}", i, t, y[i])
        return y

    def w1(l, t, a, init=False):
        x = finish(l, 1, None if init else upd(l, "u5", "H", t, a), t, a)
        for i, v in enumerate(_fwd(x)):
            st(f"fx{l % 2}", i, t, v)

    def w2(l, t, a, init=False):
        x = finish(l, 0, None if init else upd(l, "u1", "G", t, a), t, a)
        for i, v in enumerate(_fwd(x)):
            w = ld(f"fx{l % 2}", i, t)
            st("a3", i, t, v - w)
            st("a5", i, t, v + w)

    def w3(l, t, a):
        upd(l, "u2", "U", t, a)

    def w4(l, t, a):
        v6 = upd(l, "u6", "V", t, a)
        g = [v6[i] + (ld(f"G{l % 2}", i, t) - ld(f"U{l % 2}", i, t)) for i in range(4)]
        x = finish(l, 3, g, t, a)
        if x is not None:
            for i, v in enumerate(_fwd(x)):
                w = ld(f"fx{l % 2}", i, t)
                st("a4", i, t, w + v)
                st("a7", i, t, w - v)

    def w5(l, t, a):
        g = [anc(ld(f"U{l % 2}", i, t), a if (i == 0 or l == L - 1) else None)
             + ld(f"V{l % 2}", i, t) + ld(f"H{l % 2}", i, t) for i in range(4)]
        x = finish(l, 2, g, t, a)
        if x is not None:
            for i, v in enumerate(_fwd(x)):
                u = ld(f"fx{l % 2}", i, t) + v
                a1 = ld("a3", i, t) + ld("a4", i, t)
                st("a2", i, t, u + a1)
                st("a6", i, t, u - a1)

    task = {1: w1, 2: w2, 3: w3, 4: w4, 5: w5}

    @pl.when(step == 0)
    def _():
        x_copy(0).start()
        w_copy(0).start()
        w_copy(1).start()
        for k in range(_NZ):
            zs[k] = 0
        kap = _kappa()
        for l in range(L):
            bl = b_ref[l:l + 1, :].astype(f32)
            if l == 0:
                bl = bl + 1.0
            for pi, p in enumerate(_BSET):
                for qi, q in enumerate(_BSET):
                    for c3 in range(2):
                        acc = None
                        for c1 in range(2):
                            for c2 in range(2):
                                k = float(kap[c1][p] * kap[c2][q])
                                if abs(k) < 1e-12:
                                    continue
                                c = c1 * 4 + c2 * 2 + c3
                                term = bl[:, c * 128:(c + 1) * 128] * k
                                acc = term if acc is None else acc + term
                        for r3 in range(2):
                            row = l * 64 + (pi * 4 + qi) * 4 + r3 * 2 + c3
                            beta[row:row + 1, :] = acc * (_D ** (r3 - c3))
        x_copy(0).wait()
        x_copy(1).start()
        ctx.update(z=0, new_top=0)
        for t in range(4):
            w1(L - 1, t, None, init=True)
        for t in range(4):
            w2(L - 1, t, None, init=True)

        def per_layer(l, carry):
            w_copy(l).wait()

            @pl.when(l + 2 < L)
            def _():
                w_copy(l + 2).start()

            def per_rows(g, c2):
                r0 = pl.multiple_of(g * 16, 16)
                blk = {}
                for o in range(4):
                    for i in range(4):
                        for t in range(4):
                            r, c, e = _rowcol(o, i, t)
                            v = wraw[l, pl.ds(r * 128 + r0, 16), c * 128:(c + 1) * 128].astype(f32)
                            blk[o, i, t] = v * (0.125 * _D ** e)
                outer = {(i, t): _bexp([blk[o, i, t] for o in range(4)], (1,))
                         for i in range(4) for t in range(4)}
                for p in _PH:
                    mid = [_bexp([outer[i, t][p] for i in range(4)], (1, 2, 6)) for t in range(4)]
                    for q in range(1, 8):
                        qs = [mid[t][q] for t in range(4)]
                        if (p, q) in l3set:
                            inn = _bexp(qs, (1,))
                            tiles = [inn[r] for r in range(1, 8)]
                        else:
                            tiles = [v + v for v in qs]
                        for k, v in enumerate(tiles):
                            wexp[l, tile0[p, q] + k, pl.ds(r0, 16), :] = v.astype(bf16)
                return c2

            lax.fori_loop(0, 8, per_rows, 0)
            return carry

        lax.fori_loop(0, L, per_layer, 0)

    @pl.when(step + 1 < nsteps)
    def _():
        x_copy(step + 1).wait()

    @pl.when(step + 2 < nsteps)
    def _():
        x_copy(step + 2).start()

    zz = [zs[k] for k in range(_NZ)]
    ctx.update(mask=jnp.full((H, 128), zz[0], jnp.int32) != 0,
               old_top=step % 4, new_top=(step + 1) % 4,
               old_bot=(step + 3) % 4, new_bot=step % 4, oslot=step % 2)
    wu = wexp.bitcast(jnp.uint32)

    def wtile(l, k):
        return pltpu.bitcast(wu[l, k], bf16)

    prods = [(l, p, q) for l in range(L) for (p, q) in order]
    npr = len(prods)
    free = [0, 0, 0, 0]
    anchors = []
    pstart = []
    for pi, (l, p, q) in enumerate(prods):
        pstart.append(min(free))
        if (p, q) in l3set:
            for j in range(7):
                mx = int(np.argmin(free))
                anchors += [(free[mx] + g * 8, pi, j, g) for g in range(NG)]
                free[mx] += H
        else:
            anchors += [(max(free) + g * 8, pi, 0, g) for g in range(2 * NG)]
            free = [f + 2 * H for f in free]
    pstart.append(max(free))
    anchors.sort()
    times = np.array([a[0] for a in anchors])

    def tpos(x):
        i = int(np.floor(x))
        return pstart[i] + (x - i) * (pstart[min(i + 1, npr)] - pstart[i])

    sched = {}
    for l in range(L):
        for w in (1, 2, 3, 4, 5):
            b0, b1 = win[w]
            i0, i1 = l * 49 + b0, l * 49 + b1
            if i0 >= npr:
                i0, i1 = i0 - npr, i1 - npr
            assert i1 <= npr
            for t in range(4):
                al = []
                for g in range(NG):
                    tt = tpos(i0) + (tpos(i1) - tpos(i0)) * (t * NG + g) / (4 * NG)
                    ai = int(np.searchsorted(times, tt))
                    while anchors[ai][1] < int(i0):
                        ai += 1
                    al.append(anchors[ai][1:])
                sched.setdefault(max(a[0] for a in al), []).append((w, l, t, al))

    subs = {}
    l3pos = 0
    for pi, (l, p, q) in enumerate(prods):
        ctx["z"] = zz[pi % 8]
        srcs = ["a3", "a4"] if p == 1 else [f"a{p}"]
        qv = [_lin([(ld(n, b, t), s) for n in srcs for b, s in _MIDB[q]]) for t in range(4)]
        k0 = tile0[p, q]
        if (p, q) in l3set:
            a1 = qv[0] + qv[3]
            u = qv[1] + qv[2]
            av = {1: a1, 3: qv[0] - qv[1], 5: qv[0] + qv[1], 4: qv[1] + qv[3],
                  7: qv[1] - qv[3], 2: u + a1, 6: u - a1}
            so = (1, 3, 5, 4, 7, 2, 6) if l3pos % 4 == 1 else (3, 5, 1, 4, 7, 2, 6)
            l3pos += 1
            m = {r: jnp.dot(av[r].astype(bf16), wtile(l, k0 + r - 1), preferred_element_type=f32)
                 for r in so}
            subs[pi] = [m[r] for r in so]
            mq = _comb7(m)
        else:
            a = jnp.concatenate(
                [jnp.concatenate(qv[:2], 1), jnp.concatenate(qv[2:], 1)], 0).astype(bf16)
            wt = [wtile(l, k0 + t) for t in range(4)]
            wm = jnp.concatenate([jnp.concatenate(wt[:2], 1), jnp.concatenate(wt[2:], 1)], 0)
            mm = jnp.dot(a, wm, preferred_element_type=f32)
            subs[pi] = [mm[:, :128]]
            mq = [mm[:H, :128], mm[:H, 128:], mm[H:, :128], mm[H:, 128:]]
        if p in _BSET and q in _BSET:
            row = l * 64 + (_BSET.index(p) * 4 + _BSET.index(q)) * 4
            mq = [mq[t] + beta[row + t:row + t + 1, :] for t in range(4)]
        for t in range(4):
            v = mq[t]
            if p == 5:
                v = v + ld("u3", q - 1, t)
            elif p == 1:
                r3 = ld("u3", q - 1, t)
                v = v + (((ld("u4", q - 1, t) + ld("u7", q - 1, t)) + (r3 + r3)) - ld("u5", q - 1, t))
            elif p == 2:
                v = v + ld("u4", q - 1, t)
            elif p == 6:
                v = v - ld("u7", q - 1, t)
            st(f"u{p}", q - 1, t, v)
        for (w, tl, t, al) in sched.get(pi, []):
            a = jnp.concatenate([subs[api][j][g * 8:(g + 1) * 8, :] for api, j, g in al], 0)
            ctx["z"] = zz[8 + (w + tl) % 6]
            task[w](tl, t, a)

    @pl.when(step >= 1)
    def _():
        top_copy(step - 1).wait()

    @pl.when(step >= 2)
    def _():
        bot_copy(step - 1).wait()

    top_copy(step).start()

    @pl.when(step >= 1)
    def _():
        bot_copy(step).start()

    @pl.when(step == nsteps - 1)
    def _():
        ctx.update(z=0, old_bot=(nsteps - 1) % 4, new_bot=None, oslot=nsteps % 2)
        for w in (3, 4, 5):
            if win[w][0] >= 49:
                for t in range(4):
                    task[w](L - 1, t, None)
        bot_copy(nsteps).start()
        top_copy(nsteps - 1).wait()
        bot_copy(nsteps - 1).wait()
        bot_copy(nsteps).wait()


_L3SET = tuple((p, q) for p in range(2, 8) for q in range(2, 8))
_WIN = {1: (24, 34), 2: (36, 45), 3: (44, 48.5), 4: (49, 60), 5: (63, 73)}


def _build(l3set=_L3SET, win=_WIN):
    def fn(x0, ws, bs):
        B, Dm = x0.shape
        L = ws.shape[0]
        nsteps = B // _TM
        ntiles = _plan(l3set)[2]
        return pl.pallas_call(
            functools.partial(_kernel, L=L, nsteps=nsteps, l3set=l3set, win=win),
            grid=(nsteps,),
            in_specs=[
                pl.BlockSpec(memory_space=pl.ANY),
                pl.BlockSpec(memory_space=pl.ANY),
                pl.BlockSpec((L, Dm), lambda i: (0, 0), pipeline_mode=pl.Buffered(1)),
            ],
            out_specs=pl.BlockSpec(memory_space=pl.ANY),
            out_shape=jax.ShapeDtypeStruct((B, Dm), x0.dtype),
            scratch_shapes=[
                pltpu.SMEM((_NZ,), jnp.int32),
                pltpu.VMEM((4, _TM, Dm), bf16),
                pltpu.VMEM((2, _TM, Dm), bf16),
                pltpu.VMEM((L, Dm, Dm), bf16),
                pltpu.VMEM((L, ntiles, 128, 128), bf16),
                pltpu.VMEM((L * 64, 128), f32),
                pltpu.SemaphoreType.DMA((4,)),
                pltpu.SemaphoreType.DMA((L,)),
                pltpu.SemaphoreType.DMA((2,)),
                pltpu.SemaphoreType.DMA((2,)),
            ]
            + [pltpu.VMEM((1, ((n * _BS + 7) // 4 * 4) * 8, 128), f32)
               for _, n in _NAMES for _t in range(4)],
            compiler_params=pltpu.CompilerParams(
                dimension_semantics=("arbitrary",),
                vmem_limit_bytes=126 * 1024 * 1024,
            ),
        )(x0, ws, bs)

    return fn


@jax.jit
def pallas_standalone__dcn_v2_cross__recsys_kernel(
    x0: jax.Array,
    ws: jax.Array,
    bs: jax.Array,
):
    return _build()(x0, ws, bs)
```

```python
import functools

import numpy as np
import jax
import jax.numpy as jnp
from jax import lax
import jax.experimental.pallas as pl
import jax.experimental.pallas.tpu as pltpu

f32 = jnp.float32
bf16 = jnp.bfloat16

_D = float(np.sqrt(3.0))
_PH = (3, 5, 4, 7, 1, 2, 6)
_MIDB = {1: [(0, 1)], 2: [(1, 1)], 3: [(2, 1)], 5: [(3, 1)],
         4: [(0, 1), (2, -1)], 6: [(1, 1), (0, -1)], 7: [(3, 1), (0, -1)]}
_CVEC = {1: [1, 0, 0, 1], 2: [0, 0, 1, -1], 3: [1, 1, 1, 1], 4: [1, 0, 1, 0],
         5: [-1, 1, 1, -1], 6: [0, 0, 1, 1], 7: [1, 0, -1, 0]}
_BSET = (3, 4, 7, 1)
_NZ = 14


def _bs(tm):
    ng = tm // 64
    return ng // 4 * 4 + (1 if ng % 4 == 0 else 5)


def _kappa():
    m = np.array([_CVEC[p] for p in _BSET], np.float64).T
    pats = [np.array([1, 0, _D, 0]), np.array([0, 1 / _D, 0, 1])]
    return [dict(zip(_BSET, np.linalg.solve(m, t))) for t in pats]


def _lin(terms):
    terms = sorted(terms, key=lambda t: -t[1])
    acc = terms[0][0]
    for v, s in terms[1:]:
        acc = acc + v if s > 0 else acc - v
    return acc


def _comb7(m):
    s = m[3] + m[5]
    e = (m[3] - m[5]) + m[1]
    return [(e + m[4]) + m[7], s, (((s + m[4]) - m[7]) + m[2]) + m[6], (e - m[2]) + m[6]]


def _fwd(x):
    a1 = x[0] + x[3]
    return [a1, ((x[1] + x[2]) + a1) * 0.5, x[0] - x[1], x[0] + x[1]]


def _bexp(b, dbl):
    b1 = b[0] + b[3]
    u = b[1] + b[2]
    o = {1: b1, 2: b[0] - b[1], 3: b[1] - b[3], 4: u - b1, 5: b[1] + b[3], 6: b[0] + b[1], 7: u + b1}
    for p in dbl:
        o[p] = o[p] + o[p]
    return o


def _rowcol(o, i, t):
    r = (o // 2) * 4 + (i // 2) * 2 + t // 2
    c = (o % 2) * 4 + (i % 2) * 2 + t % 2
    e = (o // 2 - o % 2) + (i // 2 - i % 2) + (t // 2 - t % 2)
    return r, c, e


def _plan(l3set, cfg):
    order = []
    for p in _PH:
        ks = [q for q in range(1, 8) if (p, q) not in l3set]
        ls = [q for q in cfg["qo"] if (p, q) in l3set]
        order += [(p, q) for q in ((ks + ls) if p in (3, 4, 2) else (ls + ks))]
    tile0 = {}
    n = 0
    for pq in order:
        tile0[pq] = n
        n += 7 if pq in l3set else 4
    return order, tile0, n


_NAMES = ([(f"u{p}", 7) for p in (3, 4, 7, 5, 1, 2, 6)]
          + [(f"a{p}", 4) for p in (3, 4, 5, 7, 2, 6)]
          + [(f"{s}{k}", 4) for s in ("fx", "H", "G", "U", "V") for k in range(2)]
          + [(f"x0{o}", 4) for o in range(4)]
          + [("u2x", 7), ("u6x", 7)] + [(f"{s}{k}", 4) for s in "HGUV" for k in (2, 3)])


def _kernel(x_hbm, w_hbm, b_ref, o_hbm, ring, stage, wraw, wexp, beta, fy, fx32, fxb, fb,
            xsem, wsem, tsem, bsem, fsem, *bufs, L, nsteps, cfg):
    l3set, win, TM, TPS, ROFF = cfg["l3set"], cfg["win"], cfg["tm"], cfg["tps"], cfg["roff"]
    H = TM // 8
    NG = H // 8
    HT = TM // 2
    ST = TM * TPS
    BS = _bs(TM)
    step = pl.program_id(0)
    order, tile0, _ = _plan(l3set, cfg)
    tmp = bufs[0]
    buf = dict(zip([(n, t) for n, _ in _NAMES for t in range(4)], bufs[1:]))
    skew = {n: k % 4 for k, (n, _) in enumerate(_NAMES)}
    ctx = {}

    def x_copy(i):
        return pltpu.make_async_copy(
            x_hbm.at[pl.ds(pl.multiple_of(ROFF + i * ST, 64), ST)], ring.at[i & 3], xsem.at[i & 3])

    def w_copy(l):
        return pltpu.make_async_copy(w_hbm.at[l], wraw.at[l], wsem.at[l])

    def top_copy(i):
        return pltpu.make_async_copy(
            stage.at[i & 1, pl.ds(HT, ST - HT)],
            o_hbm.at[pl.ds(pl.multiple_of(ROFF + i * ST, 64), ST - HT)], tsem.at[i & 1])

    def bot_copy(i):
        return pltpu.make_async_copy(
            stage.at[i & 1, pl.ds(0, HT)],
            o_hbm.at[pl.ds(pl.multiple_of(ROFF + i * ST - HT, 64), HT)], bsem.at[i & 1])

    def fin(c):
        return pltpu.make_async_copy(
            x_hbm.at[pl.ds(0, ROFF), pl.ds(c * 128, 128)], fxb.at[c], fsem.at[c])

    def fout(c):
        return pltpu.make_async_copy(
            fxb.at[(L & 1) * 8 + c], o_hbm.at[pl.ds(0, ROFF), pl.ds(c * 128, 128)], fsem.at[c])

    def off(n, b, t):
        return ((skew[n] + t) % 4 + b * BS) * 8

    def ld(n, b, t):
        o = off(n, b, t)
        return buf[n, t][ctx["z"], o:o + H, :]

    def st(n, b, t, v):
        o = off(n, b, t)
        buf[n, t][0, o:o + H, :] = v

    def anc(v, a):
        return v if a is None else jnp.where(ctx["mask"], a, v)

    def xin(j, o, i, t):
        r, c, _ = _rowcol(o, i, t)
        r0 = (j % TPS) * TM + r * H
        return ring[ctx["slot"][j // TPS], r0:r0 + H, c * 128:(c + 1) * 128].astype(f32)

    def sname(s, l):
        return f"{s}{l - L + 4 if l >= L - 2 else l % 2}"

    def uname(p, l):
        return f"u{p}x" if (l == L - 1 and p in (2, 6)) else f"u{p}"

    def emit(o, g, t):
        for i in range(4):
            r, c, e = _rowcol(o, i, t)
            y = xin(ctx["j"], o, i, t) * g[i]
            if e:
                y = y * (_D ** -e)
            r0 = ctx["j"] * TM + r * H + HT
            stage[ctx["oslot"], r0:r0 + H, c * 128:(c + 1) * 128] = y.astype(bf16)

    def fresh(o, t, a):
        xs = []
        for i in range(4):
            e = _rowcol(o, i, t)[2]
            v = xin(ctx["j"] + 1, o, i, t)
            if i == 0:
                v = anc(v, a)
            st(f"x0{o}", i, t, v)
            xs.append(v * (_D ** e) if e else v)
        return xs

    def gate(o, g, t):
        return [ld(f"x0{o}", i, t) * g[i] for i in range(4)]

    def upd(l, p, s, t, a, keep=True):
        m = {q: ld(uname(p, l), q - 1, t) for q in range(1, 8)}
        m[3] = anc(m[3], a)
        y = _comb7(m)
        if l > 0:
            y = [y[i] + ld(sname(s, l - 1), i, t) for i in range(4)]
        if keep:
            for i in range(4):
                st(sname(s, l), i, t, y[i])
        return y

    def f1(l, t, x):
        for i, v in enumerate(_fwd(x)):
            st(f"fx{l % 2}", i, t, v)

    def f2(l, t, x):
        for i, v in enumerate(_fwd(x)):
            w = ld(f"fx{l % 2}", i, t)
            st("a3", i, t, v - w)
            st("a5", i, t, v + w)

    def f4(l, t, x):
        for i, v in enumerate(_fwd(x)):
            w = ld(f"fx{l % 2}", i, t)
            st("a4", i, t, w + v)
            st("a7", i, t, w - v)

    def f5(l, t, x):
        for i, v in enumerate(_fwd(x)):
            u = ld(f"fx{l % 2}", i, t) + v
            a1 = ld("a3", i, t) + ld("a4", i, t)
            st("a2", i, t, u + a1)
            st("a6", i, t, u - a1)

    def w4(l, t, a):
        v6 = upd(l, 6, "V", t, a)
        g = [v6[i] + (ld(sname("G", l), i, t) - ld(sname("U", l), i, t)) for i in range(4)]
        f4(l, t, gate(3, g, t))

    def w5(l, t, a):
        g = [anc(ld(sname("U", l), i, t), a if i == 0 else None)
             + ld(sname("V", l), i, t) + ld(sname("H", l), i, t) for i in range(4)]
        f5(l, t, gate(2, g, t))

    def o4(l, t, a):
        v6 = upd(l, 6, "V", t, a)
        emit(3, [v6[i] + (ld(sname("G", l), i, t) - ld(sname("U", l), i, t)) for i in range(4)], t)

    def o5(l, t, a):
        emit(2, [anc(ld(sname("U", l), i, t), a) + ld(sname("V", l), i, t) + ld(sname("H", l), i, t)
                 for i in range(4)], t)

    task = {
        "w1": lambda l, t, a: f1(l, t, gate(1, upd(l, 5, "H", t, a), t)),
        "w2": lambda l, t, a: f2(l, t, gate(0, upd(l, 1, "G", t, a), t)),
        "w3": lambda l, t, a: upd(l, 2, "U", t, a),
        "w4": w4,
        "w5": w5,
        "o1": lambda l, t, a: emit(1, upd(l, 5, "H", t, a), t),
        "o2": lambda l, t, a: emit(0, upd(l, 1, "G", t, a), t),
        "o3": lambda l, t, a: upd(l, 2, "U", t, a),
        "o4": o4,
        "o5": o5,
        "e1": lambda l, t, a: f1(l, t, fresh(1, t, a)),
        "e2": lambda l, t, a: f2(l, t, fresh(0, t, a)),
        "e4": lambda l, t, a: f4(l, t, fresh(3, t, a)),
        "e5": lambda l, t, a: f5(l, t, fresh(2, t, a)),
    }

    @pl.when(step == 0)
    def _():
        w_copy(0).start()
        for c in range(8):
            fin(c).start()
        kap = _kappa()
        for l in range(L):
            bl = b_ref[l:l + 1, :].astype(f32)
            for c in range(8):
                fb[l * 8 + c, 0:1, :] = bl[:, c * 128:(c + 1) * 128]
            if l == 0:
                bl = bl + 1.0
            for pi, p in enumerate(_BSET):
                for qi, q in enumerate(_BSET):
                    for c3 in range(2):
                        acc = None
                        for c1 in range(2):
                            for c2 in range(2):
                                k = float(kap[c1][p] * kap[c2][q])
                                if abs(k) < 1e-12:
                                    continue
                                c = c1 * 4 + c2 * 2 + c3
                                term = bl[:, c * 128:(c + 1) * 128] * k
                                acc = term if acc is None else acc + term
                        for r3 in range(2):
                            row = l * 64 + (pi * 4 + qi) * 4 + r3 * 2 + c3
                            beta[row:row + 1, :] = acc * (_D ** (r3 - c3))
        for c in range(8):
            fin(c).wait()
        for c in range(8):
            v = fxb[c].astype(f32)
            fx32[c] = v
            fx32[8 + c] = v

        def per_layer(l, carry):
            w_copy(l).wait()

            @pl.when(l + 1 < L)
            def _():
                w_copy(l + 1).start()

            @pl.when(l == 1)
            def _():
                x_copy(0).start()
                x_copy(1).start()

            def per_rows(g, c2):
                r0 = pl.multiple_of(g * 16, 16)
                zg = [lax.shift_right_logical(g, 12 + k) for k in range(4)]
                never = jnp.full((16, 128), zg[0], jnp.int32) != 0

                def toff(p, i, t):
                    return ((p - 1) * 37 + (i * 4 + t) * 2 + i) * 8

                pace = []
                for i in range(4):
                    for t in range(4):
                        blk = []
                        for o in range(4):
                            r, c, e = _rowcol(o, i, t)
                            v = wraw[l, pl.ds(r * 128 + r0, 16), c * 128:(c + 1) * 128].astype(f32)
                            blk.append(v * (0.125 * _D ** e))
                        ex = _bexp(blk, ())
                        for p in _PH:
                            tmp[0, toff(p, i, t):toff(p, i, t) + 16, :] = ex[p]
                        pace.append(pltpu.bitcast(ex[7], jnp.uint32))

                src = (l & 1) * 8
                xu = [fxb.bitcast(jnp.uint32)[src + c] for c in range(8)]
                nevr = jnp.full((ROFF // 2, 128), zg[0], jnp.int32) != 0
                for h in range(2):
                    xu[h] = jnp.where(
                        nevr, jnp.concatenate([v[h * 8:h * 8 + 8] for v in pace], 0), xu[h])
                xa = jnp.concatenate([pltpu.bitcast(v, bf16) for v in xu], 1)
                cs = pl.ds(pl.multiple_of(g * 128, 128), 128)
                y1 = jnp.dot(xa[:, :512], wraw[l, :512, cs], preferred_element_type=f32)
                fy[0] = y1 + fb[l * 8 + g, 0:1, :]
                y2 = jnp.dot(xa[:, 512:], wraw[l, 512:, cs], preferred_element_type=f32)
                xn = fx32[g] * (fy[zg[0]] + y2) + fx32[8 + g]
                fx32[8 + g] = xn
                fxb[8 - src + g] = xn.astype(bf16)
                yy = jnp.concatenate([y1, y2], 0)

                def put(p, q, qs):
                    if (p, q) in l3set:
                        if q in (2, 6):
                            qs = [v + v for v in qs]
                        inn = _bexp(qs, (1,))
                        tiles = [inn[r] for r in range(1, 8)]
                    else:
                        f = 2.0 * (2 if p == 1 else 1) * (2 if q in (1, 2, 6) else 1)
                        tiles = [v * f for v in qs]
                    for k, v in enumerate(tiles):
                        wexp[l, tile0[p, q] + k, pl.ds(r0, 16), :] = v.astype(bf16)

                a0, a1 = cfg["pa"]
                n = 0
                for p in _PH:
                    for un in range(3):
                        r = a0 + (a1 - a0) * n // 21
                        n += 1

                        def tl(i, t):
                            v = tmp[zg[1 + un], toff(p, i, t):toff(p, i, t) + 16, :]
                            if i == 1 and t in cfg["pt"]:
                                v = jnp.where(never, yy[r * 8:r * 8 + 16], v)
                            return v

                        if un == 0:
                            x, y = [tl(0, t) for t in range(4)], [tl(1, t) for t in range(4)]
                            put(p, 2, [x[t] - y[t] for t in range(4)])
                            put(p, 6, [x[t] + y[t] for t in range(4)])
                        elif un == 1:
                            x, y = [tl(1, t) for t in range(4)], [tl(3, t) for t in range(4)]
                            put(p, 3, [x[t] - y[t] for t in range(4)])
                            put(p, 5, [x[t] + y[t] for t in range(4)])
                        else:
                            x = [tl(1, t) + tl(2, t) for t in range(4)]
                            y = [tl(0, t) + tl(3, t) for t in range(4)]
                            put(p, 1, y)
                            put(p, 4, [x[t] - y[t] for t in range(4)])
                            put(p, 7, [x[t] + y[t] for t in range(4)])
                return c2

            lax.fori_loop(0, 8, per_rows, 0)
            return carry

        lax.fori_loop(0, L, per_layer, 0)
        for c in range(8):
            fout(c).start()
        x_copy(0).wait()
        ctx.update(z=0, slot={0: 0}, j=-1)
        for w in ("e1", "e2"):
            for t in range(4):
                task[w](L - 1, t, None)

    @pl.when(step + 1 < nsteps)
    def _():
        x_copy(step + 1).wait()

    @pl.when(step + 2 < nsteps)
    def _():
        x_copy(step + 2).start()

    zz = [lax.shift_right_logical(step, 12 + k) for k in range(_NZ)]
    ctx.update(mask=jnp.full((H, 128), zz[0], jnp.int32) != 0,
               slot={-1: (step + 3) & 3, 0: step & 3, 1: (step + 1) & 3}, oslot=step & 1)
    wu = wexp.bitcast(jnp.uint32)

    def wtile(l, k):
        return pltpu.bitcast(wu[l, k], bf16)

    prods = [(l, p, q) for _j in range(TPS) for l in range(L) for (p, q) in order]
    npr = len(prods)
    free = [0, 0, 0, 0]
    anchors = []
    pstart = []
    for pi, (l, p, q) in enumerate(prods):
        pstart.append(min(free))
        if (p, q) in l3set:
            for j in range(7):
                mx = int(np.argmin(free))
                anchors += [(free[mx] + g * 8, pi, j, g) for g in range(NG)]
                free[mx] += H
        else:
            anchors += [(max(free) + g * 8, pi, 0, g) for g in range(2 * NG)]
            free = [f + 2 * H for f in free]
    pstart.append(max(free))
    anchors.sort()
    times = np.array([a[0] for a in anchors])

    def tpos(x):
        i = int(np.floor(x))
        return pstart[i] + (x - i) * (pstart[min(i + 1, npr)] - pstart[i])

    sched = {}
    jobs = [(w, l) for l in range(L - 1) for w in ("w1", "w2", "w3", "w4", "w5")]
    jobs += [(w, L - 1) for w in ("e1", "o1", "e2", "o2", "e4", "e5", "o3", "o4", "o5")]
    for j in range(TPS):
        for jn, (w, l) in enumerate(jobs):
            wn = win.get((w, l), win[w])
            segs = wn if isinstance(wn, list) else [wn]
            cnt = 4 * NG // len(segs)
            slots = []
            jj = j
            for b0, b1 in segs:
                i0, i1 = (j * L + l) * 49 + b0, (j * L + l) * 49 + b1
                if (j * L + l) * 49 + segs[0][0] >= npr:
                    i0, i1, jj = i0 - npr, i1 - npr, j - TPS
                assert i1 <= npr
                for k in range(cnt):
                    ai = int(np.searchsorted(times, tpos(i0) + (tpos(i1) - tpos(i0)) * k / cnt))
                    while anchors[ai][1] < int(i0):
                        ai += 1
                    slots.append(anchors[ai][1:])
            for t in range(4):
                al = slots[t * NG:(t + 1) * NG]
                sched.setdefault(max(a[0] for a in al), []).append((w, l, t, al, jn, jj))

    subs = {}
    l3pos = 0
    for pi, (l, p, q) in enumerate(prods):
        ctx["z"] = zz[{1: 0, 2: 0, 3: 0, 5: 0, 4: 1, 6: 2, 7: 3}[q] + (4 if p == 1 else 0)]
        srcs = ["a3", "a4"] if p == 1 else [f"a{p}"]
        qv = [_lin([(ld(n, b, t), s) for n in srcs for b, s in _MIDB[q]]) for t in range(4)]
        k0 = tile0[p, q]
        if (p, q) in l3set:
            a1 = qv[0] + qv[3]
            u = qv[1] + qv[2]
            av = {1: a1, 3: qv[0] - qv[1], 5: qv[0] + qv[1], 4: qv[1] + qv[3],
                  7: qv[1] - qv[3], 2: u + a1, 6: u - a1}
            so = cfg["so"][l3pos % 4]
            l3pos += 1
            m = {r: jnp.dot(av[r].astype(bf16), wtile(l, k0 + r - 1), preferred_element_type=f32)
                 for r in so}
            subs[pi] = [m[r] for r in so]
            mq = _comb7(m)
        else:
            a = jnp.concatenate(
                [jnp.concatenate(qv[:2], 1), jnp.concatenate(qv[2:], 1)], 0).astype(bf16)
            wt = [wtile(l, k0 + t) for t in range(4)]
            wm = jnp.concatenate([jnp.concatenate(wt[:2], 1), jnp.concatenate(wt[2:], 1)], 0)
            mm = jnp.dot(a, wm, preferred_element_type=f32)
            subs[pi] = [mm[:, :128]]
            mq = [mm[:H, :128], mm[:H, 128:], mm[H:, :128], mm[H:, 128:]]
        if p in _BSET and q in _BSET:
            row = l * 64 + (_BSET.index(p) * 4 + _BSET.index(q)) * 4
            mq = [mq[t] + beta[row + t:row + t + 1, :] for t in range(4)]
        for t in range(4):
            v = mq[t]
            if p == 5:
                v = v + ld("u3", q - 1, t)
            elif p == 1:
                r3 = ld("u3", q - 1, t)
                v = v + (((ld("u4", q - 1, t) + ld("u7", q - 1, t)) + (r3 + r3)) - ld("u5", q - 1, t))
            elif p == 2:
                v = v + ld("u4", q - 1, t)
            elif p == 6:
                v = v - ld("u7", q - 1, t)
            st(uname(p, l), q - 1, t, v)
        for (w, tl, t, al, jn, jj) in sched.get(pi, []):
            a = jnp.concatenate([subs[api][j][g * 8:(g + 1) * 8, :] for api, j, g in al], 0)
            ctx.update(z=zz[8 + jn % 6], j=jj)
            task[w](tl, t, a)

    @pl.when(step >= 1)
    def _():
        top_copy(step - 1).wait()

    @pl.when(step >= 2)
    def _():
        bot_copy(step - 1).wait()

    top_copy(step).start()

    @pl.when(step >= 1)
    def _():
        bot_copy(step).start()

    @pl.when(step == nsteps - 1)
    def _():
        ctx.update(z=0, slot={-1: (nsteps - 1) % 4}, j=-1, oslot=nsteps % 2)
        for w in ("o3", "o4", "o5"):
            for t in range(4):
                task[w](L - 1, t, None)
        bot_copy(nsteps).start()
        for c in range(8):
            fout(c).wait()
        top_copy(nsteps - 1).wait()
        bot_copy(nsteps - 1).wait()
        bot_copy(nsteps).wait()


_L3SET = tuple((p, q) for p in range(2, 8) for q in range(2, 8))
_WIN = {"w1": (24, 34), "w2": (36, 45), "w3": (44, 48.5), "w4": (49, 60), "w5": (63, 73),
        "e1": (11, 16), "o1": (24, 34), "e2": (35, 46), "o2": (36, 48.5), "e4": (49, 60), "e5": (63, 73),
        "o3": (49, 60),
        "o4": [(60, 63), (109, 112), (158, 161), (207, 210)],
        "o5": [(83, 85), (132, 134), (181, 183), (256, 259)]}
_SO = ((3, 5, 1, 4, 7, 2, 6), (1, 3, 5, 4, 7, 2, 6), (3, 5, 1, 4, 7, 2, 6), (3, 5, 1, 4, 7, 2, 6))
_CFG = dict(l3set=_L3SET, win=_WIN, tm=384, tps=1, roff=256, pa=(16, 62), pt=(0, 1), so=_SO, qo=(3, 5, 2, 4, 7, 6, 1))


def _build(**kw):
    cfg = dict(_CFG, **kw)

    def fn(x0, ws, bs):
        B, Dm = x0.shape
        L = ws.shape[0]
        st = cfg["tm"] * cfg["tps"]
        nsteps = (B - cfg["roff"]) // st
        ntiles = _plan(cfg["l3set"], cfg)[2]
        return pl.pallas_call(
            functools.partial(_kernel, L=L, nsteps=nsteps, cfg=cfg),
            grid=(nsteps,),
            in_specs=[
                pl.BlockSpec(memory_space=pl.ANY),
                pl.BlockSpec(memory_space=pl.ANY),
                pl.BlockSpec((L, Dm), lambda i: (0, 0), pipeline_mode=pl.Buffered(1)),
            ],
            out_specs=pl.BlockSpec(memory_space=pl.ANY),
            out_shape=jax.ShapeDtypeStruct((B, Dm), x0.dtype),
            scratch_shapes=[
                pltpu.VMEM((4, st, Dm), bf16),
                pltpu.VMEM((2, st, Dm), bf16),
                pltpu.VMEM((L, Dm, Dm), bf16),
                pltpu.VMEM((L, ntiles, 128, 128), bf16),
                pltpu.VMEM((L * 64, 128), f32),
                pltpu.VMEM((1, cfg["roff"], 128), f32),
                pltpu.VMEM((16, cfg["roff"], 128), f32),
                pltpu.VMEM((16, cfg["roff"], 128), bf16),
                pltpu.VMEM((L * 8, 8, 128), f32),
                pltpu.SemaphoreType.DMA((4,)),
                pltpu.SemaphoreType.DMA((L,)),
                pltpu.SemaphoreType.DMA((2,)),
                pltpu.SemaphoreType.DMA((2,)),
                pltpu.SemaphoreType.DMA((8,)),
            ]
            + [pltpu.VMEM((1, 260 * 8, 128), f32)]
            + [pltpu.VMEM((1, ((n * _bs(cfg["tm"]) + 7) // 4 * 4) * 8, 128), f32)
               for _, n in _NAMES for _t in range(4)],
            compiler_params=pltpu.CompilerParams(
                dimension_semantics=("arbitrary",),
                vmem_limit_bytes=126 * 1024 * 1024,
                disable_bounds_checks=True,
            ),
        )(x0, ws, bs)

    return fn


@jax.jit
def pallas_standalone__dcn_v2_cross__recsys_kernel(
    x0: jax.Array,
    ws: jax.Array,
    bs: jax.Array,
):
    return _build()(x0, ws, bs)
```

```python
import functools

import numpy as np
import jax
import jax.numpy as jnp
from jax import lax
import jax.experimental.pallas as pl
import jax.experimental.pallas.tpu as pltpu

f32 = jnp.float32
bf16 = jnp.bfloat16

_D = float(np.sqrt(3.0))
_PH = (3, 5, 4, 7, 1, 2, 6)
_MIDB = {1: [(0, 1)], 2: [(1, 1)], 3: [(2, 1)], 5: [(3, 1)],
         4: [(0, 1), (2, -1)], 6: [(1, 1), (0, -1)], 7: [(3, 1), (0, -1)]}
_CVEC = {1: [1, 0, 0, 1], 2: [0, 0, 1, -1], 3: [1, 1, 1, 1], 4: [1, 0, 1, 0],
         5: [-1, 1, 1, -1], 6: [0, 0, 1, 1], 7: [1, 0, -1, 0]}
_BSET = (3, 4, 7, 1)
_NZ = 14


def _bs(tm):
    ng = tm // 64
    return ng // 4 * 4 + (1 if ng % 4 == 0 else 5)


def _kappa():
    m = np.array([_CVEC[p] for p in _BSET], np.float64).T
    pats = [np.array([1, 0, _D, 0]), np.array([0, 1 / _D, 0, 1])]
    return [dict(zip(_BSET, np.linalg.solve(m, t))) for t in pats]


def _lin(terms):
    terms = sorted(terms, key=lambda t: -t[1])
    acc = terms[0][0]
    for v, s in terms[1:]:
        acc = acc + v if s > 0 else acc - v
    return acc


def _comb7(m):
    s = m[3] + m[5]
    e = (m[3] - m[5]) + m[1]
    return [(e + m[4]) + m[7], s, (((s + m[4]) - m[7]) + m[2]) + m[6], (e - m[2]) + m[6]]


def _fwd(x):
    a1 = x[0] + x[3]
    return [a1, ((x[1] + x[2]) + a1) * 0.5, x[0] - x[1], x[0] + x[1]]


def _bexp(b, dbl):
    b1 = b[0] + b[3]
    u = b[1] + b[2]
    o = {1: b1, 2: b[0] - b[1], 3: b[1] - b[3], 4: u - b1, 5: b[1] + b[3], 6: b[0] + b[1], 7: u + b1}
    for p in dbl:
        o[p] = o[p] + o[p]
    return o


def _rowcol(o, i, t):
    r = (o // 2) * 4 + (i // 2) * 2 + t // 2
    c = (o % 2) * 4 + (i % 2) * 2 + t % 2
    e = (o // 2 - o % 2) + (i // 2 - i % 2) + (t // 2 - t % 2)
    return r, c, e


def _plan(l3set, cfg):
    order = []
    for p in _PH:
        ks = [q for q in range(1, 8) if (p, q) not in l3set]
        ls = [q for q in cfg["qo"] if (p, q) in l3set]
        kp = cfg["kpos"][p]
        order += [(p, q) for q in ls[:kp] + ks + ls[kp:]]
    tile0 = {}
    n = 0
    for pq in order:
        tile0[pq] = n
        n += 7 if pq in l3set else 4
    return order, tile0, n


_NAMES = ([(f"u{p}", 7) for p in (3, 4, 7, 5, 1, 2, 6)]
          + [(f"a{p}", 4) for p in (3, 4, 5, 7, 2, 6)]
          + [(f"{s}{k}", 4) for s in ("fx", "H", "G", "U", "V") for k in range(2)]
          + [(f"x0{o}", 4) for o in range(4)]
          + [("u2x", 7), ("u6x", 7)] + [(f"{s}{k}", 4) for s in "HGUV" for k in (2, 3)])


def _kernel(x_hbm, w_hbm, b_hbm, o_hbm, b_ref, ring, stage, wraw, wexp, beta, fx32, fxb, fb,
            xsem, wsem, tsem, bsem, fsem, *bufs, L, nsteps, cfg):
    l3set, win, TM, TPS, ROFF = cfg["l3set"], cfg["win"], cfg["tm"], cfg["tps"], cfg["roff"]
    H = TM // 8
    NG = H // 8
    HT = TM // 2
    ST = TM * TPS
    BS = _bs(TM)
    order, tile0, _ = _plan(l3set, cfg)
    tmp = bufs[:2]
    buf = dict(zip([(n, t) for n, _ in _NAMES for t in range(4)], bufs[2:]))
    skew = {n: k % 4 for k, (n, _) in enumerate(_NAMES)}
    ctx = {}

    def x_copy(i):
        return pltpu.make_async_copy(
            x_hbm.at[pl.ds(pl.multiple_of(ROFF + i * ST, 64), ST)], ring.at[i & 3], xsem.at[i & 3])

    def w_copy(l, c):
        return pltpu.make_async_copy(
            w_hbm.at[l, :, pl.ds(c * 128, 128)], wraw.at[l, c], wsem.at[l])

    def w_start(l):
        for c in range(8):
            w_copy(l, c).start()

    def w_wait(l):
        for c in range(8):
            w_copy(l, c).wait()

    def top_copy(i):
        return pltpu.make_async_copy(
            stage.at[i & 1, pl.ds(HT, ST - HT)],
            o_hbm.at[pl.ds(pl.multiple_of(ROFF + i * ST, 64), ST - HT)], tsem.at[i & 1])

    def bot_copy(i):
        return pltpu.make_async_copy(
            stage.at[i & 1, pl.ds(0, HT)],
            o_hbm.at[pl.ds(pl.multiple_of(ROFF + i * ST - HT, 64), HT)], bsem.at[i & 1])

    def fin(c):
        return pltpu.make_async_copy(
            x_hbm.at[pl.ds(0, ROFF), pl.ds(c * 128, 128)], fxb.at[c], fsem.at[c])

    def fout(c):
        return pltpu.make_async_copy(
            fxb.at[(L & 1) * 8 + c], o_hbm.at[pl.ds(0, ROFF), pl.ds(c * 128, 128)], fsem.at[c])

    def off(n, b, t):
        return ((skew[n] + t) % 4 + b * BS) * 8

    def ld(n, b, t):
        o = off(n, b, t)
        return buf[n, t][ctx["z"], o:o + H, :]

    def st(n, b, t, v):
        o = off(n, b, t)
        buf[n, t][0, o:o + H, :] = v

    def anc(v, a):
        return v if a is None else jnp.where(ctx["mask"], a, v)

    def xin(j, o, i, t):
        r, c, _ = _rowcol(o, i, t)
        r0 = (j % TPS) * TM + r * H
        return ring[ctx["slot"][j // TPS], r0:r0 + H, c * 128:(c + 1) * 128].astype(f32)

    def sname(s, l):
        return f"{s}{l - L + 4 if l >= L - 2 else l % 2}"

    def uname(p, l):
        return f"u{p}x" if (l == L - 1 and p in (2, 6)) else f"u{p}"

    def emit(o, g, t):
        for i in range(4):
            r, c, e = _rowcol(o, i, t)
            y = xin(ctx["j"], o, i, t) * g[i]
            if e:
                y = y * (_D ** -e)
            r0 = ctx["j"] * TM + r * H + HT
            stage[ctx["oslot"], r0:r0 + H, c * 128:(c + 1) * 128] = y.astype(bf16)

    def fresh(o, t, a):
        xs = []
        for i in range(4):
            e = _rowcol(o, i, t)[2]
            v = xin(ctx["j"] + 1, o, i, t)
            if i == 0:
                v = anc(v, a)
            st(f"x0{o}", i, t, v)
            xs.append(v * (_D ** e) if e else v)
        return xs

    def gate(o, g, t):
        return [ld(f"x0{o}", i, t) * g[i] for i in range(4)]

    def upd(l, p, s, t, a, keep=True):
        m = {q: ld(uname(p, l), q - 1, t) for q in range(1, 8)}
        m[3] = anc(m[3], a)
        y = _comb7(m)
        if l > 0:
            y = [y[i] + ld(sname(s, l - 1), i, t) for i in range(4)]
        if keep:
            for i in range(4):
                st(sname(s, l), i, t, y[i])
        return y

    def f1(l, t, x):
        for i, v in enumerate(_fwd(x)):
            st(f"fx{l % 2}", i, t, v)

    def f2(l, t, x):
        for i, v in enumerate(_fwd(x)):
            w = ld(f"fx{l % 2}", i, t)
            st("a3", i, t, v - w)
            st("a5", i, t, v + w)

    def f4(l, t, x):
        for i, v in enumerate(_fwd(x)):
            w = ld(f"fx{l % 2}", i, t)
            st("a4", i, t, w + v)
            st("a7", i, t, w - v)

    def f5(l, t, x):
        for i, v in enumerate(_fwd(x)):
            u = ld(f"fx{l % 2}", i, t) + v
            a1 = ld("a3", i, t) + ld("a4", i, t)
            st("a2", i, t, u + a1)
            st("a6", i, t, u - a1)

    def w4(l, t, a):
        v6 = upd(l, 6, "V", t, a)
        g = [v6[i] + (ld(sname("G", l), i, t) - ld(sname("U", l), i, t)) for i in range(4)]
        f4(l, t, gate(3, g, t))

    def w5(l, t, a):
        g = [anc(ld(sname("U", l), i, t), a if i == 0 else None)
             + ld(sname("V", l), i, t) + ld(sname("H", l), i, t) for i in range(4)]
        f5(l, t, gate(2, g, t))

    def o4(l, t, a):
        v6 = upd(l, 6, "V", t, a)
        emit(3, [v6[i] + (ld(sname("G", l), i, t) - ld(sname("U", l), i, t)) for i in range(4)], t)

    def o5(l, t, a):
        emit(2, [anc(ld(sname("U", l), i, t), a) + ld(sname("V", l), i, t) + ld(sname("H", l), i, t)
                 for i in range(4)], t)

    task = {
        "w1": lambda l, t, a: f1(l, t, gate(1, upd(l, 5, "H", t, a), t)),
        "w2": lambda l, t, a: f2(l, t, gate(0, upd(l, 1, "G", t, a), t)),
        "w3": lambda l, t, a: upd(l, 2, "U", t, a),
        "w4": w4,
        "w5": w5,
        "o1": lambda l, t, a: emit(1, upd(l, 5, "H", t, a), t),
        "o2": lambda l, t, a: emit(0, upd(l, 1, "G", t, a), t),
        "o3": lambda l, t, a: upd(l, 2, "U", t, a),
        "o4": o4,
        "o5": o5,
        "e1": lambda l, t, a: f1(l, t, fresh(1, t, a)),
        "e2": lambda l, t, a: f2(l, t, fresh(0, t, a)),
        "e4": lambda l, t, a: f4(l, t, fresh(3, t, a)),
        "e5": lambda l, t, a: f5(l, t, fresh(2, t, a)),
    }

    b_copy = pltpu.make_async_copy(b_hbm, b_ref, fsem.at[8])
    b_copy.start()
    w_start(0)
    for c in range(8):
        fin(c).start()
    b_copy.wait()
    kap = _kappa()
    for l in range(L):
        bl = b_ref[l:l + 1, :].astype(f32)
        for c in range(8):
            fb[l * 8 + c, 0:1, :] = bl[:, c * 128:(c + 1) * 128]
        if l == 0:
            bl = bl + 1.0
        for pi, p in enumerate(_BSET):
            for qi, q in enumerate(_BSET):
                for c3 in range(2):
                    acc = None
                    for c1 in range(2):
                        for c2 in range(2):
                            k = float(kap[c1][p] * kap[c2][q])
                            if abs(k) < 1e-12:
                                continue
                            c = c1 * 4 + c2 * 2 + c3
                            term = bl[:, c * 128:(c + 1) * 128] * k
                            acc = term if acc is None else acc + term
                    for r3 in range(2):
                        row = l * 64 + (pi * 4 + qi) * 4 + r3 * 2 + c3
                        beta[row:row + 1, :] = acc * (_D ** (r3 - c3))
    for c in range(8):
        fin(c).wait()
    for c in range(8):
        v = fxb[c].astype(f32)
        fx32[c] = v
        fx32[8 + c] = v

    def toff(p, i, t):
        return ((p - 1) * 37 + (i * 4 + t) * 2 + i) * 8

    def s1_units(l, g, dst):
        r0 = pl.multiple_of(g * 16, 16)

        def unit(i, t):
            blk = []
            for o in range(4):
                r, c, e = _rowcol(o, i, t)
                v = wraw[l, c, pl.ds(r * 128 + r0, 16), :].astype(f32)
                blk.append(v * (0.125 * _D ** e))
            ex = _bexp(blk, ())
            for p in _PH:
                dst[0, toff(p, i, t):toff(p, i, t) + 16, :] = ex[p]
            return [ex[7][:8], ex[7][8:]]

        return [(34, functools.partial(unit, i, t)) for i in range(4) for t in range(4)]

    def s2_units(l, g, src, zg):
        r0 = pl.multiple_of(g * 16, 16)

        def put(p, q, qs):
            if (p, q) in l3set:
                f = (2.0 if p == 1 else 1.0) * (2 if q in (1, 2, 6) else 1)
                if f != 1:
                    qs = [v * f for v in qs]
                inn = _bexp(qs, (1,))
                tiles = [inn[r] for r in range(1, 8)]
            else:
                f = 2.0 * (2 if p == 1 else 1) * (2 if q in (1, 2, 6) else 1)
                tiles = [v * f for v in qs]
            for k, v in enumerate(tiles):
                wexp[l, tile0[p, q] + k, pl.ds(r0, 16), :] = v.astype(bf16)
            return tiles

        def unit(p, un, a=None):
            def tl(i):
                vs = [src[zg[1 + un], toff(p, i, t):toff(p, i, t) + 16, :] for t in range(4)]
                if a is not None and i == 1:
                    nv = jnp.full((16, 128), zg[0], jnp.int32) != 0
                    for t in cfg["pt"]:
                        vs[t] = jnp.where(nv, a, vs[t])
                return vs

            if un == 0:
                x, y, qa, qb = tl(0), tl(1), 2, 6
            elif un == 1:
                x, y, qa, qb = tl(1), tl(3), 3, 5
            else:
                x = [u + v for u, v in zip(tl(1), tl(2))]
                y = [u + v for u, v in zip(tl(0), tl(3))]
                qa, qb = 4, 7
                put(p, 1, y)
            ta = put(p, qa, [u - v for u, v in zip(x, y)])
            tb = put(p, qb, [u + v for u, v in zip(x, y)])
            if len(tb) == 4:
                return [v[:8] for v in tb]
            return [ta[-1][:8], tb[-1][8:]]

        cost = lambda p, un: (40, 40, 68)[un] if p == 1 else (82, 66, 94)[un]
        return [(cost(p, un), functools.partial(unit, p, un)) for p in _PH for un in range(3)]

    def half(l, g, ln, gn, src, dst, zg, tail):
        u2 = s2_units(l, g, src, zg)
        u1 = s1_units(ln, gn, dst)
        units = sorted([(k / len(u2), c, f) for k, (c, f) in enumerate(u2)]
                       + [((k + 0.5) / len(u1) * cfg["s1f"], c, f) for k, (c, f) in enumerate(u1)],
                       key=lambda e: e[0])
        late = [f for _, _, f in units[len(units) - len(tail):]]
        units = units[:len(units) - len(tail)]
        total = sum(c for _, c, _ in units)
        nsl = ROFF // 16
        links = {}
        acc = 0
        for _, c, f in units:
            acc += c
            vals = f()
            sl = min(int(np.ceil(acc / total * 2 * nsl)), 2 * nsl) - 1
            links.setdefault(sl, []).extend(vals)
        fsrc = (l & 1) * 8
        fu = fxb.bitcast(jnp.uint32)
        never = jnp.full((8, 128), zg[0], jnp.int32) != 0
        cols = []
        for c in range(8):
            rows = []
            for r in range(nsl):
                v = fu[fsrc + c, r * 8:(r + 1) * 8, :]
                for a in links.get((c // 4) * nsl + r, [])[c % 4::4]:
                    v = jnp.where(never, pltpu.bitcast(a, jnp.uint32), v)
                rows.append(v)
            cols.append(pltpu.bitcast(jnp.concatenate(rows, 0), bf16))
        wg = pltpu.bitcast(wraw.bitcast(jnp.uint32)[l, g], bf16)
        y = jnp.dot(jnp.concatenate(cols, 1), wg, preferred_element_type=f32)
        xn = fx32[g] * (y + fb[l * 8 + g, 0:1, :]) + fx32[8 + g]
        fx32[8 + g] = xn
        fxb[8 - fsrc + g] = xn.astype(bf16)
        for r, f in zip(tail, late):
            f(y[r * 8:r * 8 + 16])

    w_wait(0)
    w_start(1)
    for _, f in s1_units(0, 0, tmp[0]):
        f()

    def pair(n, carry):
        l = lax.shift_right_logical(n, 2)
        g = (n & 3) * 2

        @pl.when(jnp.logical_and(g == 6, l + 1 < L))
        def _():
            w_wait(l + 1)

        @pl.when(jnp.logical_and(g == 6, l + 2 < L))
        def _():
            w_start(l + 2)

        @pl.when(n == 8)
        def _():
            x_copy(0).start()
            x_copy(1).start()

        zg = [lax.shift_right_logical(n, 12 + k) for k in range(8)]
        nn = jnp.minimum(2 * n + 2, 8 * L - 1)
        half(l, g, l, g + 1, tmp[0], tmp[1], zg[:4], ())
        half(l, g + 1, lax.shift_right_logical(nn, 3), nn & 7, tmp[1], tmp[0], zg[4:], cfg["tail"])
        return carry

    lax.fori_loop(0, 4 * L, pair, 0)
    for c in range(8):
        fout(c).start()
    x_copy(0).wait()
    ctx.update(z=0, slot={0: 0}, j=-1)
    for w in ("e1", "e2"):
        for t in range(4):
            task[w](L - 1, t, None)

    def main(step, carry):
        @pl.when(step + 1 < nsteps)
        def _():
            x_copy(step + 1).wait()

        @pl.when(step + 2 < nsteps)
        def _():
            x_copy(step + 2).start()

        zz = [lax.shift_right_logical(step, 12 + k) for k in range(_NZ)]
        ctx.update(mask=jnp.full((H, 128), zz[0], jnp.int32) != 0,
                   slot={-1: (step + 3) & 3, 0: step & 3, 1: (step + 1) & 3}, oslot=step & 1)
        wu = wexp.bitcast(jnp.uint32)

        def wtile(l, k):
            return pltpu.bitcast(wu[l, k], bf16)

        prods = [(l, p, q) for _j in range(TPS) for l in range(L) for (p, q) in order]
        npr = len(prods)
        free = [0, 0, 0, 0]
        anchors = []
        pstart = []
        for pi, (l, p, q) in enumerate(prods):
            pstart.append(min(free))
            if (p, q) in l3set:
                for j in range(7):
                    mx = int(np.argmin(free))
                    anchors += [(free[mx] + g * 8, pi, j, g) for g in range(NG)]
                    free[mx] += H
            else:
                anchors += [(max(free) + g * 8, pi, 0, g) for g in range(2 * NG)]
                free = [f + 2 * H for f in free]
        pstart.append(max(free))
        anchors.sort()
        times = np.array([a[0] for a in anchors])

        def tpos(x):
            i = int(np.floor(x))
            return pstart[i] + (x - i) * (pstart[min(i + 1, npr)] - pstart[i])

        wv, ws, wl = cfg["wts"]
        P = 4 * NG
        nb = pstart[-1] // 8 + 1
        load = np.zeros(nb)

        def spread(t0, t1, valu, st_, ld_):
            b0, b1 = max(int(t0 // 8), 0), max(int(t1 // 8), 1)
            load[b0:b1] += (valu / 4 * wv + st_ * ws + ld_ / 3 * wl) / max(int(t1 // 8) - int(t0 // 8), 1)

        for pi, (l, p, q) in enumerate(prods):
            t = len(_MIDB[q]) * (2 if p == 1 else 1)
            big = (p, q) in l3set
            t0, t1 = pstart[pi], pstart[pi + 1]
            spread(t0 - cfg["lat"], t1 - cfg["lat"], (t - 1 + (2.875 if big else 0.5)) * P, 0,
                   t * P + (56 if big else 32))
            sa, sl = {5: (1, 1), 1: (5, 4), 2: (1, 1), 6: (1, 1)}.get(p, (0, 0))
            bias = 1 if (p in _BSET and q in _BSET) else 0
            spread(t0, t1 + (H // 2 if big else 0), ((2.75 if big else 1) + bias + sa) * P, P, sl * P)

        tcost = {"w1": (26, 8, 15), "w2": (34, 12, 19), "w3": (16, 4, 11), "w4": (42, 12, 27),
                 "w5": (35, 8, 28), "o1": (31, 8, 15), "o2": (31, 8, 15), "o3": (16, 4, 11),
                 "o4": (39, 8, 23), "o5": (27, 4, 16), "e1": (14, 8, 4), "e2": (22, 12, 8),
                 "e4": (22, 12, 8), "e5": (30, 12, 16)}
        kern = np.hanning(cfg["sm"] + 2)[1:-1]
        kern /= kern.sum()
        sched = {}
        jobs = [(w, l) for l in range(L - 1) for w in ("w1", "w2", "w3", "w4", "w5")]
        jobs += [(w, L - 1) for w in ("e1", "o1", "e2", "o2", "e4", "e5", "o3", "o4", "o5")]
        todo = [(jn, w, l, j) for j in range(TPS) for jn, (w, l) in enumerate(jobs)]
        wof = lambda w, l: win.get((w, l), win[w])
        todo.sort(key=lambda e: wof(e[1], e[2])[1] - wof(e[1], e[2])[0])
        for jn, w, l, j in todo:
            b0, b1 = wof(w, l)
            i0, i1, jj = (j * L + l) * 49 + b0, (j * L + l) * 49 + b1, j
            if i0 >= npr:
                i0, i1, jj = i0 - npr, i1 - npr, j - TPS
            assert i1 <= npr
            lo, hi = int(np.ceil(tpos(i0) / 8)), int(tpos(i1) // 8)
            picks = []
            for _k in range(P):
                sm = np.convolve(load, kern, mode="same")
                bb = lo + int(np.argmin(sm[lo + 1:hi + 1]))
                picks.append(bb)
                spread(bb * 8, bb * 8 + 24, *tcost[w])
            slots = []
            for bb in sorted(picks):
                ai = int(np.searchsorted(times, bb * 8))
                while anchors[ai][1] < int(i0):
                    ai += 1
                slots.append(anchors[ai][1:])
            for t in range(4):
                al = slots[t * NG:(t + 1) * NG]
                sched.setdefault(max(a[0] for a in al), []).append((w, l, t, al, jn, jj))
        for v in sched.values():
            v.sort(key=lambda e: (e[5], e[4], e[2]))

        subs = {}
        l3pos = 0
        for pi, (l, p, q) in enumerate(prods):
            ctx["z"] = zz[{1: 0, 2: 0, 3: 0, 5: 0, 4: 1, 6: 2, 7: 3}[q] + (4 if p == 1 else 0)]
            srcs = ["a3", "a4"] if p == 1 else [f"a{p}"]
            qv = [_lin([(ld(n, b, t), s) for n in srcs for b, s in _MIDB[q]]) for t in range(4)]
            k0 = tile0[p, q]
            if (p, q) in l3set:
                a1 = qv[0] + qv[3]
                u = qv[1] + qv[2]
                av = {1: a1, 3: qv[0] - qv[1], 5: qv[0] + qv[1], 4: qv[1] + qv[3],
                      7: qv[1] - qv[3], 2: u + a1, 6: u - a1}
                so = cfg["so"][l3pos % 4]
                l3pos += 1
                m = {r: jnp.dot(av[r].astype(bf16), wtile(l, k0 + r - 1), preferred_element_type=f32)
                     for r in so}
                subs[pi] = [m[r] for r in so]
                mq = _comb7(m)
            else:
                a = jnp.concatenate(
                    [jnp.concatenate(qv[:2], 1), jnp.concatenate(qv[2:], 1)], 0).astype(bf16)
                wt = [wtile(l, k0 + t) for t in range(4)]
                wm = jnp.concatenate([jnp.concatenate(wt[:2], 1), jnp.concatenate(wt[2:], 1)], 0)
                mm = jnp.dot(a, wm, preferred_element_type=f32)
                subs[pi] = [mm[:, :128]]
                mq = [mm[:H, :128], mm[:H, 128:], mm[H:, :128], mm[H:, 128:]]
            if p in _BSET and q in _BSET:
                row = l * 64 + (_BSET.index(p) * 4 + _BSET.index(q)) * 4
                mq = [mq[t] + beta[row + t:row + t + 1, :] for t in range(4)]
            for t in range(4):
                v = mq[t]
                if p == 5:
                    v = v + ld("u3", q - 1, t)
                elif p == 1:
                    r3 = ld("u3", q - 1, t)
                    v = v + (((ld("u4", q - 1, t) + ld("u7", q - 1, t)) + (r3 + r3)) - ld("u5", q - 1, t))
                elif p == 2:
                    v = v + ld("u4", q - 1, t)
                elif p == 6:
                    v = v - ld("u7", q - 1, t)
                st(uname(p, l), q - 1, t, v)
            for (w, tl, t, al, jn, jj) in sched.get(pi, []):
                a = jnp.concatenate([subs[api][j][g * 8:(g + 1) * 8, :] for api, j, g in al], 0)
                ctx.update(z=zz[8 + jn % 6], j=jj)
                task[w](tl, t, a)

        @pl.when(step >= 1)
        def _():
            top_copy(step - 1).wait()

        @pl.when(step >= 2)
        def _():
            bot_copy(step - 1).wait()

        top_copy(step).start()

        @pl.when(step >= 1)
        def _():
            bot_copy(step).start()

        return carry

    lax.fori_loop(0, nsteps, main, 0)

    ctx.update(z=0, slot={-1: (nsteps - 1) % 4}, j=-1, oslot=nsteps % 2)
    for w in ("o3", "o4", "o5"):
        for t in range(4):
            task[w](L - 1, t, None)
    bot_copy(nsteps).start()
    for c in range(8):
        fout(c).wait()
    top_copy(nsteps - 1).wait()
    bot_copy(nsteps - 1).wait()
    bot_copy(nsteps).wait()


_L3SET = tuple((p, q) for p in range(2, 8) for q in range(2, 8))
_WIN = {"w1": (24, 35), "w2": (35, 46), "w3": (42, 49), "w4": (49, 60), "w5": (60, 73),
        "e1": (0, 35), "o1": (14, 35), "e2": (35, 46), "o2": (35, 48.5), "e4": (49, 60), "e5": (60, 80),
        "o3": (49, 60), "o4": (60, 170), "o5": (170, 290)}
_SO = ((3, 5, 1, 4, 7, 2, 6), (1, 3, 5, 4, 7, 2, 6), (3, 5, 1, 4, 7, 2, 6), (3, 5, 1, 4, 7, 2, 6))
_CFG = dict(l3set=_L3SET, win=_WIN, tm=384, tps=1, roff=256, kpos={3: 4, 5: 2, 4: 4, 7: 2, 1: 0, 2: 4, 6: 2}, wts=(1, 0.2, 0), lat=135, sm=6, s1f=0.75, tail=(14, 17, 20, 23, 26), pt=(1,), so=_SO, qo=(3, 5, 2, 4, 7, 6, 1))


def _build(**kw):
    cfg = dict(_CFG, **kw)

    def fn(x0, ws, bs):
        B, Dm = x0.shape
        L = ws.shape[0]
        st = cfg["tm"] * cfg["tps"]
        nsteps = (B - cfg["roff"]) // st
        ntiles = _plan(cfg["l3set"], cfg)[2]
        return pl.pallas_call(
            functools.partial(_kernel, L=L, nsteps=nsteps, cfg=cfg),
            in_specs=[
                pl.BlockSpec(memory_space=pl.ANY),
                pl.BlockSpec(memory_space=pl.ANY),
                pl.BlockSpec(memory_space=pl.ANY),
            ],
            out_specs=pl.BlockSpec(memory_space=pl.ANY),
            out_shape=jax.ShapeDtypeStruct((B, Dm), x0.dtype),
            scratch_shapes=[
                pltpu.VMEM((L, Dm), bf16),
                pltpu.VMEM((4, st, Dm), bf16),
                pltpu.VMEM((2, st, Dm), bf16),
                pltpu.VMEM((L, 8, Dm, 128), bf16),
                pltpu.VMEM((L, ntiles, 128, 128), bf16),
                pltpu.VMEM((L * 64, 128), f32),
                pltpu.VMEM((16, cfg["roff"], 128), f32),
                pltpu.VMEM((16, cfg["roff"], 128), bf16),
                pltpu.VMEM((L * 8, 8, 128), f32),
                pltpu.SemaphoreType.DMA((4,)),
                pltpu.SemaphoreType.DMA((L,)),
                pltpu.SemaphoreType.DMA((2,)),
                pltpu.SemaphoreType.DMA((2,)),
                pltpu.SemaphoreType.DMA((9,)),
            ]
            + [pltpu.VMEM((1, 260 * 8, 128), f32)] * 2
            + [pltpu.VMEM((1, ((n * _bs(cfg["tm"]) + 7) // 4 * 4) * 8, 128), f32)
               for _, n in _NAMES for _t in range(4)],
            compiler_params=pltpu.CompilerParams(
                vmem_limit_bytes=126 * 1024 * 1024,
                disable_bounds_checks=True,
            ),
        )(x0, ws, bs)

    return fn


@jax.jit
def pallas_standalone__dcn_v2_cross__recsys_kernel(
    x0: jax.Array,
    ws: jax.Array,
    bs: jax.Array,
):
    return _build()(x0, ws, bs)
```

```python
import functools

import numpy as np
import jax
import jax.numpy as jnp
from jax import lax
import jax.experimental.pallas as pl
import jax.experimental.pallas.tpu as pltpu

f32 = jnp.float32
bf16 = jnp.bfloat16

_D = float(np.sqrt(3.0))
_PH = (3, 5, 4, 7, 1, 2, 6)
_MIDB = {1: [(0, 1)], 2: [(1, 1)], 3: [(2, 1)], 5: [(3, 1)],
         4: [(0, 1), (2, -1)], 6: [(1, 1), (0, -1)], 7: [(3, 1), (0, -1)]}
_CVEC = {1: [1, 0, 0, 1], 2: [0, 0, 1, -1], 3: [1, 1, 1, 1], 4: [1, 0, 1, 0],
         5: [-1, 1, 1, -1], 6: [0, 0, 1, 1], 7: [1, 0, -1, 0]}
_NZ = 14


def _bs(tm):
    ng = tm // 64
    return ng // 4 * 4 + (1 if ng % 4 == 0 else 5)


def _kappa(bset):
    m = np.array([_CVEC[p] for p in bset], np.float64).T
    pats = [np.array([1, 0, _D, 0]), np.array([0, 1 / _D, 0, 1])]
    return [dict(zip(bset, np.linalg.solve(m, t))) for t in pats]


def _lin(terms):
    terms = sorted(terms, key=lambda t: -t[1])
    acc = terms[0][0]
    for v, s in terms[1:]:
        acc = acc + v if s > 0 else acc - v
    return acc


def _comb7(m):
    s = m[3] + m[5]
    e = (m[3] - m[5]) + m[1]
    return [(e + m[4]) + m[7], s, (((s + m[4]) - m[7]) + m[2]) + m[6], (e - m[2]) + m[6]]


def _fwd(x):
    a1 = x[0] + x[3]
    return [a1, ((x[1] + x[2]) + a1) * 0.5, x[0] - x[1], x[0] + x[1]]


def _bexp(b, dbl):
    b1 = b[0] + b[3]
    u = b[1] + b[2]
    o = {1: b1, 2: b[0] - b[1], 3: b[1] - b[3], 4: u - b1, 5: b[1] + b[3], 6: b[0] + b[1], 7: u + b1}
    for p in dbl:
        o[p] = o[p] + o[p]
    return o


def _rowcol(o, i, t):
    r = (o // 2) * 4 + (i // 2) * 2 + t // 2
    c = (o % 2) * 4 + (i % 2) * 2 + t % 2
    e = (o // 2 - o % 2) + (i // 2 - i % 2) + (t // 2 - t % 2)
    return r, c, e


def _plan(l3set, cfg):
    order = []
    for p in _PH:
        ks = [q for q in range(1, 8) if (p, q) not in l3set]
        ls = [q for q in cfg["qo"] if (p, q) in l3set]
        kp = cfg["kpos"][p]
        order += [(p, q) for q in ls[:kp] + ks + ls[kp:]]
    tile0 = {}
    n = 0
    for pq in order:
        tile0[pq] = n
        n += 7 if pq in l3set else 4
    return order, tile0, n


_NAMES = ([(f"u{p}", 7) for p in (3, 4, 7, 5, 1, 2, 6)]
          + [(f"a{p}", 4) for p in (3, 4, 5, 7, 2, 6, 1)]
          + [(f"{s}{k}", 4) for s in ("fx", "H", "G", "U", "V") for k in range(2)]
          + [(f"x0{o}", 4) for o in range(4)]
          + [("u2x", 7), ("u6x", 7)] + [(f"{s}{k}", 4) for s in "HGUV" for k in (2, 3)])


def _bufkeys(cfg):
    keys = []
    for n, k in _NAMES:
        sz = (k * _bs(cfg["tm"]) + 7) // 4 * 4
        if n[0] in cfg["merge"]:
            keys.append(((n, 0), 4 * sz))
        else:
            keys += [((n, t), sz) for t in range(4)]
    return keys


def _kernel(x_hbm, w_hbm, b_hbm, o_hbm, b_ref, ring, stage, wraw, wexp, beta, fx32, fxb, fb,
            xsem, wsem, tsem, bsem, fsem, *bufs, L, nsteps, cfg):
    l3set, win, TM, TPS, ROFF = cfg["l3set"], cfg["win"], cfg["tm"], cfg["tps"], cfg["roff"]
    BP, BQ = cfg["bp"], cfg["bq"]
    H = TM // 8
    NG = H // 8
    HT = TM // 2
    ST = TM * TPS
    BS = _bs(TM)
    order, tile0, _ = _plan(l3set, cfg)
    tmp = bufs[:2]
    keys = _bufkeys(cfg)
    buf = dict(zip([k for k, _ in keys], bufs[2:]))
    nblk = dict(_NAMES)
    for n, _ in _NAMES:
        if n[0] in cfg["merge"]:
            for t in range(1, 4):
                buf[n, t] = buf[n, 0]
    skew = {n: k % 4 for k, (n, _) in enumerate(_NAMES)}
    ctx = {}

    def x_copy(i):
        return pltpu.make_async_copy(
            x_hbm.at[pl.ds(pl.multiple_of(ROFF + i * ST, 64), ST)], ring.at[i & 3], xsem.at[i & 3])

    def w_copy(l, c):
        return pltpu.make_async_copy(
            w_hbm.at[l, :, pl.ds(c * 128, 128)], wraw.at[l, c], wsem.at[l])

    def w_start(l):
        for c in range(8):
            w_copy(l, c).start()

    def w_wait(l):
        for c in range(8):
            w_copy(l, c).wait()

    def top_copy(i):
        return pltpu.make_async_copy(
            stage.at[i & 1, pl.ds(HT, ST - HT)],
            o_hbm.at[pl.ds(pl.multiple_of(ROFF + i * ST, 64), ST - HT)], tsem.at[i & 1])

    def bot_copy(i):
        return pltpu.make_async_copy(
            stage.at[i & 1, pl.ds(0, HT)],
            o_hbm.at[pl.ds(pl.multiple_of(ROFF + i * ST - HT, 64), HT)], bsem.at[i & 1])

    def fin(c):
        return pltpu.make_async_copy(
            x_hbm.at[pl.ds(0, ROFF), pl.ds(c * 128, 128)], fxb.at[c], fsem.at[c])

    def fout(c):
        return pltpu.make_async_copy(
            fxb.at[(L & 1) * 8 + c], o_hbm.at[pl.ds(0, ROFF), pl.ds(c * 128, 128)], fsem.at[c])

    def off(n, b, t):
        q0 = t * ((nblk[n] * BS + 7) // 4 * 4) if n[0] in cfg["merge"] else 0
        return (q0 + (skew[n] + t) % 4 + b * BS) * 8

    def ld(n, b, t):
        o = off(n, b, t)
        return buf[n, t][ctx["z"], o:o + H, :]

    def st(n, b, t, v):
        o = off(n, b, t)
        buf[n, t][0, o:o + H, :] = v

    def anc(v, a):
        return v if a is None else jnp.where(ctx["mask"], a, v)

    def xin(j, o, i, t):
        r, c, _ = _rowcol(o, i, t)
        r0 = (j % TPS) * TM + r * H
        return ring[ctx["slot"][j // TPS], r0:r0 + H, c * 128:(c + 1) * 128].astype(f32)

    def sname(s, l):
        return f"{s}{l - L + 4 if l >= L - 2 else l % 2}"

    def uname(p, l):
        return f"u{p}x" if (l == L - 1 and p in (2, 6)) else f"u{p}"

    def emit(o, g, t):
        for i in range(4):
            r, c, e = _rowcol(o, i, t)
            y = xin(ctx["j"], o, i, t) * g[i]
            if e:
                y = y * (_D ** -e)
            r0 = ctx["j"] * TM + r * H + HT
            stage[ctx["oslot"], r0:r0 + H, c * 128:(c + 1) * 128] = y.astype(bf16)

    def fresh(o, t, a):
        xs = []
        for i in range(4):
            e = _rowcol(o, i, t)[2]
            v = xin(ctx["j"] + 1, o, i, t)
            if i == 0:
                v = anc(v, a)
            st(f"x0{o}", i, t, v)
            xs.append(v * (_D ** e) if e else v)
        return xs

    def gate(o, g, t):
        g = list(g)
        for i in cfg["a2i"]:
            g[i] = anc(g[i], ctx.get("a2"))
        return [ld(f"x0{o}", i, t) * g[i] for i in range(4)]

    def upd(l, p, s, t, a, keep=True):
        m = {q: ld(uname(p, l), q - 1, t) for q in range(1, 8)}
        m[3] = anc(m[3], a)
        y = _comb7(m)
        if l > 0:
            y = [y[i] + ld(sname(s, l - 1), i, t) for i in range(4)]
        if keep:
            for i in range(4):
                st(sname(s, l), i, t, y[i])
        return y

    def f1(l, t, x):
        for i, v in enumerate(_fwd(x)):
            st(f"fx{l % 2}", i, t, v)

    def f2(l, t, x):
        for i, v in enumerate(_fwd(x)):
            w = ld(f"fx{l % 2}", i, t)
            st("a3", i, t, v - w)
            st("a5", i, t, v + w)

    def f4(l, t, x):
        for i, v in enumerate(_fwd(x)):
            w = ld(f"fx{l % 2}", i, t)
            st("a4", i, t, w + v)
            st("a7", i, t, w - v)

    def f5(l, t, x):
        for i, v in enumerate(_fwd(x)):
            u = ld(f"fx{l % 2}", i, t) + v
            a1 = ld("a3", i, t) + ld("a4", i, t)
            st("a1", i, t, a1)
            st("a2", i, t, u + a1)
            st("a6", i, t, u - a1)

    def w4(l, t, a):
        v6 = upd(l, 6, "V", t, a)
        g = [v6[i] + (ld(sname("G", l), i, t) - ld(sname("U", l), i, t)) for i in range(4)]
        f4(l, t, gate(3, g, t))

    def w5(l, t, a):
        g = [anc(ld(sname("U", l), i, t), a if i == 0 else None)
             + ld(sname("V", l), i, t) + ld(sname("H", l), i, t) for i in range(4)]
        f5(l, t, gate(2, g, t))

    def o4(l, t, a):
        v6 = upd(l, 6, "V", t, a)
        emit(3, [v6[i] + (ld(sname("G", l), i, t) - ld(sname("U", l), i, t)) for i in range(4)], t)

    def o5(l, t, a):
        emit(2, [anc(ld(sname("U", l), i, t), a) + ld(sname("V", l), i, t) + ld(sname("H", l), i, t)
                 for i in range(4)], t)

    task = {
        "w1": lambda l, t, a: f1(l, t, gate(1, upd(l, 5, "H", t, a), t)),
        "w2": lambda l, t, a: f2(l, t, gate(0, upd(l, 1, "G", t, a), t)),
        "w3": lambda l, t, a: upd(l, 2, "U", t, a),
        "w4": w4,
        "w5": w5,
        "o1": lambda l, t, a: emit(1, upd(l, 5, "H", t, a), t),
        "o2": lambda l, t, a: emit(0, upd(l, 1, "G", t, a), t),
        "o3": lambda l, t, a: upd(l, 2, "U", t, a),
        "o4": o4,
        "o5": o5,
        "e1": lambda l, t, a: f1(l, t, fresh(1, t, a)),
        "e2": lambda l, t, a: f2(l, t, fresh(0, t, a)),
        "e4": lambda l, t, a: f4(l, t, fresh(3, t, a)),
        "e5": lambda l, t, a: f5(l, t, fresh(2, t, a)),
    }

    b_copy = pltpu.make_async_copy(b_hbm, b_ref, fsem.at[8])
    b_copy.start()
    for c in range(8):
        fin(c).start()
    w_start(0)
    b_copy.wait()
    kap, kaq = _kappa(BP), _kappa(BQ)
    for l in range(L):
        bl = b_ref[l:l + 1, :].astype(f32)
        for c in range(8):
            fb[l * 8 + c, 0:1, :] = bl[:, c * 128:(c + 1) * 128]
        if l == 0:
            bl = bl + 1.0
        for pi, p in enumerate(BP):
            for qi, q in enumerate(BQ):
                for c3 in range(2):
                    acc = None
                    for c1 in range(2):
                        for c2 in range(2):
                            k = float(kap[c1][p] * kaq[c2][q])
                            if abs(k) < 1e-12:
                                continue
                            c = c1 * 4 + c2 * 2 + c3
                            term = bl[:, c * 128:(c + 1) * 128] * k
                            acc = term if acc is None else acc + term
                    for r3 in range(2):
                        row = l * 64 + (pi * 4 + qi) * 4 + r3 * 2 + c3
                        beta[row:row + 1, :] = acc * (_D ** (r3 - c3))
    for c in range(8):
        fin(c).wait()
    for c in range(8):
        v = fxb[c].astype(f32)
        fx32[c] = v
        fx32[8 + c] = v

    def toff(p, i, t):
        return ((p - 1) * 37 + (i * 4 + t) * 2 + i) * 8

    def s1_units(l, g, dst):
        r0 = pl.multiple_of(g * 16, 16)

        def unit(i, t):
            blk = []
            for o in range(4):
                r, c, e = _rowcol(o, i, t)
                v = wraw[l, c, pl.ds(r * 128 + r0, 16), :].astype(f32)
                blk.append(v * (0.125 * _D ** e))
            ex = _bexp(blk, ())
            for p in _PH:
                dst[0, toff(p, i, t):toff(p, i, t) + 16, :] = ex[p]
            return [ex[7][:8], ex[7][8:]]

        return [(34, functools.partial(unit, i, t)) for i in range(4) for t in range(4)]

    def s2_units(l, g, src, zg):
        r0 = pl.multiple_of(g * 16, 16)

        def put(p, q, qs):
            if (p, q) in l3set:
                f = (2.0 if p == 1 else 1.0) * (2 if q in (1, 2, 6) else 1)
                if f != 1:
                    qs = [v * f for v in qs]
                inn = _bexp(qs, (1,))
                tiles = [inn[r] for r in range(1, 8)]
            else:
                f = 2.0 * (2 if p == 1 else 1) * (2 if q in (1, 2, 6) else 1)
                tiles = [v * f for v in qs]
            for k, v in enumerate(tiles):
                wexp[l, tile0[p, q] + k, pl.ds(r0, 16), :] = v.astype(bf16)
            return tiles

        def unit(p, un, a=None):
            def tl(i):
                vs = [src[zg[1 + un], toff(p, i, t):toff(p, i, t) + 16, :] for t in range(4)]
                if a is not None and i == 1:
                    nv = jnp.full((16, 128), zg[0], jnp.int32) != 0
                    for t in cfg["pt"]:
                        vs[t] = jnp.where(nv, a, vs[t])
                return vs

            if un == 0:
                x, y, qa, qb = tl(0), tl(1), 2, 6
            elif un == 1:
                x, y, qa, qb = tl(1), tl(3), 3, 5
            else:
                x = [u + v for u, v in zip(tl(1), tl(2))]
                y = [u + v for u, v in zip(tl(0), tl(3))]
                qa, qb = 4, 7
                put(p, 1, y)
            ta = put(p, qa, [u - v for u, v in zip(x, y)])
            tb = put(p, qb, [u + v for u, v in zip(x, y)])
            if len(tb) == 4:
                return [v[:8] for v in tb]
            return [ta[-1][:8], tb[-1][8:]]

        cost = lambda p, un: (40, 40, 68)[un] if p == 1 else (82, 66, 94)[un]
        return [(cost(p, un), functools.partial(unit, p, un)) for p in _PH for un in range(3)]

    def half(l, g, ln, gn, src, dst, zg, tail):
        u2 = s2_units(l, g, src, zg)
        u1 = s1_units(ln, gn, dst)
        units = sorted([(k / len(u2), c, f) for k, (c, f) in enumerate(u2)]
                       + [((k + 0.5) / len(u1) * cfg["s1f"], c, f) for k, (c, f) in enumerate(u1)],
                       key=lambda e: e[0])
        late = [f for _, _, f in units[len(units) - len(tail):]]
        units = units[:len(units) - len(tail)]
        total = sum(c for _, c, _ in units)
        nsl = ROFF // 16
        links = {}
        acc = 0
        for _, c, f in units:
            acc += c
            vals = f()
            sl = min(int(np.ceil(acc / total * 2 * nsl)), 2 * nsl) - 1
            links.setdefault(sl, []).extend(vals)
        fsrc = (l & 1) * 8
        fu = fxb.bitcast(jnp.uint32)
        never = jnp.full((8, 128), zg[0], jnp.int32) != 0
        cols = []
        for c in range(8):
            rows = []
            for r in range(nsl):
                v = fu[fsrc + c, r * 8:(r + 1) * 8, :]
                for a in links.get((c // 4) * nsl + r, [])[c % 4::4]:
                    v = jnp.where(never, pltpu.bitcast(a, jnp.uint32), v)
                rows.append(v)
            cols.append(pltpu.bitcast(jnp.concatenate(rows, 0), bf16))
        wg = pltpu.bitcast(wraw.bitcast(jnp.uint32)[l, g], bf16)
        y = jnp.dot(jnp.concatenate(cols, 1), wg, preferred_element_type=f32)
        xn = fx32[g] * (y + fb[l * 8 + g, 0:1, :]) + fx32[8 + g]
        fx32[8 + g] = xn
        fxb[8 - fsrc + g] = xn.astype(bf16)
        for r, f in zip(tail, late):
            f(y[r * 8:r * 8 + 16])

    w_wait(0)
    w_start(1)
    for _, f in s1_units(0, 0, tmp[0]):
        f()

    def pair(n, carry):
        l = lax.shift_right_logical(n, 2)
        g = (n & 3) * 2

        @pl.when(jnp.logical_and(g == 6, l + 1 < L))
        def _():
            w_wait(l + 1)

        @pl.when(jnp.logical_and(g == 6, l + 2 < L))
        def _():
            w_start(l + 2)

        @pl.when(n == 4 * L - 5)
        def _():
            x_copy(0).start()
            x_copy(1).start()

        zg = [lax.shift_right_logical(n, 12 + k) for k in range(8)]
        nn = jnp.minimum(2 * n + 2, 8 * L - 1)
        half(l, g, l, g + 1, tmp[0], tmp[1], zg[:4], ())
        half(l, g + 1, lax.shift_right_logical(nn, 3), nn & 7, tmp[1], tmp[0], zg[4:], cfg["tail"])
        return carry

    lax.fori_loop(0, 4 * L, pair, 0)
    for c in range(8):
        fout(c).start()
    x_copy(0).wait()
    ctx.update(z=0, slot={0: 0}, j=-1)
    for w in ("e1", "e2"):
        for t in range(4):
            task[w](L - 1, t, None)

    def main(step, carry):
        @pl.when(step + 1 < nsteps)
        def _():
            x_copy(step + 1).wait()

        @pl.when(step + 2 < nsteps)
        def _():
            x_copy(step + 2).start()

        zz = [lax.shift_right_logical(step, 12 + k) for k in range(_NZ)]
        ctx.update(mask=jnp.full((H, 128), zz[0], jnp.int32) != 0,
                   slot={-1: (step + 3) & 3, 0: step & 3, 1: (step + 1) & 3}, oslot=step & 1)
        wu = wexp.bitcast(jnp.uint32)

        def wtile(l, k):
            return pltpu.bitcast(wu[l, k], bf16)

        prods = [(l, p, q) for _j in range(TPS) for l in range(L) for (p, q) in order]
        npr = len(prods)
        free = [0, 0, 0, 0]
        anchors = []
        pstart = []
        for pi, (l, p, q) in enumerate(prods):
            pstart.append(min(free))
            if (p, q) in l3set:
                for j in range(7):
                    mx = int(np.argmin(free))
                    anchors += [(free[mx] + g * 8, pi, j, g) for g in range(NG)]
                    free[mx] += H
            else:
                anchors += [(max(free) + g * 8, pi, 0, g) for g in range(2 * NG)]
                free = [f + 2 * H for f in free]
        pstart.append(max(free))
        anchors.sort()
        times = np.array([a[0] for a in anchors])

        def tpos(x):
            i = int(np.floor(x))
            return pstart[i] + (x - i) * (pstart[min(i + 1, npr)] - pstart[i])

        wv, ws, wl = cfg["wts"]
        P = 4 * NG
        nb = pstart[-1] // 8 + 1
        load = np.zeros(nb)

        def spread(t0, t1, valu, st_, ld_):
            b0, b1 = max(int(t0 // 8), 0), max(int(t1 // 8), 1)
            load[b0:b1] += (valu / 4 * wv + st_ * ws + ld_ / 3 * wl) / max(int(t1 // 8) - int(t0 // 8), 1)

        for pi, (l, p, q) in enumerate(prods):
            t = len(_MIDB[q])
            big = (p, q) in l3set
            t0, t1 = pstart[pi], pstart[pi + 1]
            spread(t0 - cfg["lat"], t1 - cfg["lat"], (t - 1 + (2.875 if big else 0.5)) * P, 0,
                   t * P + (56 if big else 32))
            sa, sl = {5: (1, 1), 1: (5, 4), 2: (1, 1), 6: (1, 1)}.get(p, (0, 0))
            bias = 1 if (p in BP and q in BQ) else 0
            spread(t0, t1 + (H // 2 if big else 0), ((2.75 if big else 1) + bias + sa) * P, P, sl * P)

        amp, seeds = cfg["jit"]
        for k, sd in enumerate(seeds):
            b0, b1 = pstart[k * 49] // 8, pstart[k * 49 + 49] // 8
            load[b0:b1] += amp * np.random.RandomState(sd).randn(b1 - b0)

        tcost = {"w1": (26, 8, 15), "w2": (34, 12, 19), "w3": (16, 4, 11), "w4": (42, 12, 27),
                 "w5": (35, 12, 28), "o1": (31, 8, 15), "o2": (31, 8, 15), "o3": (16, 4, 11),
                 "o4": (39, 8, 23), "o5": (27, 4, 16), "e1": (14, 8, 4), "e2": (22, 12, 8),
                 "e4": (22, 12, 8), "e5": (30, 16, 16)}
        kern = np.hanning(cfg["sm"] + 2)[1:-1]
        kern /= kern.sum()
        sched = {}
        jobs = [(w, l) for l in range(L - 1) for w in ("w1", "w2", "w3", "w4", "w5")]
        jobs += [(w, L - 1) for w in ("e1", "o1", "e2", "o2", "e4", "e5", "o3", "o4", "o5")]
        todo = [(jn, w, l, j) for j in range(TPS) for jn, (w, l) in enumerate(jobs)]
        wof = lambda w, l: win.get((w, l), win[w])
        todo.sort(key=lambda e: wof(e[1], e[2])[1] - wof(e[1], e[2])[0])
        for jn, w, l, j in todo:
            b0, b1 = wof(w, l)
            i0, i1, jj = (j * L + l) * 49 + b0, (j * L + l) * 49 + b1, j
            if i0 >= npr:
                i0, i1, jj = i0 - npr, i1 - npr, j - TPS
            assert i1 <= npr
            lo, hi = int(np.ceil(tpos(i0) / 8)), int(tpos(i1) // 8)
            picks = []
            for _k in range(P):
                sm = np.convolve(load, kern, mode="same")
                bb = lo + int(np.argmin(sm[lo + 1:hi + 1]))
                picks.append(bb)
                spread(bb * 8, bb * 8 + 24 + (cfg["a2d"] - 8 if w in cfg["a2w"] else 0), *tcost[w])
            slots = []
            for bb in sorted(picks):
                ai = int(np.searchsorted(times, bb * 8))
                while anchors[ai][1] < int(i0):
                    ai += 1
                slots.append(anchors[ai][1:])
            if w in cfg["a2w"]:
                for bb in sorted(picks):
                    slots.append(anchors[int(np.searchsorted(times, bb * 8 + cfg["a2d"]))][1:])
            for t in range(4):
                al = slots[t * NG:(t + 1) * NG] + slots[P + t * NG:P + (t + 1) * NG]
                sched.setdefault(max(a[0] for a in al), []).append((w, l, t, al, jn, jj))
        for v in sched.values():
            v.sort(key=lambda e: (e[5], e[4], e[2]))

        subs = {}
        l3pos = 0
        for pi, (l, p, q) in enumerate(prods):
            ctx["z"] = zz[{1: 0, 2: 0, 3: 0, 5: 0, 4: 1, 6: 2, 7: 3}[q]]
            srcs = [f"a{p}"]
            qv = [_lin([(ld(n, b, t), s) for n in srcs for b, s in _MIDB[q]]) for t in range(4)]
            k0 = tile0[p, q]
            if (p, q) in l3set:
                a1 = qv[0] + qv[3]
                u = qv[1] + qv[2]
                av = {1: a1, 3: qv[0] - qv[1], 5: qv[0] + qv[1], 4: qv[1] + qv[3],
                      7: qv[1] - qv[3], 2: u + a1, 6: u - a1}
                so = cfg["so"][l3pos % 4]
                l3pos += 1
                m = {r: jnp.dot(av[r].astype(bf16), wtile(l, k0 + r - 1), preferred_element_type=f32)
                     for r in so}
                subs[pi] = [m[r] for r in so]
                mq = _comb7(m)
            else:
                a = jnp.concatenate(
                    [jnp.concatenate(qv[:2], 1), jnp.concatenate(qv[2:], 1)], 0).astype(bf16)
                wt = [wtile(l, k0 + t) for t in range(4)]
                wm = jnp.concatenate([jnp.concatenate(wt[:2], 1), jnp.concatenate(wt[2:], 1)], 0)
                mm = jnp.dot(a, wm, preferred_element_type=f32)
                subs[pi] = [mm[:, :128]]
                mq = [mm[:H, :128], mm[:H, 128:], mm[H:, :128], mm[H:, 128:]]
            if p in BP and q in BQ:
                row = l * 64 + (BP.index(p) * 4 + BQ.index(q)) * 4
                mq = [mq[t] + beta[row + t:row + t + 1, :] for t in range(4)]
            for t in range(4):
                v = mq[t]
                if p == 5:
                    v = v + ld("u3", q - 1, t)
                elif p == 1:
                    r3 = ld("u3", q - 1, t)
                    v = v + (((ld("u4", q - 1, t) + ld("u7", q - 1, t)) + (r3 + r3)) - ld("u5", q - 1, t))
                elif p == 2:
                    v = v + ld("u4", q - 1, t)
                elif p == 6:
                    v = v - ld("u7", q - 1, t)
                st(uname(p, l), q - 1, t, v)
            for (w, tl, t, al, jn, jj) in sched.get(pi, []):
                a = jnp.concatenate([subs[api][j][g * 8:(g + 1) * 8, :] for api, j, g in al], 0)
                ctx.update(z=zz[8 + jn % 6], j=jj, a2=a[H:] if len(al) > NG else None)
                task[w](tl, t, a[:H])

        @pl.when(step >= 1)
        def _():
            top_copy(step - 1).wait()

        @pl.when(step >= 2)
        def _():
            bot_copy(step - 1).wait()

        top_copy(step).start()

        @pl.when(step >= 1)
        def _():
            bot_copy(step).start()

        return carry

    lax.fori_loop(0, nsteps, main, 0)

    ctx.update(z=0, slot={-1: (nsteps - 1) % 4}, j=-1, oslot=nsteps % 2)
    for w in ("o3", "o4", "o5"):
        for t in range(4):
            task[w](L - 1, t, None)
    bot_copy(nsteps).start()
    for c in range(8):
        fout(c).wait()
    top_copy(nsteps - 1).wait()
    bot_copy(nsteps - 1).wait()
    bot_copy(nsteps).wait()


_L3SET = tuple((p, q) for p in range(2, 8) for q in range(2, 8))
_WIN = {"w1": (14, 35), "w2": (35, 46), "w3": (42, 49), "w4": (49, 60), "w5": (60, 74),
        "e1": (0, 35), "o1": (14, 35), "e2": (35, 46), "o2": (35, 48.5), "e4": (49, 60), "e5": (60, 74),
        "o3": (49, 60), "o4": (60, 170), "o5": (170, 290)}
_SO = ((3, 5, 1, 4, 7, 2, 6), (1, 3, 5, 4, 7, 2, 6), (3, 5, 1, 4, 7, 2, 6), (3, 5, 1, 4, 7, 2, 6))
_CFG = dict(l3set=_L3SET + ((4, 1), (7, 1), (1, 3), (1, 5)), win=_WIN, tm=384, tps=1, roff=256, kpos={3: 4, 5: 2, 4: 0, 7: 0, 1: 2, 2: 4, 6: 2}, wts=(1, 0.2, 0), lat=135, sm=6, merge="a", bp=(3, 4, 7, 1), bq=(5, 2, 1, 6), jit=(0.0, (0,) * 6), a2w=("w4", "w2"), a2d=24, a2i=(0,), s1f=0.75, tail=(14, 17, 20, 23, 26), pt=(1,), so=_SO, qo=(3, 5, 2, 4, 7, 6, 1))


def _build(**kw):
    cfg = dict(_CFG, **kw)

    def fn(x0, ws, bs):
        B, Dm = x0.shape
        L = ws.shape[0]
        st = cfg["tm"] * cfg["tps"]
        nsteps = (B - cfg["roff"]) // st
        ntiles = _plan(cfg["l3set"], cfg)[2]
        return pl.pallas_call(
            functools.partial(_kernel, L=L, nsteps=nsteps, cfg=cfg),
            in_specs=[
                pl.BlockSpec(memory_space=pl.ANY),
                pl.BlockSpec(memory_space=pl.ANY),
                pl.BlockSpec(memory_space=pl.ANY),
            ],
            out_specs=pl.BlockSpec(memory_space=pl.ANY),
            out_shape=jax.ShapeDtypeStruct((B, Dm), x0.dtype),
            scratch_shapes=[
                pltpu.VMEM((L, Dm), bf16),
                pltpu.VMEM((4, st, Dm), bf16),
                pltpu.VMEM((2, st, Dm), bf16),
                pltpu.VMEM((L, 8, Dm, 128), bf16),
                pltpu.VMEM((L, ntiles, 128, 128), bf16),
                pltpu.VMEM((L * 64, 128), f32),
                pltpu.VMEM((16, cfg["roff"], 128), f32),
                pltpu.VMEM((16, cfg["roff"], 128), bf16),
                pltpu.VMEM((L * 8, 8, 128), f32),
                pltpu.SemaphoreType.DMA((4,)),
                pltpu.SemaphoreType.DMA((L,)),
                pltpu.SemaphoreType.DMA((2,)),
                pltpu.SemaphoreType.DMA((2,)),
                pltpu.SemaphoreType.DMA((9,)),
            ]
            + [pltpu.VMEM((1, 260 * 8, 128), f32)] * 2
            + [pltpu.VMEM((1, sz * 8, 128), f32) for _, sz in _bufkeys(cfg)],
            compiler_params=pltpu.CompilerParams(
                vmem_limit_bytes=126 * 1024 * 1024,
                disable_bounds_checks=True,
            ),
        )(x0, ws, bs)

    return fn


@jax.jit
def pallas_standalone__dcn_v2_cross__recsys_kernel(
    x0: jax.Array,
    ws: jax.Array,
    bs: jax.Array,
):
    return _build()(x0, ws, bs)
```

```python
import functools

import numpy as np
import jax
import jax.numpy as jnp
from jax import lax
import jax.experimental.pallas as pl
import jax.experimental.pallas.tpu as pltpu

f32 = jnp.float32
bf16 = jnp.bfloat16

_D = float(np.sqrt(3.0))
_PH = (3, 5, 4, 7, 1, 2, 6)
_MIDB = {1: [(0, 1)], 2: [(1, 1)], 3: [(2, 1)], 5: [(3, 1)],
         4: [(0, 1), (2, -1)], 6: [(1, 1), (0, -1)], 7: [(3, 1), (0, -1)]}
_CVEC = {1: [1, 0, 0, 1], 2: [0, 0, 1, -1], 3: [1, 1, 1, 1], 4: [1, 0, 1, 0],
         5: [-1, 1, 1, -1], 6: [0, 0, 1, 1], 7: [1, 0, -1, 0]}
_NZ = 14


def _bs(tm):
    ng = tm // 64
    return ng // 4 * 4 + (1 if ng % 4 == 0 else 5)


def _kappa(bset):
    m = np.array([_CVEC[p] for p in bset], np.float64).T
    pats = [np.array([1, 0, _D, 0]), np.array([0, 1 / _D, 0, 1])]
    return [dict(zip(bset, np.linalg.solve(m, t))) for t in pats]


def _lin(terms):
    terms = sorted(terms, key=lambda t: -t[1])
    acc = terms[0][0]
    for v, s in terms[1:]:
        acc = acc + v if s > 0 else acc - v
    return acc


def _comb7(m):
    s = m[3] + m[5]
    e = (m[3] - m[5]) + m[1]
    return [(e + m[4]) + m[7], s, (((s + m[4]) - m[7]) + m[2]) + m[6], (e - m[2]) + m[6]]


def _comb7o(m, so, link=None):
    pos = {r: so.index(r) for r in so}

    def acc(terms):
        terms = sorted(terms, key=lambda e: e[2])
        if terms[0][1] < 0:
            terms[0], terms[1] = terms[1], terms[0]
        v = terms[0][0]
        for x, sg, _ in terms[1:]:
            v = v + x if sg > 0 else v - x
        return v

    s = m[3] + m[5]
    ps = max(pos[3], pos[5])
    e = acc([(m[3], 1, pos[3]), (m[5], -1, pos[5]), (m[1], 1, pos[1])])
    pe = max(ps, pos[1])
    t = lambda r, sg: (m[r], sg, pos[r])
    c1 = s if link is None else link(s, e)
    return [acc([(e, 1, pe), t(4, 1), t(7, 1)]), c1,
            acc([(s, 1, ps), t(4, 1), t(7, -1), t(2, 1), t(6, 1)]),
            acc([(e, 1, pe), t(2, -1), t(6, 1)])]


def _fwd(x):
    a1 = x[0] + x[3]
    return [a1, ((x[1] + x[2]) + a1) * 0.5, x[0] - x[1], x[0] + x[1]]


def _bexp(b, dbl):
    b1 = b[0] + b[3]
    u = b[1] + b[2]
    o = {1: b1, 2: b[0] - b[1], 3: b[1] - b[3], 4: u - b1, 5: b[1] + b[3], 6: b[0] + b[1], 7: u + b1}
    for p in dbl:
        o[p] = o[p] + o[p]
    return o


def _rowcol(o, i, t):
    r = (o // 2) * 4 + (i // 2) * 2 + t // 2
    c = (o % 2) * 4 + (i % 2) * 2 + t % 2
    e = (o // 2 - o % 2) + (i // 2 - i % 2) + (t // 2 - t % 2)
    return r, c, e


def _plan(l3set, cfg):
    order = []
    for p in _PH:
        ks = [q for q in range(1, 8) if (p, q) not in l3set]
        ls = [q for q in cfg["qo"] if (p, q) in l3set]
        kp = cfg["kpos"][p]
        order += [(p, q) for q in ls[:kp] + ks + ls[kp:]]
    tile0 = {}
    n = 0
    for pq in order:
        tile0[pq] = n
        n += 7 if pq in l3set else 4
    return order, tile0, n


_NAMES = ([(f"u{p}", 7) for p in (3, 4, 7, 5, 1, 2, 6)]
          + [(f"a{p}", 4) for p in (3, 4, 5, 7, 2, 6, 1)]
          + [(f"{s}{k}", 4) for s in ("fx", "H", "G", "U", "V") for k in range(2)]
          + [(f"x0{o}", 4) for o in range(4)]
          + [("u2x", 7), ("u6x", 7)] + [(f"{s}{k}", 4) for s in "HGUV" for k in (2, 3)])


def _bufkeys(cfg):
    keys = []
    for n, k in _NAMES:
        sz = (k * _bs(cfg["tm"]) + 7) // 4 * 4
        if n[0] in cfg["merge"]:
            keys.append(((n, 0), 4 * sz))
        else:
            keys += [((n, t), sz) for t in range(4)]
    return keys


def _kernel(x_hbm, w_hbm, b_hbm, o_hbm, b_ref, ring, stage, wraw, wexp, beta, fx32, fxb, fb,
            xsem, wsem, tsem, bsem, fsem, *bufs, L, nsteps, cfg):
    l3set, win, TM, TPS, ROFF = cfg["l3set"], cfg["win"], cfg["tm"], cfg["tps"], cfg["roff"]
    BP, BQ = cfg["bp"], cfg["bq"]
    H = TM // 8
    NG = H // 8
    HT = TM // 2
    ST = TM * TPS
    BS = _bs(TM)
    order, tile0, _ = _plan(l3set, cfg)
    tmp = bufs[:2]
    keys = _bufkeys(cfg)
    buf = dict(zip([k for k, _ in keys], bufs[2:]))
    nblk = dict(_NAMES)
    for n, _ in _NAMES:
        if n[0] in cfg["merge"]:
            for t in range(1, 4):
                buf[n, t] = buf[n, 0]
    skew = {n: k % 4 for k, (n, _) in enumerate(_NAMES)}
    ctx = {}

    def x_copy(i):
        return pltpu.make_async_copy(
            x_hbm.at[pl.ds(pl.multiple_of(ROFF + i * ST, 64), ST)], ring.at[i & 3], xsem.at[i & 3])

    def w_copy(l, c):
        return pltpu.make_async_copy(
            w_hbm.at[l, :, pl.ds(c * 128, 128)], wraw.at[l, c], wsem.at[l])

    def w_start(l):
        for c in range(8):
            w_copy(l, c).start()

    def w_wait(l):
        for c in range(8):
            w_copy(l, c).wait()

    def top_copy(i):
        return pltpu.make_async_copy(
            stage.at[i & 1, pl.ds(HT, ST - HT)],
            o_hbm.at[pl.ds(pl.multiple_of(ROFF + i * ST, 64), ST - HT)], tsem.at[i & 1])

    def bot_copy(i):
        return pltpu.make_async_copy(
            stage.at[i & 1, pl.ds(0, HT)],
            o_hbm.at[pl.ds(pl.multiple_of(ROFF + i * ST - HT, 64), HT)], bsem.at[i & 1])

    def fin(c):
        return pltpu.make_async_copy(
            x_hbm.at[pl.ds(0, ROFF), pl.ds(c * 128, 128)], fxb.at[c], fsem.at[c])

    def fout(c):
        return pltpu.make_async_copy(
            fxb.at[(L & 1) * 8 + c], o_hbm.at[pl.ds(0, ROFF), pl.ds(c * 128, 128)], fsem.at[c])

    def off(n, b, t):
        q0 = t * ((nblk[n] * BS + 7) // 4 * 4) if n[0] in cfg["merge"] else 0
        return (q0 + (skew[n] + t) % 4 + b * BS) * 8

    def ld(n, b, t):
        o = off(n, b, t)
        return buf[n, t][ctx["z"], o:o + H, :]

    def st(n, b, t, v):
        o = off(n, b, t)
        buf[n, t][0, o:o + H, :] = v

    def anc(v, a):
        return v if a is None else jnp.where(ctx["mask"], a, v)

    def xin(j, o, i, t):
        r, c, _ = _rowcol(o, i, t)
        r0 = (j % TPS) * TM + r * H
        return ring[ctx["slot"][j // TPS], r0:r0 + H, c * 128:(c + 1) * 128].astype(f32)

    def sname(s, l):
        return f"{s}{l - L + 4 if l >= L - 2 else l % 2}"

    def uname(p, l):
        return f"u{p}x" if (l == L - 1 and p in (2, 6)) else f"u{p}"

    def emit(o, g, t):
        for i in range(4):
            r, c, e = _rowcol(o, i, t)
            y = xin(ctx["j"], o, i, t) * g[i]
            if e:
                y = y * (_D ** -e)
            r0 = ctx["j"] * TM + r * H + HT
            stage[ctx["oslot"], r0:r0 + H, c * 128:(c + 1) * 128] = y.astype(bf16)

    def fresh(o, t, a):
        xs = []
        for i in range(4):
            e = _rowcol(o, i, t)[2]
            v = xin(ctx["j"] + 1, o, i, t)
            if i == 0:
                v = anc(v, a)
            st(f"x0{o}", i, t, v)
            xs.append(v * (_D ** e) if e else v)
        return xs

    def gate(o, g, t):
        g = list(g)
        for i in cfg["a2i"]:
            g[i] = anc(g[i], ctx.get("a2"))
        return [ld(f"x0{o}", i, t) * g[i] for i in range(4)]

    def upd(l, p, s, t, a, keep=True):
        m = {q: ld(uname(p, l), q - 1, t) for q in range(1, 8)}
        m[3] = anc(m[3], a)
        y = _comb7(m)
        if l > 0:
            y = [y[i] + ld(sname(s, l - 1), i, t) for i in range(4)]
        if keep:
            for i in range(4):
                st(sname(s, l), i, t, y[i])
        return y

    def f1(l, t, x):
        for i, v in enumerate(_fwd(x)):
            st(f"fx{l % 2}", i, t, v)

    def f2(l, t, x):
        for i, v in enumerate(_fwd(x)):
            w = ld(f"fx{l % 2}", i, t)
            st("a3", i, t, v - w)
            st("a5", i, t, v + w)

    def f4(l, t, x):
        for i, v in enumerate(_fwd(x)):
            w = ld(f"fx{l % 2}", i, t)
            st("a4", i, t, w + v)
            st("a7", i, t, w - v)

    def f5(l, t, x):
        for i, v in enumerate(_fwd(x)):
            u = ld(f"fx{l % 2}", i, t) + v
            a1 = ld("a3", i, t) + ld("a4", i, t)
            st("a1", i, t, a1)
            st("a2", i, t, u + a1)
            st("a6", i, t, u - a1)

    def w4(l, t, a):
        v6 = upd(l, 6, "V", t, a)
        g = [v6[i] + (ld(sname("G", l), i, t) - ld(sname("U", l), i, t)) for i in range(4)]
        f4(l, t, gate(3, g, t))

    def w5(l, t, a):
        g = [anc(ld(sname("U", l), i, t), a if i == 0 else None)
             + ld(sname("V", l), i, t) + ld(sname("H", l), i, t) for i in range(4)]
        f5(l, t, gate(2, g, t))

    def o4(l, t, a):
        v6 = upd(l, 6, "V", t, a)
        emit(3, [v6[i] + (ld(sname("G", l), i, t) - ld(sname("U", l), i, t)) for i in range(4)], t)

    def o5(l, t, a):
        emit(2, [anc(ld(sname("U", l), i, t), a) + ld(sname("V", l), i, t) + ld(sname("H", l), i, t)
                 for i in range(4)], t)

    task = {
        "w1": lambda l, t, a: f1(l, t, gate(1, upd(l, 5, "H", t, a), t)),
        "w2": lambda l, t, a: f2(l, t, gate(0, upd(l, 1, "G", t, a), t)),
        "w3": lambda l, t, a: upd(l, 2, "U", t, a),
        "w4": w4,
        "w5": w5,
        "o1": lambda l, t, a: emit(1, upd(l, 5, "H", t, a), t),
        "o2": lambda l, t, a: emit(0, upd(l, 1, "G", t, a), t),
        "o3": lambda l, t, a: upd(l, 2, "U", t, a),
        "o4": o4,
        "o5": o5,
        "e1": lambda l, t, a: f1(l, t, fresh(1, t, a)),
        "e2": lambda l, t, a: f2(l, t, fresh(0, t, a)),
        "e4": lambda l, t, a: f4(l, t, fresh(3, t, a)),
        "e5": lambda l, t, a: f5(l, t, fresh(2, t, a)),
    }

    b_copy = pltpu.make_async_copy(b_hbm, b_ref, fsem.at[8])
    b_copy.start()
    for c in range(8):
        fin(c).start()
    w_start(0)
    b_copy.wait()
    kap, kaq = _kappa(BP), _kappa(BQ)
    for l in range(L):
        bl = b_ref[l:l + 1, :].astype(f32)
        for c in range(8):
            fb[l * 8 + c, 0:1, :] = bl[:, c * 128:(c + 1) * 128]
        if l == 0:
            bl = bl + 1.0
        for pi, p in enumerate(BP):
            for qi, q in enumerate(BQ):
                for c3 in range(2):
                    acc = None
                    for c1 in range(2):
                        for c2 in range(2):
                            k = float(kap[c1][p] * kaq[c2][q])
                            if abs(k) < 1e-12:
                                continue
                            c = c1 * 4 + c2 * 2 + c3
                            term = bl[:, c * 128:(c + 1) * 128] * k
                            acc = term if acc is None else acc + term
                    for r3 in range(2):
                        row = l * 64 + (pi * 4 + qi) * 4 + r3 * 2 + c3
                        beta[row:row + 1, :] = acc * (_D ** (r3 - c3))
    for c in range(8):
        fin(c).wait()
    for c in range(8):
        v = fxb[c].astype(f32)
        fx32[c] = v
        fx32[8 + c] = v

    def toff(p, i, t):
        return ((p - 1) * 37 + (i * 4 + t) * 2 + i) * 8

    def s1_units(l, g, dst):
        r0 = pl.multiple_of(g * 16, 16)

        def unit(i, t):
            blk = []
            for o in range(4):
                r, c, e = _rowcol(o, i, t)
                v = wraw[l, c, pl.ds(r * 128 + r0, 16), :].astype(f32)
                blk.append(v * (0.125 * _D ** e))
            ex = _bexp(blk, ())
            for p in _PH:
                dst[0, toff(p, i, t):toff(p, i, t) + 16, :] = ex[p]
            return [ex[7][:8], ex[7][8:]]

        return [(34, functools.partial(unit, i, t)) for i in range(4) for t in range(4)]

    def s2_units(l, g, src, zg):
        r0 = pl.multiple_of(g * 16, 16)

        def put(p, q, qs):
            if (p, q) in l3set:
                f = (2.0 if p == 1 else 1.0) * (2 if q in (1, 2, 6) else 1)
                if f != 1:
                    qs = [v * f for v in qs]
                inn = _bexp(qs, (1,))
                tiles = [inn[r] for r in range(1, 8)]
            else:
                f = 2.0 * (2 if p == 1 else 1) * (2 if q in (1, 2, 6) else 1)
                tiles = [v * f for v in qs]
            for k, v in enumerate(tiles):
                wexp[l, tile0[p, q] + k, pl.ds(r0, 16), :] = v.astype(bf16)
            return tiles

        def unit(p, un, a=None):
            def tl(i):
                vs = [src[zg[1 + un], toff(p, i, t):toff(p, i, t) + 16, :] for t in range(4)]
                if a is not None and i == 1:
                    nv = jnp.full((16, 128), zg[0], jnp.int32) != 0
                    for t in cfg["pt"]:
                        vs[t] = jnp.where(nv, a, vs[t])
                return vs

            if un == 0:
                x, y, qa, qb = tl(0), tl(1), 2, 6
            elif un == 1:
                x, y, qa, qb = tl(1), tl(3), 3, 5
            else:
                x = [u + v for u, v in zip(tl(1), tl(2))]
                y = [u + v for u, v in zip(tl(0), tl(3))]
                qa, qb = 4, 7
                put(p, 1, y)
            ta = put(p, qa, [u - v for u, v in zip(x, y)])
            tb = put(p, qb, [u + v for u, v in zip(x, y)])
            if len(tb) == 4:
                return [v[:8] for v in tb]
            return [ta[-1][:8], tb[-1][8:]]

        cost = lambda p, un: (40, 40, 68)[un] if p == 1 else (82, 66, 94)[un]
        return [(cost(p, un), functools.partial(unit, p, un)) for p in _PH for un in range(3)]

    def half(l, g, ln, gn, src, dst, zg, tail):
        u2 = s2_units(l, g, src, zg)
        u1 = s1_units(ln, gn, dst)
        units = sorted([(k / len(u2), c, f) for k, (c, f) in enumerate(u2)]
                       + [((k + 0.5) / len(u1) * cfg["s1f"], c, f) for k, (c, f) in enumerate(u1)],
                       key=lambda e: e[0])
        late = [f for _, _, f in units[len(units) - len(tail):]]
        units = units[:len(units) - len(tail)]
        total = sum(c for _, c, _ in units)
        nsl = ROFF // 16
        links = {}
        acc = 0
        for _, c, f in units:
            acc += c
            vals = f()
            sl = min(int(np.ceil(acc / total * 2 * nsl)), 2 * nsl) - 1
            links.setdefault(sl, []).extend(vals)
        fsrc = (l & 1) * 8
        fu = fxb.bitcast(jnp.uint32)
        never = jnp.full((8, 128), zg[0], jnp.int32) != 0
        cols = []
        for c in range(8):
            rows = []
            for r in range(nsl):
                v = fu[fsrc + c, r * 8:(r + 1) * 8, :]
                for a in links.get((c // 4) * nsl + r, [])[c % 4::4]:
                    v = jnp.where(never, pltpu.bitcast(a, jnp.uint32), v)
                rows.append(v)
            cols.append(pltpu.bitcast(jnp.concatenate(rows, 0), bf16))
        wg = pltpu.bitcast(wraw.bitcast(jnp.uint32)[l, g], bf16)
        y = jnp.dot(jnp.concatenate(cols, 1), wg, preferred_element_type=f32)
        xn = fx32[g] * (y + fb[l * 8 + g, 0:1, :]) + fx32[8 + g]
        fx32[8 + g] = xn
        fxb[8 - fsrc + g] = xn.astype(bf16)
        for r, f in zip(tail, late):
            f(y[r * 8:r * 8 + 16])

    w_wait(0)
    w_start(1)
    for _, f in s1_units(0, 0, tmp[0]):
        f()

    def pair(n, carry):
        l = lax.shift_right_logical(n, 2)
        g = (n & 3) * 2

        @pl.when(jnp.logical_and(g == 6, l + 1 < L))
        def _():
            w_wait(l + 1)

        @pl.when(jnp.logical_and(g == 6, l + 2 < L))
        def _():
            w_start(l + 2)

        @pl.when(n == 4 * L - 5)
        def _():
            x_copy(0).start()
            x_copy(1).start()

        zg = [lax.shift_right_logical(n, 12 + k) for k in range(8)]
        nn = jnp.minimum(2 * n + 2, 8 * L - 1)
        half(l, g, l, g + 1, tmp[0], tmp[1], zg[:4], ())
        half(l, g + 1, lax.shift_right_logical(nn, 3), nn & 7, tmp[1], tmp[0], zg[4:], cfg["tail"])
        return carry

    lax.fori_loop(0, 4 * L, pair, 0)
    for c in range(8):
        fout(c).start()
    x_copy(0).wait()
    ctx.update(z=0, slot={0: 0}, j=-1)
    for w in ("e1", "e2"):
        for t in range(4):
            task[w](L - 1, t, None)

    def main(step, carry):
        @pl.when(step + 1 < nsteps)
        def _():
            x_copy(step + 1).wait()

        @pl.when(step + 2 < nsteps)
        def _():
            x_copy(step + 2).start()

        zz = [lax.shift_right_logical(step, 12 + k) for k in range(_NZ)]
        ctx.update(mask=jnp.full((H, 128), zz[0], jnp.int32) != 0,
                   slot={-1: (step + 3) & 3, 0: step & 3, 1: (step + 1) & 3}, oslot=step & 1)
        wu = wexp.bitcast(jnp.uint32)

        def wtile(l, k):
            return pltpu.bitcast(wu[l, k], bf16)

        prods = [(l, p, q) for _j in range(TPS) for l in range(L) for (p, q) in order]
        npr = len(prods)
        free = [0, 0, 0, 0]
        anchors = []
        pstart = []
        for pi, (l, p, q) in enumerate(prods):
            pstart.append(min(free))
            if (p, q) in l3set:
                for j in range(7):
                    mx = int(np.argmin(free))
                    anchors += [(free[mx] + g * 8, pi, j, g) for g in range(NG)]
                    free[mx] += H
            else:
                anchors += [(max(free) + g * 8, pi, 0, g) for g in range(2 * NG)]
                free = [f + 2 * H for f in free]
        pstart.append(max(free))
        anchors.sort()
        times = np.array([a[0] for a in anchors])

        def tpos(x):
            i = int(np.floor(x))
            return pstart[i] + (x - i) * (pstart[min(i + 1, npr)] - pstart[i])

        wv, ws, wl = cfg["wts"]
        P = 4 * NG
        nb = pstart[-1] // 8 + 1
        load = np.zeros(nb)

        def spread(t0, t1, valu, st_, ld_):
            b0, b1 = max(int(t0 // 8), 0), max(int(t1 // 8), 1)
            load[b0:b1] += (valu / 4 * wv + st_ * ws + ld_ / 3 * wl) / max(int(t1 // 8) - int(t0 // 8), 1)

        for pi, (l, p, q) in enumerate(prods):
            t = len(_MIDB[q])
            big = (p, q) in l3set
            t0, t1 = pstart[pi], pstart[pi + 1]
            spread(t0 - cfg["lat"], t1 - cfg["lat"], (t - 1 + (2.875 if big else 0.5)) * P, 0,
                   t * P + (56 if big else 32))
            sa, sl = {5: (1, 1), 1: (5, 4), 2: (1, 1), 6: (1, 1)}.get(p, (0, 0))
            bias = 1 if (p in BP and q in BQ) else 0
            spread(t0, t1 + (H // 2 if big else 0), ((2.75 if big else 1) + bias + sa) * P, P, sl * P)

        amp, seeds = cfg["jit"]
        for k, sd in enumerate(seeds):
            b0, b1 = pstart[k * 49] // 8, pstart[k * 49 + 49] // 8
            if sd:
                load[b0:b1] += amp * np.random.RandomState(sd).randn(b1 - b0)

        tcost = {"w1": (26, 8, 15), "w2": (34, 12, 19), "w3": (16, 4, 11), "w4": (42, 12, 27),
                 "w5": (35, 12, 28), "o1": (31, 8, 15), "o2": (31, 8, 15), "o3": (16, 4, 11),
                 "o4": (39, 8, 23), "o5": (27, 4, 16), "e1": (14, 8, 4), "e2": (22, 12, 8),
                 "e4": (22, 12, 8), "e5": (30, 16, 16)}
        kern = np.hanning(cfg["sm"] + 2)[1:-1]
        kern /= kern.sum()
        sched = {}
        jobs = [(w, l) for l in range(L - 1) for w in ("w1", "w2", "w3", "w4", "w5")]
        jobs += [(w, L - 1) for w in ("e1", "o1", "e2", "o2", "e4", "e5", "o3", "o4", "o5")]
        todo = [(jn, w, l, j) for j in range(TPS) for jn, (w, l) in enumerate(jobs)]
        wof = lambda w, l: win.get((w, l), win[w])
        todo.sort(key=lambda e: wof(e[1], e[2])[1] - wof(e[1], e[2])[0])
        for jn, w, l, j in todo:
            b0, b1 = wof(w, l)
            i0, i1, jj = (j * L + l) * 49 + b0, (j * L + l) * 49 + b1, j
            if i0 >= npr:
                i0, i1, jj = i0 - npr, i1 - npr, j - TPS
            assert i1 <= npr
            lo, hi = int(np.ceil(tpos(i0) / 8)), int(tpos(i1) // 8)
            picks = []
            for _k in range(P):
                sm = np.convolve(load, kern, mode="same")
                bb = lo + int(np.argmin(sm[lo + 1:hi + 1]))
                picks.append(bb)
                spread(bb * 8, bb * 8 + 24 + (cfg["a2d"] - 8 if w in cfg["a2w"] else 0), *tcost[w])
            slots = []
            for bb in sorted(picks):
                ai = int(np.searchsorted(times, bb * 8))
                while anchors[ai][1] < int(i0):
                    ai += 1
                slots.append(anchors[ai][1:])
            if w in cfg["a2w"]:
                for bb in sorted(picks):
                    slots.append(anchors[int(np.searchsorted(times, bb * 8 + cfg["a2d"]))][1:])
            for t in range(4):
                al = slots[t * NG:(t + 1) * NG] + slots[P + t * NG:P + (t + 1) * NG]
                sched.setdefault(max(a[0] for a in al), []).append((w, l, t, al, jn, jj))
        for v in sched.values():
            v.sort(key=lambda e: (e[5], e[4], e[2]))

        subs = {}
        l3pos = 0
        for pi, (l, p, q) in enumerate(prods):
            ctx["z"] = zz[{1: 0, 2: 0, 3: 0, 5: 0, 4: 1, 6: 2, 7: 3}[q]]
            srcs = [f"a{p}"]
            qv = [_lin([(ld(n, b, t), s) for n in srcs for b, s in _MIDB[q]]) for t in range(4)]
            k0 = tile0[p, q]
            if (p, q) in l3set:
                a1 = qv[0] + qv[3]
                u = qv[1] + qv[2]
                if l in cfg["ug"][0] and l3pos % 4 in cfg["ug"][1] and pstart[pi] >= 200:
                    gl = []
                    for g in range(NG):
                        gt = pstart[pi] + (g // 2) * 16 - cfg["ug"][2]
                        ai = int(np.searchsorted(times, gt, side="right")) - 1
                        while anchors[ai][1] >= pi:
                            ai -= 1
                        _, api, j, ag = anchors[ai]
                        gl.append(subs[api][j][ag * 8:(ag + 1) * 8, :])
                    u = anc(u, jnp.concatenate(gl, 0))
                av = {1: a1, 3: qv[0] - qv[1], 5: qv[0] + qv[1], 4: qv[1] + qv[3],
                      7: qv[1] - qv[3], 2: u + a1, 6: u - a1}
                so = cfg["so"][l3pos % 4]
                l3pos += 1
                m = {r: jnp.dot(av[r].astype(bf16), wtile(l, k0 + r - 1), preferred_element_type=f32)
                     for r in so}
                subs[pi] = [m[r] for r in so]
                mq = _comb7o(m, so, anc if (l3pos - 1) % 4 in cfg["elink"] else None)
            else:
                a = jnp.concatenate(
                    [jnp.concatenate(qv[:2], 1), jnp.concatenate(qv[2:], 1)], 0).astype(bf16)
                wt = [wtile(l, k0 + t) for t in range(4)]
                wm = jnp.concatenate([jnp.concatenate(wt[:2], 1), jnp.concatenate(wt[2:], 1)], 0)
                mm = jnp.dot(a, wm, preferred_element_type=f32)
                subs[pi] = [mm[:, :128]]
                mq = [mm[:H, :128], mm[:H, 128:], mm[H:, :128], mm[H:, 128:]]
            if p in BP and q in BQ:
                row = l * 64 + (BP.index(p) * 4 + BQ.index(q)) * 4
                mq = [mq[t] + beta[row + t:row + t + 1, :] for t in range(4)]
            for t in range(4):
                v = mq[t]
                if p == 5:
                    v = v + ld("u3", q - 1, t)
                elif p == 1:
                    r3 = ld("u3", q - 1, t)
                    v = v + (((ld("u4", q - 1, t) + ld("u7", q - 1, t)) + (r3 + r3)) - ld("u5", q - 1, t))
                elif p == 2:
                    v = v + ld("u4", q - 1, t)
                elif p == 6:
                    v = v - ld("u7", q - 1, t)
                st(uname(p, l), q - 1, t, v)
            for (w, tl, t, al, jn, jj) in sched.get(pi, []):
                a = jnp.concatenate([subs[api][j][g * 8:(g + 1) * 8, :] for api, j, g in al], 0)
                ctx.update(z=zz[8 + jn % 6], j=jj, a2=a[H:] if len(al) > NG else None)
                task[w](tl, t, a[:H])

        @pl.when(step >= 1)
        def _():
            top_copy(step - 1).wait()

        @pl.when(step >= 2)
        def _():
            bot_copy(step - 1).wait()

        top_copy(step).start()

        @pl.when(step >= 1)
        def _():
            bot_copy(step).start()

        return carry

    lax.fori_loop(0, nsteps, main, 0)

    ctx.update(z=0, slot={-1: (nsteps - 1) % 4}, j=-1, oslot=nsteps % 2)
    for w in ("o3", "o4", "o5"):
        for t in range(4):
            task[w](L - 1, t, None)
    bot_copy(nsteps).start()
    for c in range(8):
        fout(c).wait()
    top_copy(nsteps - 1).wait()
    bot_copy(nsteps - 1).wait()
    bot_copy(nsteps).wait()


_L3SET = tuple((p, q) for p in range(2, 8) for q in range(2, 8))
_WIN = {"w1": (14, 35), "w2": (35, 46), "w3": (42, 49), "w4": (49, 60), "w5": (60, 74),
        "e1": (0, 35), "o1": (14, 35), "e2": (35, 46), "o2": (35, 48.5), "e4": (49, 60), "e5": (60, 74),
        "o3": (49, 60), "o4": (60, 170), "o5": (170, 290)}
_SO = ((3, 5, 1, 4, 7, 2, 6),) * 4
_CFG = dict(l3set=_L3SET + ((1, 3), (1, 5), (1, 2), (1, 7)), win=_WIN, tm=384, tps=1, roff=256, kpos={3: 4, 5: 2, 4: 4, 7: 2, 1: 4, 2: 4, 6: 2}, wts=(1, 0.2, 0), lat=135, sm=6, merge="a", elink=(3,), ug=((0,), (0, 1, 2, 3), 100), bp=(3, 4, 7, 1), bq=(5, 2, 1, 6), jit=(0.0, (0,) * 6), a2w=("w4", "w2"), a2d=24, a2i=(0,), s1f=0.75, tail=(14, 17, 20, 23, 26), pt=(1,), so=_SO, qo=(3, 5, 2, 4, 7, 6, 1))


def _build(**kw):
    cfg = dict(_CFG, **kw)

    def fn(x0, ws, bs):
        B, Dm = x0.shape
        L = ws.shape[0]
        st = cfg["tm"] * cfg["tps"]
        nsteps = (B - cfg["roff"]) // st
        ntiles = _plan(cfg["l3set"], cfg)[2]
        return pl.pallas_call(
            functools.partial(_kernel, L=L, nsteps=nsteps, cfg=cfg),
            in_specs=[
                pl.BlockSpec(memory_space=pl.ANY),
                pl.BlockSpec(memory_space=pl.ANY),
                pl.BlockSpec(memory_space=pl.ANY),
            ],
            out_specs=pl.BlockSpec(memory_space=pl.ANY),
            out_shape=jax.ShapeDtypeStruct((B, Dm), x0.dtype),
            scratch_shapes=[
                pltpu.VMEM((L, Dm), bf16),
                pltpu.VMEM((4, st, Dm), bf16),
                pltpu.VMEM((2, st, Dm), bf16),
                pltpu.VMEM((L, 8, Dm, 128), bf16),
                pltpu.VMEM((L, ntiles, 128, 128), bf16),
                pltpu.VMEM((L * 64, 128), f32),
                pltpu.VMEM((16, cfg["roff"], 128), f32),
                pltpu.VMEM((16, cfg["roff"], 128), bf16),
                pltpu.VMEM((L * 8, 8, 128), f32),
                pltpu.SemaphoreType.DMA((4,)),
                pltpu.SemaphoreType.DMA((L,)),
                pltpu.SemaphoreType.DMA((2,)),
                pltpu.SemaphoreType.DMA((2,)),
                pltpu.SemaphoreType.DMA((9,)),
            ]
            + [pltpu.VMEM((1, 260 * 8, 128), f32)] * 2
            + [pltpu.VMEM((1, sz * 8, 128), f32) for _, sz in _bufkeys(cfg)],
            compiler_params=pltpu.CompilerParams(
                vmem_limit_bytes=126 * 1024 * 1024,
                disable_bounds_checks=True,
            ),
        )(x0, ws, bs)

    return fn


@jax.jit
def pallas_standalone__dcn_v2_cross__recsys_kernel(
    x0: jax.Array,
    ws: jax.Array,
    bs: jax.Array,
):
    return _build()(x0, ws, bs)
```

```python
import functools

import numpy as np
import jax
import jax.numpy as jnp
from jax import lax
import jax.experimental.pallas as pl
import jax.experimental.pallas.tpu as pltpu

f32 = jnp.float32
bf16 = jnp.bfloat16

_D = float(np.sqrt(3.0))
_TM = 384
_ROFF = 256
_H = _TM // 8
_NG = _H // 8
_BS = 9
_PH = (3, 5, 4, 7, 1, 2, 6)
_SO = (3, 5, 1, 4, 7, 2, 6)
_MIDB = {1: [(0, 1)], 2: [(1, 1)], 3: [(2, 1)], 5: [(3, 1)],
         4: [(0, 1), (2, -1)], 6: [(1, 1), (0, -1)], 7: [(3, 1), (0, -1)]}
_ZQ = {1: 0, 2: 0, 3: 0, 5: 0, 4: 1, 6: 2, 7: 3}
_CVEC = {1: [1, 0, 0, 1], 2: [0, 0, 1, -1], 3: [1, 1, 1, 1], 4: [1, 0, 1, 0],
         5: [-1, 1, 1, -1], 6: [0, 0, 1, 1], 7: [1, 0, -1, 0]}

_NAMES = ([(f"u{p}", 7) for p in (3, 4, 7, 5, 1, 2, 6)]
          + [(f"a{p}", 4) for p in (3, 4, 5, 7, 2, 6, 1)]
          + [(f"{s}{k}", 4) for s in ("fx", "H", "G", "U", "V") for k in range(2)]
          + [(f"x0{o}", 4) for o in range(4)]
          + [("u2x", 7), ("u6x", 7)] + [(f"{s}{k}", 4) for s in "HGUV" for k in (2, 3)])

_WIN = {"w1": (14, 35, 35), "w2": (35, 46, 48), "w3": (42, 49, 49), "w4": (49, 60, 62),
        "w5": (60, 74, 76), "e1": (0, 35, 35), "o1": (14, 35, 48), "e2": (35, 46, 48),
        "o2": (35, 48.5, 48), "e4": (49, 60, 62), "e5": (60, 74, 76), "o3": (49, 60, 85),
        "o4": (60, 170, 285), "o5": (170, 290, 300)}
_TCOST = {"w1": (26, 8), "w2": (34, 12), "w3": (16, 4), "w4": (42, 12), "w5": (35, 12),
          "o1": (31, 8), "o2": (31, 8), "o3": (16, 4), "o4": (39, 8), "o5": (27, 4),
          "e1": (14, 8), "e2": (22, 12), "e4": (22, 12), "e5": (30, 16)}
_CFG = dict(
    inner=tuple((p, q) for p in range(2, 8) for q in range(2, 8)) + ((1, 3), (1, 5), (1, 2), (1, 7)),
    kpos={3: 4, 5: 2, 4: 4, 7: 2, 1: 4, 2: 4, 6: 2},
    qo=(3, 5, 2, 4, 7, 6, 1),
    bp=(3, 4, 7, 1),
    bq=(5, 2, 1, 6),
    win=_WIN, ws=0.2, lat=135, sm=6, two=("w4", "w2"), gap=24, ulead=100,
    s1f=0.75, tail=(14, 17, 20, 23, 26),
)


def _kappa(bset):
    m = np.array([_CVEC[p] for p in bset], np.float64).T
    pats = [np.array([1, 0, _D, 0]), np.array([0, 1 / _D, 0, 1])]
    return [dict(zip(bset, np.linalg.solve(m, t))) for t in pats]


def _comb7(m, link=None):
    s = m[3] + m[5]
    e = (m[3] - m[5]) + m[1]
    return [(e + m[4]) + m[7], s if link is None else link(s, e),
            (((s + m[4]) - m[7]) + m[2]) + m[6], (e - m[2]) + m[6]]


def _fwd(x):
    a1 = x[0] + x[3]
    return [a1, ((x[1] + x[2]) + a1) * 0.5, x[0] - x[1], x[0] + x[1]]


def _bexp(b):
    b1 = b[0] + b[3]
    u = b[1] + b[2]
    return {1: b1, 2: b[0] - b[1], 3: b[1] - b[3], 4: u - b1, 5: b[1] + b[3], 6: b[0] + b[1],
            7: u + b1}


def _rowcol(o, i, t):
    r = (o // 2) * 4 + (i // 2) * 2 + t // 2
    c = (o % 2) * 4 + (i % 2) * 2 + t % 2
    e = (o // 2 - o % 2) + (i // 2 - i % 2) + (t // 2 - t % 2)
    return r, c, e


def _products(cfg):
    order = []
    for p in _PH:
        ks = [q for q in range(1, 8) if (p, q) not in cfg["inner"]]
        ls = [q for q in cfg["qo"] if (p, q) in cfg["inner"]]
        kp = cfg["kpos"][p]
        order += [(p, q) for q in ls[:kp] + ks + ls[kp:]]
    tile0 = {}
    n = 0
    for pq in order:
        tile0[pq] = n
        n += 7 if pq in cfg["inner"] else 4
    return order, tile0, n


def _qsize(k):
    return (k * _BS + 7) // 4 * 4


def _bufkeys():
    keys = []
    for n, k in _NAMES:
        if n[0] == "a":
            keys.append(((n, 0), 4 * _qsize(k)))
        else:
            keys += [((n, t), _qsize(k)) for t in range(4)]
    return keys


def _schedule(L, order, cfg):
    inner, win = cfg["inner"], cfg["win"]
    prods = [(l, p, q) for l in range(L) for (p, q) in order]
    npr = len(prods)
    free = [0, 0, 0, 0]
    anchors = []
    pstart = []
    for pi, (l, p, q) in enumerate(prods):
        pstart.append(min(free))
        if (p, q) in inner:
            for j in range(7):
                mx = int(np.argmin(free))
                anchors += [(free[mx] + g * 8, pi, j, g) for g in range(_NG)]
                free[mx] += _H
        else:
            anchors += [(max(free) + g * 8, pi, 0, g) for g in range(2 * _NG)]
            free = [f + 2 * _H for f in free]
    pstart.append(max(free))
    anchors.sort()
    times = np.array([a[0] for a in anchors])

    def tpos(x):
        i = int(np.floor(x))
        return pstart[i] + (x - i) * (pstart[min(i + 1, npr)] - pstart[i])

    npos = 4 * _NG
    load = np.zeros(pstart[-1] // 8 + 1)

    def spread(t0, t1, valu, stores):
        b0, b1 = max(int(t0 // 8), 0), max(int(t1 // 8), 1)
        load[b0:b1] += (valu / 4 + stores * cfg["ws"]) / max(int(t1 // 8) - int(t0 // 8), 1)

    for pi, (l, p, q) in enumerate(prods):
        big = (p, q) in inner
        t0, t1 = pstart[pi], pstart[pi + 1]
        spread(t0 - cfg["lat"], t1 - cfg["lat"],
               (len(_MIDB[q]) - 1 + (2.875 if big else 0.5)) * npos, 0)
        extra = {5: 1, 1: 5, 2: 1, 6: 1}.get(p, 0) + (p in cfg["bp"] and q in cfg["bq"])
        spread(t0, t1 + (_H // 2 if big else 0), ((2.75 if big else 1) + extra) * npos, npos)

    kern = np.hanning(cfg["sm"] + 2)[1:-1]
    kern /= kern.sum()
    jobs = [(w, l) for l in range(L - 1) for w in ("w1", "w2", "w3", "w4", "w5")]
    jobs += [(w, L - 1) for w in ("e1", "o1", "e2", "o2", "e4", "e5", "o3", "o4", "o5")]
    sched = {}
    for jn, (w, l) in sorted(enumerate(jobs), key=lambda e: win[e[1][0]][1] - win[e[1][0]][0]):
        i0, i1, last = (l * 49 + v for v in win[w])
        prev = i0 >= npr
        if prev:
            i0, i1, last = i0 - npr, i1 - npr, last - npr
        lo, hi = int(np.ceil(tpos(i0) / 8)), int(tpos(i1) // 8)
        picks = []
        for _ in range(npos):
            sm = np.convolve(load, kern, mode="same")
            bb = lo + int(np.argmin(sm[lo + 1:hi + 1]))
            picks.append(bb)
            spread(bb * 8, bb * 8 + 16 + (cfg["gap"] if w in cfg["two"] else 8), *_TCOST[w])
        picks.sort()
        slots = []
        for bb in picks:
            ai = int(np.searchsorted(times, bb * 8))
            while anchors[ai][1] < i0:
                ai += 1
            slots.append(anchors[ai][1:])
        if w in cfg["two"]:
            slots += [anchors[int(np.searchsorted(times, bb * 8 + cfg["gap"]))][1:] for bb in picks]
        for t in range(4):
            al = slots[t * _NG:(t + 1) * _NG] + slots[npos + t * _NG:npos + (t + 1) * _NG]
            at = max(a[0] for a in al)
            assert i0 <= at <= last, (w, l, t, at)
            sched.setdefault(at, []).append((-1 if prev else 0, jn, t, w, l, al))
    where = {}
    for at, v in sched.items():
        v.sort(key=lambda e: e[:3])
        for k, e in enumerate(v):
            where[e[3], e[4], e[2]] = (at, k)
    for a, b in (("w1", "w2"), ("w2", "w4"), ("w3", "w4"), ("w4", "w5"), ("e1", "e2"),
                 ("e4", "e5"), ("o3", "o4"), ("o4", "o5")):
        for l in (range(L - 1) if a[0] == "w" else (L - 1,)):
            assert all(where[a, l, t] < where[b, l, t] for t in range(4)), (a, b, l)

    ugate = {}
    for pi in range(49):
        if prods[pi][1:] in inner and pstart[pi] >= 200:
            al = []
            for g in range(_NG):
                gt = pstart[pi] + (g // 2) * 16 - cfg["ulead"]
                ai = int(np.searchsorted(times, gt, side="right")) - 1
                while anchors[ai][1] >= pi:
                    ai -= 1
                al.append(anchors[ai][1:])
            ugate[pi] = al
    return prods, sched, ugate


def _kernel(x_hbm, w_hbm, b_hbm, o_hbm, b_ref, ring, stage, wraw, wexp, beta, fx32, fxb, fb,
            xsem, wsem, tsem, bsem, fsem, *bufs, L, nsteps, cfg):
    H, HT = _H, _TM // 2
    inner, bp, bq = cfg["inner"], cfg["bp"], cfg["bq"]
    order, tile0, _ = _products(cfg)
    tmp = bufs[:2]
    buf = dict(zip([k for k, _ in _bufkeys()], bufs[2:]))
    skew = {n: k % 4 for k, (n, _) in enumerate(_NAMES)}
    ctx = {}

    def x_copy(i):
        return pltpu.make_async_copy(
            x_hbm.at[pl.ds(pl.multiple_of(_ROFF + i * _TM, 64), _TM)], ring.at[i & 3],
            xsem.at[i & 3])

    def w_copies(l):
        return [pltpu.make_async_copy(w_hbm.at[l, :, pl.ds(c * 128, 128)], wraw.at[l, c],
                                      wsem.at[l]) for c in range(8)]

    def top_copy(i):
        return pltpu.make_async_copy(
            stage.at[i & 1, pl.ds(HT, HT)],
            o_hbm.at[pl.ds(pl.multiple_of(_ROFF + i * _TM, 64), HT)], tsem.at[i & 1])

    def bot_copy(i):
        return pltpu.make_async_copy(
            stage.at[i & 1, pl.ds(0, HT)],
            o_hbm.at[pl.ds(pl.multiple_of(_ROFF + i * _TM - HT, 64), HT)], bsem.at[i & 1])

    def fin(c):
        return pltpu.make_async_copy(
            x_hbm.at[pl.ds(0, _ROFF), pl.ds(c * 128, 128)], fxb.at[c], fsem.at[c])

    def fout(c):
        return pltpu.make_async_copy(
            fxb.at[(L & 1) * 8 + c], o_hbm.at[pl.ds(0, _ROFF), pl.ds(c * 128, 128)], fsem.at[c])

    def loc(n, b, t):
        if n[0] == "a":
            return buf[n, 0], (t * _qsize(4) + (skew[n] + t) % 4 + b * _BS) * 8
        return buf[n, t], ((skew[n] + t) % 4 + b * _BS) * 8

    def ld(n, b, t):
        ref, o = loc(n, b, t)
        return ref[ctx["z"], o:o + H, :]

    def st(n, b, t, v):
        ref, o = loc(n, b, t)
        ref[0, o:o + H, :] = v

    def anc(v, a):
        return v if a is None else jnp.where(ctx["never"], a, v)

    def xin(j, o, i, t):
        r, c, _ = _rowcol(o, i, t)
        return ring[ctx["slot"][j], r * H:(r + 1) * H, c * 128:(c + 1) * 128].astype(f32)

    def sname(s, l):
        return f"{s}{l - L + 4 if l >= L - 2 else l % 2}"

    def uname(p, l):
        return f"u{p}x" if (l == L - 1 and p in (2, 6)) else f"u{p}"

    def upd(l, p, s, t, a):
        m = {q: ld(uname(p, l), q - 1, t) for q in range(1, 8)}
        m[3] = anc(m[3], a)
        y = _comb7(m)
        if l > 0:
            y = [y[i] + ld(sname(s, l - 1), i, t) for i in range(4)]
        for i in range(4):
            st(sname(s, l), i, t, y[i])
        return y

    def g22(l, t, a):
        v = upd(l, 6, "V", t, a)
        return [v[i] + (ld(sname("G", l), i, t) - ld(sname("U", l), i, t)) for i in range(4)]

    def g21(l, t, a):
        return [anc(ld(sname("U", l), i, t), a[i]) + ld(sname("V", l), i, t)
                + ld(sname("H", l), i, t) for i in range(4)]

    def gate(o, g, t):
        g = [anc(g[0], ctx["a2"])] + g[1:]
        return [ld(f"x0{o}", i, t) * g[i] for i in range(4)]

    def emit(o, g, t):
        for i in range(4):
            r, c, e = _rowcol(o, i, t)
            y = xin(ctx["j"], o, i, t) * g[i]
            if e:
                y = y * (_D ** -e)
            r0 = ctx["j"] * _TM + r * H + HT
            stage[ctx["oslot"], r0:r0 + H, c * 128:(c + 1) * 128] = y.astype(bf16)

    def fresh(o, t, a):
        xs = []
        for i in range(4):
            e = _rowcol(o, i, t)[2]
            v = xin(ctx["j"] + 1, o, i, t)
            if i == 0:
                v = anc(v, a)
            st(f"x0{o}", i, t, v)
            xs.append(v * (_D ** e) if e else v)
        return xs

    def f1(l, t, x):
        for i, v in enumerate(_fwd(x)):
            st(f"fx{l % 2}", i, t, v)

    def f2(l, t, x):
        for i, v in enumerate(_fwd(x)):
            w = ld(f"fx{l % 2}", i, t)
            st("a3", i, t, v - w)
            st("a5", i, t, v + w)

    def f4(l, t, x):
        for i, v in enumerate(_fwd(x)):
            w = ld(f"fx{l % 2}", i, t)
            st("a4", i, t, w + v)
            st("a7", i, t, w - v)

    def f5(l, t, x):
        for i, v in enumerate(_fwd(x)):
            u = ld(f"fx{l % 2}", i, t) + v
            a1 = ld("a3", i, t) + ld("a4", i, t)
            st("a1", i, t, a1)
            st("a2", i, t, u + a1)
            st("a6", i, t, u - a1)

    task = {
        "w1": lambda l, t, a: f1(l, t, gate(1, upd(l, 5, "H", t, a), t)),
        "w2": lambda l, t, a: f2(l, t, gate(0, upd(l, 1, "G", t, a), t)),
        "w3": lambda l, t, a: upd(l, 2, "U", t, a),
        "w4": lambda l, t, a: f4(l, t, gate(3, g22(l, t, a), t)),
        "w5": lambda l, t, a: f5(l, t, gate(2, g21(l, t, [a, None, None, None]), t)),
        "o1": lambda l, t, a: emit(1, upd(l, 5, "H", t, a), t),
        "o2": lambda l, t, a: emit(0, upd(l, 1, "G", t, a), t),
        "o3": lambda l, t, a: upd(l, 2, "U", t, a),
        "o4": lambda l, t, a: emit(3, g22(l, t, a), t),
        "o5": lambda l, t, a: emit(2, g21(l, t, [a] * 4), t),
        "e1": lambda l, t, a: f1(l, t, fresh(1, t, a)),
        "e2": lambda l, t, a: f2(l, t, fresh(0, t, a)),
        "e4": lambda l, t, a: f4(l, t, fresh(3, t, a)),
        "e5": lambda l, t, a: f5(l, t, fresh(2, t, a)),
    }

    b_copy = pltpu.make_async_copy(b_hbm, b_ref, fsem.at[8])
    b_copy.start()
    for c in range(8):
        fin(c).start()
    for cp in w_copies(0):
        cp.start()

    for n in ("u2x", "u6x", sname("U", L - 2), sname("V", L - 2), sname("G", L - 1),
              sname("H", L - 1)):
        for t in range(4):
            buf[n, t][...] = jnp.zeros(buf[n, t].shape, f32)
    ring[3, HT:, :] = jnp.zeros((HT, ring.shape[2]), bf16)

    b_copy.wait()
    kap, kaq = _kappa(bp), _kappa(bq)
    for l in range(L):
        bl = b_ref[l:l + 1, :].astype(f32)
        for c in range(8):
            fb[l * 8 + c, 0:1, :] = bl[:, c * 128:(c + 1) * 128]
        if l == 0:
            bl = bl + 1.0
        for pi, p in enumerate(bp):
            for qi, q in enumerate(bq):
                for c3 in range(2):
                    acc = None
                    for c1 in range(2):
                        for c2 in range(2):
                            k = float(kap[c1][p] * kaq[c2][q])
                            if abs(k) < 1e-12:
                                continue
                            c = c1 * 4 + c2 * 2 + c3
                            term = bl[:, c * 128:(c + 1) * 128] * k
                            acc = term if acc is None else acc + term
                    for r3 in range(2):
                        row = l * 64 + (pi * 4 + qi) * 4 + r3 * 2 + c3
                        beta[row:row + 1, :] = acc * (_D ** (r3 - c3))
    for c in range(8):
        fin(c).wait()
    for c in range(8):
        v = fxb[c].astype(f32)
        fx32[c] = v
        fx32[8 + c] = v

    def toff(p, i, t):
        return ((p - 1) * 37 + (i * 4 + t) * 2 + i) * 8

    def s1_units(l, g, dst):
        r0 = pl.multiple_of(g * 16, 16)

        def unit(i, t):
            blk = []
            for o in range(4):
                r, c, e = _rowcol(o, i, t)
                v = wraw[l, c, pl.ds(r * 128 + r0, 16), :].astype(f32)
                blk.append(v * (0.125 * _D ** e))
            ex = _bexp(blk)
            for p in _PH:
                dst[0, toff(p, i, t):toff(p, i, t) + 16, :] = ex[p]
            return [ex[7][:8], ex[7][8:]]

        return [(34, functools.partial(unit, i, t)) for i in range(4) for t in range(4)]

    def s2_units(l, g, src, zg):
        r0 = pl.multiple_of(g * 16, 16)

        def put(p, q, qs):
            f = (2.0 if p == 1 else 1.0) * (2 if q in (1, 2, 6) else 1)
            if (p, q) in inner:
                inn = _bexp([v * f for v in qs] if f != 1 else qs)
                tiles = [inn[1] + inn[1]] + [inn[r] for r in range(2, 8)]
            else:
                tiles = [v * (2 * f) for v in qs]
            for k, v in enumerate(tiles):
                wexp[l, tile0[p, q] + k, pl.ds(r0, 16), :] = v.astype(bf16)
            return tiles

        def unit(p, un, a=None):
            def tl(i):
                vs = [src[zg[1 + un], toff(p, i, t):toff(p, i, t) + 16, :] for t in range(4)]
                if a is not None and i == 1:
                    vs[1] = jnp.where(jnp.full((16, 128), zg[0], jnp.int32) != 0, a, vs[1])
                return vs

            if un == 0:
                x, y, qa, qb = tl(0), tl(1), 2, 6
            elif un == 1:
                x, y, qa, qb = tl(1), tl(3), 3, 5
            else:
                x = [u + v for u, v in zip(tl(1), tl(2))]
                y = [u + v for u, v in zip(tl(0), tl(3))]
                qa, qb = 4, 7
                put(p, 1, y)
            ta = put(p, qa, [u - v for u, v in zip(x, y)])
            tb = put(p, qb, [u + v for u, v in zip(x, y)])
            if len(tb) == 4:
                return [v[:8] for v in tb]
            return [ta[-1][:8], tb[-1][8:]]

        return [(((40, 40, 68) if p == 1 else (82, 66, 94))[un], functools.partial(unit, p, un))
                for p in _PH for un in range(3)]

    def half(l, g, ln, gn, src, dst, zg, tail):
        u2 = s2_units(l, g, src, zg)
        u1 = s1_units(ln, gn, dst)
        units = sorted([(k / len(u2), c, f) for k, (c, f) in enumerate(u2)]
                       + [((k + 0.5) / len(u1) * cfg["s1f"], c, f) for k, (c, f) in enumerate(u1)],
                       key=lambda e: e[0])
        late = [f for _, _, f in units[len(units) - len(tail):]]
        units = units[:len(units) - len(tail)]
        total = sum(c for _, c, _ in units)
        nsl = _ROFF // 16
        links = {}
        acc = 0
        for _, c, f in units:
            acc += c
            sl = min(int(np.ceil(acc / total * 2 * nsl)), 2 * nsl) - 1
            links.setdefault(sl, []).extend(f())
        fsrc = (l & 1) * 8
        fu = fxb.bitcast(jnp.uint32)
        never = jnp.full((8, 128), zg[0], jnp.int32) != 0
        cols = []
        for c in range(8):
            rows = []
            for r in range(nsl):
                v = fu[fsrc + c, r * 8:(r + 1) * 8, :]
                for a in links.get((c // 4) * nsl + r, [])[c % 4::4]:
                    v = jnp.where(never, pltpu.bitcast(a, jnp.uint32), v)
                rows.append(v)
            cols.append(pltpu.bitcast(jnp.concatenate(rows, 0), bf16))
        wg = pltpu.bitcast(wraw.bitcast(jnp.uint32)[l, g], bf16)
        y = jnp.dot(jnp.concatenate(cols, 1), wg, preferred_element_type=f32)
        xn = fx32[g] * (y + fb[l * 8 + g, 0:1, :]) + fx32[8 + g]
        fx32[8 + g] = xn
        fxb[8 - fsrc + g] = xn.astype(bf16)
        for r, f in zip(tail, late):
            f(y[r * 8:r * 8 + 16])

    for cp in w_copies(0):
        cp.wait()
    for cp in w_copies(1):
        cp.start()
    for _, f in s1_units(0, 0, tmp[0]):
        f()

    def pair(n, carry):
        l = lax.shift_right_logical(n, 2)
        g = (n & 3) * 2

        @pl.when(jnp.logical_and(g == 6, l + 1 < L))
        def _():
            for cp in w_copies(l + 1):
                cp.wait()

        @pl.when(jnp.logical_and(g == 6, l + 2 < L))
        def _():
            for cp in w_copies(l + 2):
                cp.start()

        @pl.when(n == 4 * L - 5)
        def _():
            x_copy(0).start()
            x_copy(1).start()

        zg = [lax.shift_right_logical(n, 12 + k) for k in range(8)]
        nn = jnp.minimum(2 * n + 2, 8 * L - 1)
        half(l, g, l, g + 1, tmp[0], tmp[1], zg[:4], ())
        half(l, g + 1, lax.shift_right_logical(nn, 3), nn & 7, tmp[1], tmp[0], zg[4:], cfg["tail"])
        return carry

    lax.fori_loop(0, 4 * L, pair, 0)
    for c in range(8):
        fout(c).start()
    x_copy(0).wait()
    ctx.update(z=0, slot={0: 0}, j=-1)
    for w in ("e1", "e2"):
        for t in range(4):
            task[w](L - 1, t, None)

    prods, sched, ugate = _schedule(L, order, cfg)

    def main(step, carry):
        @pl.when(step + 1 < nsteps)
        def _():
            x_copy(step + 1).wait()

        @pl.when(step + 2 < nsteps)
        def _():
            x_copy(step + 2).start()

        zz = [lax.shift_right_logical(step, 12 + k) for k in range(14)]
        ctx.update(never=jnp.full((H, 128), zz[0], jnp.int32) != 0,
                   slot={-1: (step + 3) & 3, 0: step & 3, 1: (step + 1) & 3}, oslot=step & 1)
        wu = wexp.bitcast(jnp.uint32)
        subs = {}

        def wtile(l, k):
            return pltpu.bitcast(wu[l, k], bf16)

        def gather(al):
            return jnp.concatenate([subs[pi][j][g * 8:(g + 1) * 8, :] for pi, j, g in al], 0)

        ninner = 0
        for pi, (l, p, q) in enumerate(prods):
            ctx["z"] = zz[_ZQ[q]]
            qv = []
            for t in range(4):
                vs = [ld(f"a{p}", b, t) for b, _ in _MIDB[q]]
                qv.append(vs[0] if len(vs) == 1 else vs[0] - vs[1])
            k0 = tile0[p, q]
            if (p, q) in inner:
                a1 = qv[0] + qv[3]
                u = qv[1] + qv[2]
                if pi in ugate:
                    u = anc(u, gather(ugate[pi]))
                av = {1: a1, 3: qv[0] - qv[1], 5: qv[0] + qv[1], 4: qv[1] + qv[3],
                      7: qv[1] - qv[3], 2: u + a1, 6: u - a1}
                m = {r: jnp.dot(av[r].astype(bf16), wtile(l, k0 + r - 1),
                                preferred_element_type=f32) for r in _SO}
                subs[pi] = [m[r] for r in _SO]
                mq = _comb7(m, anc if ninner % 4 == 3 else None)
                ninner += 1
            else:
                a = jnp.concatenate(
                    [jnp.concatenate(qv[:2], 1), jnp.concatenate(qv[2:], 1)], 0).astype(bf16)
                wt = [wtile(l, k0 + t) for t in range(4)]
                wm = jnp.concatenate([jnp.concatenate(wt[:2], 1), jnp.concatenate(wt[2:], 1)], 0)
                mm = jnp.dot(a, wm, preferred_element_type=f32)
                subs[pi] = [mm[:, :128]]
                mq = [mm[:H, :128], mm[:H, 128:], mm[H:, :128], mm[H:, 128:]]
            if p in bp and q in bq:
                row = l * 64 + (bp.index(p) * 4 + bq.index(q)) * 4
                mq = [mq[t] + beta[row + t:row + t + 1, :] for t in range(4)]
            for t in range(4):
                v = mq[t]
                if p == 5:
                    v = v + ld("u3", q - 1, t)
                elif p == 1:
                    r3 = ld("u3", q - 1, t)
                    v = v + (((ld("u4", q - 1, t) + ld("u7", q - 1, t)) + (r3 + r3))
                             - ld("u5", q - 1, t))
                elif p == 2:
                    v = v + ld("u4", q - 1, t)
                elif p == 6:
                    v = v - ld("u7", q - 1, t)
                st(uname(p, l), q - 1, t, v)
            for j, jn, t, w, tl, al in sched.get(pi, []):
                a = gather(al)
                ctx.update(z=zz[8 + jn % 6], j=j, a2=a[H:] if len(al) > _NG else None)
                task[w](tl, t, a[:H])

        @pl.when(step >= 1)
        def _():
            top_copy(step - 1).wait()

        @pl.when(step >= 2)
        def _():
            bot_copy(step - 1).wait()

        top_copy(step).start()

        @pl.when(step >= 1)
        def _():
            bot_copy(step).start()

        return carry

    lax.fori_loop(0, nsteps, main, 0)

    ctx.update(z=0, slot={-1: (nsteps - 1) % 4}, j=-1, oslot=nsteps % 2)
    for w in ("o3", "o4", "o5"):
        for t in range(4):
            task[w](L - 1, t, None)
    bot_copy(nsteps).start()
    for c in range(8):
        fout(c).wait()
    top_copy(nsteps - 1).wait()
    bot_copy(nsteps - 1).wait()
    bot_copy(nsteps).wait()


def _build(**kw):
    cfg = dict(_CFG, **kw)

    def fn(x0, ws, bs):
        B, Dm = x0.shape
        L = ws.shape[0]
        assert Dm == 1024 and L == 6 and (B - _ROFF) % _TM == 0
        nsteps = (B - _ROFF) // _TM
        assert 4 <= nsteps < 4096
        ntiles = _products(cfg)[2]
        return pl.pallas_call(
            functools.partial(_kernel, L=L, nsteps=nsteps, cfg=cfg),
            in_specs=[pl.BlockSpec(memory_space=pl.ANY)] * 3,
            out_specs=pl.BlockSpec(memory_space=pl.ANY),
            out_shape=jax.ShapeDtypeStruct((B, Dm), x0.dtype),
            scratch_shapes=[
                pltpu.VMEM((L, Dm), bf16),
                pltpu.VMEM((4, _TM, Dm), bf16),
                pltpu.VMEM((2, _TM, Dm), bf16),
                pltpu.VMEM((L, 8, Dm, 128), bf16),
                pltpu.VMEM((L, ntiles, 128, 128), bf16),
                pltpu.VMEM((L * 64, 128), f32),
                pltpu.VMEM((16, _ROFF, 128), f32),
                pltpu.VMEM((16, _ROFF, 128), bf16),
                pltpu.VMEM((L * 8, 8, 128), f32),
                pltpu.SemaphoreType.DMA((4,)),
                pltpu.SemaphoreType.DMA((L,)),
                pltpu.SemaphoreType.DMA((2,)),
                pltpu.SemaphoreType.DMA((2,)),
                pltpu.SemaphoreType.DMA((9,)),
            ]
            + [pltpu.VMEM((1, 260 * 8, 128), f32)] * 2
            + [pltpu.VMEM((1, sz * 8, 128), f32) for _, sz in _bufkeys()],
            compiler_params=pltpu.CompilerParams(
                vmem_limit_bytes=126 * 1024 * 1024,
                disable_bounds_checks=True,
            ),
        )(x0, ws, bs)

    return fn


@jax.jit
def pallas_standalone__dcn_v2_cross__recsys_kernel(
    x0: jax.Array,
    ws: jax.Array,
    bs: jax.Array,
):
    return _build()(x0, ws, bs)
```

```python
import functools

import numpy as np
import jax
import jax.numpy as jnp
from jax import lax
import jax.experimental.pallas as pl
import jax.experimental.pallas.tpu as pltpu

f32 = jnp.float32
bf16 = jnp.bfloat16

_D = float(np.sqrt(3.0))
_TM = 384
_ROFF = 256
_H = _TM // 8
_NG = _H // 8
_BS = 9
_PH = (3, 5, 4, 7, 1, 2, 6)
_SO = (3, 5, 1, 4, 7, 2, 6)
_MIDB = {1: [(0, 1)], 2: [(1, 1)], 3: [(2, 1)], 5: [(3, 1)],
         4: [(0, 1), (2, -1)], 6: [(1, 1), (0, -1)], 7: [(3, 1), (0, -1)]}
_ZQ = {1: 0, 2: 0, 3: 0, 5: 0, 4: 1, 6: 2, 7: 3}
_CVEC = {1: [1, 0, 0, 1], 2: [0, 0, 1, -1], 3: [1, 1, 1, 1], 4: [1, 0, 1, 0],
         5: [-1, 1, 1, -1], 6: [0, 0, 1, 1], 7: [1, 0, -1, 0]}

_NAMES = ([(f"u{p}", 7) for p in (3, 4, 7, 5, 1, 2, 6)]
          + [(f"a{p}", 4) for p in (3, 4, 5, 7, 2, 6, 1)]
          + [(f"{s}{k}", 4) for s in ("fx", "H", "G", "U", "V") for k in range(2)]
          + [(f"x0{o}", 4) for o in range(4)]
          + [("u2x", 7), ("u6x", 7)] + [(f"{s}{k}", 4) for s in "HGUV" for k in (2, 3)])

_WIN = {"w1": (14, 35, 35), "w2": (35, 46, 48), "w3": (42, 49, 49), "w4": (49, 60, 62),
        "w5": (60, 74, 76), "e1": (0, 35, 35), "o1": (14, 35, 48), "e2": (35, 46, 48),
        "o2": (35, 48.5, 48), "e4": (49, 60, 62), "e5": (60, 74, 76), "o3": (49, 60, 85),
        "o4": (60, 170, 285), "o5": (170, 290, 300)}
_TCOST = {"w1": (26, 8), "w2": (34, 12), "w3": (16, 4), "w4": (42, 12), "w5": (35, 12),
          "o1": (31, 8), "o2": (31, 8), "o3": (16, 4), "o4": (39, 8), "o5": (27, 4),
          "e1": (14, 8), "e2": (22, 12), "e4": (22, 12), "e5": (30, 16)}
_CFG = dict(
    inner=tuple((p, q) for p in range(2, 8) for q in range(2, 8)) + ((1, 3), (1, 5), (1, 2), (1, 7)),
    kpos={3: 4, 5: 2, 4: 4, 7: 2, 1: 4, 2: 4, 6: 2},
    qo=(3, 5, 2, 4, 7, 6, 1),
    bp=(3, 4, 7, 1),
    bq=(5, 2, 1, 6),
    win=_WIN, ws=0.2, lat=135, sm=6, two=("w4", "w2"), gap=24, ulead=100,
    s1f=0.75, tail=(14, 17, 20, 23, 26),
)


def _kappa(bset):
    m = np.array([_CVEC[p] for p in bset], np.float64).T
    pats = [np.array([1, 0, _D, 0]), np.array([0, 1 / _D, 0, 1])]
    return [dict(zip(bset, np.linalg.solve(m, t))) for t in pats]


def _comb7(m, link=None):
    s = m[3] + m[5]
    e = (m[3] - m[5]) + m[1]
    return [(e + m[4]) + m[7], s if link is None else link(s, e),
            (((s + m[4]) - m[7]) + m[2]) + m[6], (e - m[2]) + m[6]]


def _fwd(x):
    a1 = x[0] + x[3]
    return [a1, ((x[1] + x[2]) + a1) * 0.5, x[0] - x[1], x[0] + x[1]]


def _bexp(b):
    b1 = b[0] + b[3]
    u = b[1] + b[2]
    return {1: b1, 2: b[0] - b[1], 3: b[1] - b[3], 4: u - b1, 5: b[1] + b[3], 6: b[0] + b[1],
            7: u + b1}


def _rowcol(o, i, t):
    r = (o // 2) * 4 + (i // 2) * 2 + t // 2
    c = (o % 2) * 4 + (i % 2) * 2 + t % 2
    e = (o // 2 - o % 2) + (i // 2 - i % 2) + (t // 2 - t % 2)
    return r, c, e


def _products(cfg):
    order = []
    for p in _PH:
        ks = [q for q in range(1, 8) if (p, q) not in cfg["inner"]]
        ls = [q for q in cfg["qo"] if (p, q) in cfg["inner"]]
        kp = cfg["kpos"][p]
        order += [(p, q) for q in ls[:kp] + ks + ls[kp:]]
    tile0 = {}
    n = 0
    for pq in order:
        tile0[pq] = n
        n += 7 if pq in cfg["inner"] else 4
    return order, tile0, n


def _qsize(k):
    return (k * _BS + 7) // 4 * 4


def _bufkeys():
    keys = []
    for n, k in _NAMES:
        if n[0] == "a":
            keys.append(((n, 0), 4 * _qsize(k)))
        else:
            keys += [((n, t), _qsize(k)) for t in range(4)]
    return keys


def _schedule(L, order, cfg):
    inner, win = cfg["inner"], cfg["win"]
    prods = [(l, p, q) for l in range(L) for (p, q) in order]
    npr = len(prods)
    free = [0, 0, 0, 0]
    anchors = []
    pstart = []
    for pi, (l, p, q) in enumerate(prods):
        pstart.append(min(free))
        if (p, q) in inner:
            for j in range(7):
                mx = int(np.argmin(free))
                anchors += [(free[mx] + g * 8, pi, j, g) for g in range(_NG)]
                free[mx] += _H
        else:
            anchors += [(max(free) + g * 8, pi, 0, g) for g in range(2 * _NG)]
            free = [f + 2 * _H for f in free]
    pstart.append(max(free))
    anchors.sort()
    times = np.array([a[0] for a in anchors])

    def tpos(x):
        i = int(np.floor(x))
        return pstart[i] + (x - i) * (pstart[min(i + 1, npr)] - pstart[i])

    npos = 4 * _NG
    load = np.zeros(pstart[-1] // 8 + 1)

    def spread(t0, t1, valu, stores):
        b0, b1 = max(int(t0 // 8), 0), max(int(t1 // 8), 1)
        load[b0:b1] += (valu / 4 + stores * cfg["ws"]) / max(int(t1 // 8) - int(t0 // 8), 1)

    for pi, (l, p, q) in enumerate(prods):
        big = (p, q) in inner
        t0, t1 = pstart[pi], pstart[pi + 1]
        spread(t0 - cfg["lat"], t1 - cfg["lat"],
               (len(_MIDB[q]) - 1 + (2.875 if big else 0.5)) * npos, 0)
        extra = {5: 1, 1: 5, 2: 1, 6: 1}.get(p, 0) + (p in cfg["bp"] and q in cfg["bq"])
        spread(t0, t1 + (_H // 2 if big else 0), ((2.75 if big else 1) + extra) * npos, npos)

    kern = np.hanning(cfg["sm"] + 2)[1:-1]
    kern /= kern.sum()
    jobs = [(w, l) for l in range(L - 1) for w in ("w1", "w2", "w3", "w4", "w5")]
    jobs += [(w, L - 1) for w in ("e1", "o1", "e2", "o2", "e4", "e5", "o3", "o4", "o5")]
    sched = {}
    for jn, (w, l) in sorted(enumerate(jobs), key=lambda e: win[e[1][0]][1] - win[e[1][0]][0]):
        i0, i1, last = (l * 49 + v for v in win[w])
        prev = i0 >= npr
        if prev:
            i0, i1, last = i0 - npr, i1 - npr, last - npr
        lo, hi = int(np.ceil(tpos(i0) / 8)), int(tpos(i1) // 8)
        picks = []
        for _ in range(npos):
            sm = np.convolve(load, kern, mode="same")
            bb = lo + int(np.argmin(sm[lo + 1:hi + 1]))
            picks.append(bb)
            spread(bb * 8, bb * 8 + 16 + (cfg["gap"] if w in cfg["two"] else 8), *_TCOST[w])
        picks.sort()
        slots = []
        for bb in picks:
            ai = int(np.searchsorted(times, bb * 8))
            while anchors[ai][1] < i0:
                ai += 1
            slots.append(anchors[ai][1:])
        if w in cfg["two"]:
            slots += [anchors[int(np.searchsorted(times, bb * 8 + cfg["gap"]))][1:] for bb in picks]
        for t in range(4):
            al = slots[t * _NG:(t + 1) * _NG] + slots[npos + t * _NG:npos + (t + 1) * _NG]
            at = max(a[0] for a in al)
            assert i0 <= at <= last, (w, l, t, at)
            sched.setdefault(at, []).append((-1 if prev else 0, jn, t, w, l, al))
    where = {}
    for at, v in sched.items():
        v.sort(key=lambda e: e[:3])
        for k, e in enumerate(v):
            where[e[3], e[4], e[2]] = (at, k)
    for a, b in (("w1", "w2"), ("w2", "w4"), ("w3", "w4"), ("w4", "w5"), ("e1", "e2"),
                 ("e4", "e5"), ("o3", "o4"), ("o4", "o5")):
        for l in (range(L - 1) if a[0] == "w" else (L - 1,)):
            assert all(where[a, l, t] < where[b, l, t] for t in range(4)), (a, b, l)

    ugate = {}
    for pi in range(49):
        if prods[pi][1:] in inner and pstart[pi] >= 200:
            al = []
            for g in range(_NG):
                gt = pstart[pi] + (g // 2) * 16 - cfg["ulead"]
                ai = int(np.searchsorted(times, gt, side="right")) - 1
                while anchors[ai][1] >= pi:
                    ai -= 1
                al.append(anchors[ai][1:])
            ugate[pi] = al
    return prods, sched, ugate


def _kernel(x_hbm, w_hbm, b_hbm, o_hbm, b_ref, ring, stage, wraw, wexp, beta, fx32, fxb, fb,
            xsem, wsem, tsem, bsem, fsem, *bufs, L, nsteps, cfg):
    H, HT = _H, _TM // 2
    inner, bp, bq = cfg["inner"], cfg["bp"], cfg["bq"]
    order, tile0, _ = _products(cfg)
    tmp = bufs[:2]
    buf = dict(zip([k for k, _ in _bufkeys()], bufs[2:]))
    skew = {n: k % 4 for k, (n, _) in enumerate(_NAMES)}
    ctx = {}

    def x_copy(i):
        return pltpu.make_async_copy(
            x_hbm.at[pl.ds(pl.multiple_of(_ROFF + i * _TM, 64), _TM)], ring.at[i & 3],
            xsem.at[i & 3])

    def w_copies(l):
        return [pltpu.make_async_copy(w_hbm.at[l, :, pl.ds(c * 128, 128)], wraw.at[l, c],
                                      wsem.at[l]) for c in range(8)]

    def top_copy(i):
        return pltpu.make_async_copy(
            stage.at[i & 1, pl.ds(HT, HT)],
            o_hbm.at[pl.ds(pl.multiple_of(_ROFF + i * _TM, 64), HT)], tsem.at[i & 1])

    def bot_copy(i):
        return pltpu.make_async_copy(
            stage.at[i & 1, pl.ds(0, HT)],
            o_hbm.at[pl.ds(pl.multiple_of(_ROFF + i * _TM - HT, 64), HT)], bsem.at[i & 1])

    def fin(c):
        return pltpu.make_async_copy(
            x_hbm.at[pl.ds(0, _ROFF), pl.ds(c * 128, 128)], fxb.at[c], fsem.at[c])

    def fout(c):
        return pltpu.make_async_copy(
            fxb.at[(L & 1) * 8 + c], o_hbm.at[pl.ds(0, _ROFF), pl.ds(c * 128, 128)], fsem.at[c])

    def loc(n, b, t):
        if n[0] == "a":
            return buf[n, 0], (t * _qsize(4) + (skew[n] + t) % 4 + b * _BS) * 8
        return buf[n, t], ((skew[n] + t) % 4 + b * _BS) * 8

    def ld(n, b, t):
        ref, o = loc(n, b, t)
        return ref[ctx["z"], o:o + H, :]

    def st(n, b, t, v):
        ref, o = loc(n, b, t)
        ref[0, o:o + H, :] = v

    def anc(v, a):
        return v if a is None else jnp.where(ctx["never"], a, v)

    def xin(j, o, i, t):
        r, c, _ = _rowcol(o, i, t)
        return ring[ctx["slot"][j], r * H:(r + 1) * H, c * 128:(c + 1) * 128].astype(f32)

    def sname(s, l):
        return f"{s}{l - L + 4 if l >= L - 2 else l % 2}"

    def uname(p, l):
        return f"u{p}x" if (l == L - 1 and p in (2, 6)) else f"u{p}"

    def upd(l, p, s, t, a):
        m = {q: ld(uname(p, l), q - 1, t) for q in range(1, 8)}
        m[3] = anc(m[3], a)
        y = _comb7(m)
        if l > 0:
            y = [y[i] + ld(sname(s, l - 1), i, t) for i in range(4)]
        for i in range(4):
            st(sname(s, l), i, t, y[i])
        return y

    def g22(l, t, a):
        v = upd(l, 6, "V", t, a)
        return [v[i] + (ld(sname("G", l), i, t) - ld(sname("U", l), i, t)) for i in range(4)]

    def g21(l, t, a):
        return [anc(ld(sname("U", l), i, t), a[i]) + ld(sname("V", l), i, t)
                + ld(sname("H", l), i, t) for i in range(4)]

    def gate(o, g, t):
        g = [anc(g[0], ctx["a2"])] + g[1:]
        return [ld(f"x0{o}", i, t) * g[i] for i in range(4)]

    def emit(o, g, t):
        for i in range(4):
            r, c, e = _rowcol(o, i, t)
            y = xin(ctx["j"], o, i, t) * g[i]
            if e:
                y = y * (_D ** -e)
            r0 = ctx["j"] * _TM + r * H + HT
            stage[ctx["oslot"], r0:r0 + H, c * 128:(c + 1) * 128] = y.astype(bf16)

    def fresh(o, t, a):
        xs = []
        for i in range(4):
            e = _rowcol(o, i, t)[2]
            v = xin(ctx["j"] + 1, o, i, t)
            if i == 0:
                v = anc(v, a)
            st(f"x0{o}", i, t, v)
            xs.append(v * (_D ** e) if e else v)
        return xs

    def f1(l, t, x):
        for i, v in enumerate(_fwd(x)):
            st(f"fx{l % 2}", i, t, v)

    def f2(l, t, x):
        for i, v in enumerate(_fwd(x)):
            w = ld(f"fx{l % 2}", i, t)
            st("a3", i, t, v - w)
            st("a5", i, t, v + w)

    def f4(l, t, x):
        for i, v in enumerate(_fwd(x)):
            w = ld(f"fx{l % 2}", i, t)
            st("a4", i, t, w + v)
            st("a7", i, t, w - v)

    def f5(l, t, x):
        for i, v in enumerate(_fwd(x)):
            u = ld(f"fx{l % 2}", i, t) + v
            a1 = ld("a3", i, t) + ld("a4", i, t)
            st("a1", i, t, a1)
            st("a2", i, t, u + a1)
            st("a6", i, t, u - a1)

    task = {
        "w1": lambda l, t, a: f1(l, t, gate(1, upd(l, 5, "H", t, a), t)),
        "w2": lambda l, t, a: f2(l, t, gate(0, upd(l, 1, "G", t, a), t)),
        "w3": lambda l, t, a: upd(l, 2, "U", t, a),
        "w4": lambda l, t, a: f4(l, t, gate(3, g22(l, t, a), t)),
        "w5": lambda l, t, a: f5(l, t, gate(2, g21(l, t, [a, None, None, None]), t)),
        "o1": lambda l, t, a: emit(1, upd(l, 5, "H", t, a), t),
        "o2": lambda l, t, a: emit(0, upd(l, 1, "G", t, a), t),
        "o3": lambda l, t, a: upd(l, 2, "U", t, a),
        "o4": lambda l, t, a: emit(3, g22(l, t, a), t),
        "o5": lambda l, t, a: emit(2, g21(l, t, [a] * 4), t),
        "e1": lambda l, t, a: f1(l, t, fresh(1, t, a)),
        "e2": lambda l, t, a: f2(l, t, fresh(0, t, a)),
        "e4": lambda l, t, a: f4(l, t, fresh(3, t, a)),
        "e5": lambda l, t, a: f5(l, t, fresh(2, t, a)),
    }

    b_copy = pltpu.make_async_copy(b_hbm, b_ref, fsem.at[8])
    b_copy.start()
    for c in range(8):
        fin(c).start()
    for cp in w_copies(0):
        cp.start()

    for n in ("u2x", "u6x", sname("U", L - 2), sname("V", L - 2), sname("G", L - 1),
              sname("H", L - 1)):
        for t in range(4):
            buf[n, t][...] = jnp.zeros(buf[n, t].shape, f32)
    ring[3, HT:, :] = jnp.zeros((HT, ring.shape[2]), bf16)

    b_copy.wait()
    kap, kaq = _kappa(bp), _kappa(bq)
    for l in range(L):
        bl = b_ref[l:l + 1, :].astype(f32)
        for c in range(8):
            fb[l * 8 + c, 0:1, :] = bl[:, c * 128:(c + 1) * 128]
        if l == 0:
            bl = bl + 1.0
        for pi, p in enumerate(bp):
            for qi, q in enumerate(bq):
                for c3 in range(2):
                    acc = None
                    for c1 in range(2):
                        for c2 in range(2):
                            k = float(kap[c1][p] * kaq[c2][q])
                            if abs(k) < 1e-12:
                                continue
                            c = c1 * 4 + c2 * 2 + c3
                            term = bl[:, c * 128:(c + 1) * 128] * k
                            acc = term if acc is None else acc + term
                    for r3 in range(2):
                        row = l * 64 + (pi * 4 + qi) * 4 + r3 * 2 + c3
                        beta[row:row + 1, :] = acc * (_D ** (r3 - c3))
    for c in range(8):
        fin(c).wait()
    for c in range(8):
        v = fxb[c].astype(f32)
        fx32[c] = v
        fx32[8 + c] = v

    def toff(p, i, t):
        return ((p - 1) * 37 + (i * 4 + t) * 2 + i) * 8

    def s1_units(l, g, dst):
        r0 = pl.multiple_of(g * 16, 16)

        def unit(i, t):
            blk = []
            for o in range(4):
                r, c, e = _rowcol(o, i, t)
                v = wraw[l, c, pl.ds(r * 128 + r0, 16), :].astype(f32)
                blk.append(v * (0.125 * _D ** e))
            ex = _bexp(blk)
            for p in _PH:
                dst[0, toff(p, i, t):toff(p, i, t) + 16, :] = ex[p]
            return [ex[7][:8]]

        return [(34, functools.partial(unit, i, t)) for i in range(4) for t in range(4)]

    def s2_units(l, g, src, zg):
        r0 = pl.multiple_of(g * 16, 16)

        def put(p, q, qs):
            f = (2.0 if p == 1 else 1.0) * (2 if q in (1, 2, 6) else 1)
            if (p, q) in inner:
                inn = _bexp([v * f for v in qs] if f != 1 else qs)
                tiles = [inn[1] + inn[1]] + [inn[r] for r in range(2, 8)]
            else:
                tiles = [v * (2 * f) for v in qs]
            for k, v in enumerate(tiles):
                wexp[l, tile0[p, q] + k, pl.ds(r0, 16), :] = v.astype(bf16)
            return tiles

        def unit(p, un, a=None):
            def tl(i):
                vs = [src[zg[1 + un], toff(p, i, t):toff(p, i, t) + 16, :] for t in range(4)]
                if a is not None and i == 1:
                    vs[1] = jnp.where(jnp.full((16, 128), zg[0], jnp.int32) != 0, a, vs[1])
                return vs

            if un == 0:
                x, y, qa, qb = tl(0), tl(1), 2, 6
            elif un == 1:
                x, y, qa, qb = tl(1), tl(3), 3, 5
            else:
                x = [u + v for u, v in zip(tl(1), tl(2))]
                y = [u + v for u, v in zip(tl(0), tl(3))]
                qa, qb = 4, 7
                put(p, 1, y)
            put(p, qa, [u - v for u, v in zip(x, y)])
            tb = put(p, qb, [u + v for u, v in zip(x, y)])
            if len(tb) == 4:
                return [v[:8] for v in tb]
            return [tb[-1][8:]]

        return [(((61, 82, 89) if p == 1 else (82, 66, 94))[un], functools.partial(unit, p, un))
                for p in _PH for un in range(3)]

    def half(l, g, ln, gn, src, dst, zg, tail):
        u2 = s2_units(l, g, src, zg)
        u1 = s1_units(ln, gn, dst)
        units = sorted([(k / len(u2), c, f) for k, (c, f) in enumerate(u2)]
                       + [((k + 0.5) / len(u1) * cfg["s1f"], c, f) for k, (c, f) in enumerate(u1)],
                       key=lambda e: e[0])
        late = [f for _, _, f in units[len(units) - len(tail):]]
        units = units[:len(units) - len(tail)]
        total = sum(c for _, c, _ in units)
        nsl = _ROFF // 16
        links = {}
        acc = 0
        for _, c, f in units:
            acc += c
            sl = min(int(np.ceil(acc / total * 2 * nsl)), 2 * nsl) - 1
            links.setdefault(sl, []).extend(f())
        fsrc = (l & 1) * 8
        fu = fxb.bitcast(jnp.uint32)
        never = jnp.full((8, 128), zg[0], jnp.int32) != 0
        cols = []
        for c in range(8):
            rows = []
            for r in range(nsl):
                v = fu[fsrc + c, r * 8:(r + 1) * 8, :]
                for a in links.get((c // 4) * nsl + r, [])[c % 4::4]:
                    v = jnp.where(never, pltpu.bitcast(a, jnp.uint32), v)
                rows.append(v)
            cols.append(pltpu.bitcast(jnp.concatenate(rows, 0), bf16))
        wg = pltpu.bitcast(wraw.bitcast(jnp.uint32)[l, g], bf16)
        y = jnp.dot(jnp.concatenate(cols, 1), wg, preferred_element_type=f32)
        xn = fx32[g] * (y + fb[l * 8 + g, 0:1, :]) + fx32[8 + g]
        fx32[8 + g] = xn
        fxb[8 - fsrc + g] = xn.astype(bf16)
        for r, f in zip(tail, late):
            f(y[r * 8:r * 8 + 16])

    for cp in w_copies(0):
        cp.wait()
    for cp in w_copies(1):
        cp.start()
    for _, f in s1_units(0, 0, tmp[0]):
        f()

    def pair(n, carry):
        l = lax.shift_right_logical(n, 2)
        g = (n & 3) * 2

        @pl.when(jnp.logical_and(g == 6, l + 1 < L))
        def _():
            for cp in w_copies(l + 1):
                cp.wait()

        @pl.when(jnp.logical_and(g == 6, l + 2 < L))
        def _():
            for cp in w_copies(l + 2):
                cp.start()

        @pl.when(n == 4 * L - 5)
        def _():
            x_copy(0).start()
            x_copy(1).start()

        zg = [lax.shift_right_logical(n, 12 + k) for k in range(8)]
        nn = jnp.minimum(2 * n + 2, 8 * L - 1)
        half(l, g, l, g + 1, tmp[0], tmp[1], zg[:4], ())
        half(l, g + 1, lax.shift_right_logical(nn, 3), nn & 7, tmp[1], tmp[0], zg[4:], cfg["tail"])
        return carry

    lax.fori_loop(0, 4 * L, pair, 0)
    for c in range(8):
        fout(c).start()
    x_copy(0).wait()
    ctx.update(z=0, slot={0: 0}, j=-1)
    for w in ("e1", "e2"):
        for t in range(4):
            task[w](L - 1, t, None)

    prods, sched, ugate = _schedule(L, order, cfg)

    def main(step, carry):
        @pl.when(step + 1 < nsteps)
        def _():
            x_copy(step + 1).wait()

        @pl.when(step >= 2)
        def _():
            top_copy(step - 2).wait()

        @pl.when(step >= 3)
        def _():
            bot_copy(step - 2).wait()

        @pl.when(step >= 1)
        def _():
            top_copy(step - 1).start()

        @pl.when(step >= 2)
        def _():
            bot_copy(step - 1).start()

        @pl.when(step + 2 < nsteps)
        def _():
            x_copy(step + 2).start()

        zz = [lax.shift_right_logical(step, 12 + k) for k in range(14)]
        ctx.update(never=jnp.full((H, 128), zz[0], jnp.int32) != 0,
                   slot={-1: (step + 3) & 3, 0: step & 3, 1: (step + 1) & 3}, oslot=step & 1)
        wu = wexp.bitcast(jnp.uint32)
        subs = {}

        def wtile(l, k):
            return pltpu.bitcast(wu[l, k], bf16)

        def gather(al):
            return jnp.concatenate([subs[pi][j][g * 8:(g + 1) * 8, :] for pi, j, g in al], 0)

        ninner = 0
        for pi, (l, p, q) in enumerate(prods):
            ctx["z"] = zz[_ZQ[q]]
            qv = []
            for t in range(4):
                vs = [ld(f"a{p}", b, t) for b, _ in _MIDB[q]]
                qv.append(vs[0] if len(vs) == 1 else vs[0] - vs[1])
            k0 = tile0[p, q]
            if (p, q) in inner:
                a1 = qv[0] + qv[3]
                u = qv[1] + qv[2]
                if pi in ugate:
                    u = anc(u, gather(ugate[pi]))
                av = {1: a1, 3: qv[0] - qv[1], 5: qv[0] + qv[1], 4: qv[1] + qv[3],
                      7: qv[1] - qv[3], 2: u + a1, 6: u - a1}
                m = {r: jnp.dot(av[r].astype(bf16), wtile(l, k0 + r - 1),
                                preferred_element_type=f32) for r in _SO}
                subs[pi] = [m[r] for r in _SO]
                mq = _comb7(m, anc if ninner % 4 == 3 else None)
                ninner += 1
            else:
                a = jnp.concatenate(
                    [jnp.concatenate(qv[:2], 1), jnp.concatenate(qv[2:], 1)], 0).astype(bf16)
                wt = [wtile(l, k0 + t) for t in range(4)]
                wm = jnp.concatenate([jnp.concatenate(wt[:2], 1), jnp.concatenate(wt[2:], 1)], 0)
                mm = jnp.dot(a, wm, preferred_element_type=f32)
                subs[pi] = [mm[:, :128]]
                mq = [mm[:H, :128], mm[:H, 128:], mm[H:, :128], mm[H:, 128:]]
            if p in bp and q in bq:
                row = l * 64 + (bp.index(p) * 4 + bq.index(q)) * 4
                mq = [mq[t] + beta[row + t:row + t + 1, :] for t in range(4)]
            for t in range(4):
                v = mq[t]
                if p == 5:
                    v = v + ld("u3", q - 1, t)
                elif p == 1:
                    r3 = ld("u3", q - 1, t)
                    v = v + (((ld("u4", q - 1, t) + ld("u7", q - 1, t)) + (r3 + r3))
                             - ld("u5", q - 1, t))
                elif p == 2:
                    v = v + ld("u4", q - 1, t)
                elif p == 6:
                    v = v - ld("u7", q - 1, t)
                st(uname(p, l), q - 1, t, v)
            for j, jn, t, w, tl, al in sched.get(pi, []):
                a = gather(al)
                ctx.update(z=zz[8 + jn % 6], j=j, a2=a[H:] if len(al) > _NG else None)
                task[w](tl, t, a[:H])

        return carry

    lax.fori_loop(0, nsteps, main, 0)

    top_copy(nsteps - 1).start()
    bot_copy(nsteps - 1).start()
    top_copy(nsteps - 2).wait()
    bot_copy(nsteps - 2).wait()
    ctx.update(z=0, slot={-1: (nsteps - 1) % 4}, j=-1, oslot=nsteps % 2)
    for w in ("o3", "o4", "o5"):
        for t in range(4):
            task[w](L - 1, t, None)
    bot_copy(nsteps).start()
    for c in range(8):
        fout(c).wait()
    top_copy(nsteps - 1).wait()
    bot_copy(nsteps - 1).wait()
    bot_copy(nsteps).wait()


def _build(**kw):
    cfg = dict(_CFG, **kw)

    def fn(x0, ws, bs):
        B, Dm = x0.shape
        L = ws.shape[0]
        assert Dm == 1024 and L == 6 and (B - _ROFF) % _TM == 0
        nsteps = (B - _ROFF) // _TM
        assert 4 <= nsteps < 4096
        ntiles = _products(cfg)[2]
        return pl.pallas_call(
            functools.partial(_kernel, L=L, nsteps=nsteps, cfg=cfg),
            in_specs=[pl.BlockSpec(memory_space=pl.ANY)] * 3,
            out_specs=pl.BlockSpec(memory_space=pl.ANY),
            out_shape=jax.ShapeDtypeStruct((B, Dm), x0.dtype),
            scratch_shapes=[
                pltpu.VMEM((L, Dm), bf16),
                pltpu.VMEM((4, _TM, Dm), bf16),
                pltpu.VMEM((2, _TM, Dm), bf16),
                pltpu.VMEM((L, 8, Dm, 128), bf16),
                pltpu.VMEM((L, ntiles, 128, 128), bf16),
                pltpu.VMEM((L * 64, 128), f32),
                pltpu.VMEM((16, _ROFF, 128), f32),
                pltpu.VMEM((16, _ROFF, 128), bf16),
                pltpu.VMEM((L * 8, 8, 128), f32),
                pltpu.SemaphoreType.DMA((4,)),
                pltpu.SemaphoreType.DMA((L,)),
                pltpu.SemaphoreType.DMA((2,)),
                pltpu.SemaphoreType.DMA((2,)),
                pltpu.SemaphoreType.DMA((9,)),
            ]
            + [pltpu.VMEM((1, 260 * 8, 128), f32)] * 2
            + [pltpu.VMEM((1, sz * 8, 128), f32) for _, sz in _bufkeys()],
            compiler_params=pltpu.CompilerParams(
                vmem_limit_bytes=126 * 1024 * 1024,
                disable_bounds_checks=True,
            ),
        )(x0, ws, bs)

    return fn


@jax.jit
def pallas_standalone__dcn_v2_cross__recsys_kernel(
    x0: jax.Array,
    ws: jax.Array,
    bs: jax.Array,
):
    return _build()(x0, ws, bs)
```

```python
import functools

import numpy as np
import jax
import jax.numpy as jnp
from jax import lax
import jax.experimental.pallas as pl
import jax.experimental.pallas.tpu as pltpu

f32 = jnp.float32
bf16 = jnp.bfloat16

_D = float(np.sqrt(3.0))
_TM = 384
_ROFF = 256
_H = _TM // 8
_NG = _H // 8
_BS = 9
_PH = (3, 5, 4, 7, 1, 2, 6)
_SO = (3, 5, 1, 4, 7, 2, 6)
_MIDB = {1: [(0, 1)], 2: [(1, 1)], 3: [(2, 1)], 5: [(3, 1)],
         4: [(0, 1), (2, -1)], 6: [(1, 1), (0, -1)], 7: [(3, 1), (0, -1)]}
_ZQ = {1: 0, 2: 0, 3: 0, 5: 0, 4: 1, 6: 2, 7: 3}
_CVEC = {1: [1, 0, 0, 1], 2: [0, 0, 1, -1], 3: [1, 1, 1, 1], 4: [1, 0, 1, 0],
         5: [-1, 1, 1, -1], 6: [0, 0, 1, 1], 7: [1, 0, -1, 0]}

_NAMES = ([(f"u{p}", 7) for p in (3, 4, 7, 5, 1, 2, 6)]
          + [(f"a{p}", 4) for p in (3, 4, 5, 7, 2, 6, 1)]
          + [(f"{s}{k}", 4) for s in ("fx", "H", "G", "U", "V") for k in range(2)]
          + [(f"x0{o}", 4) for o in range(4)]
          + [("u2x", 7), ("u6x", 7)] + [(f"{s}{k}", 4) for s in "HGUV" for k in (2, 3)])

_WIN = {"w1": (14, 35, 35), "w2": (35, 46, 48), "w3": (42, 49, 49), "w4": (49, 60, 62),
        "w5": (60, 74, 76), "e1": (0, 35, 35), "o1": (14, 35, 48), "e2": (35, 46, 48),
        "o2": (35, 48.5, 48), "e4": (49, 60, 62), "e5": (60, 74, 76), "o3": (49, 60, 85),
        "o4": (60, 170, 285), "o5": (170, 290, 299)}
_BOT_DONE = 250
_TCOST = {"w1": (26, 8), "w2": (34, 12), "w3": (16, 4), "w4": (42, 12), "w5": (35, 12),
          "o1": (31, 8), "o2": (31, 8), "o3": (16, 4), "o4": (39, 8), "o5": (27, 4),
          "e1": (14, 8), "e2": (22, 12), "e4": (22, 12), "e5": (30, 16)}
_CFG = dict(
    inner=tuple((p, q) for p in range(2, 8) for q in range(2, 8)) + ((1, 3), (1, 5), (1, 2), (1, 7)),
    kpos={3: 4, 5: 2, 4: 4, 7: 2, 1: 4, 2: 4, 6: 2},
    qo=(3, 5, 2, 4, 7, 6, 1),
    bp=(3, 4, 7, 1),
    bq=(5, 2, 1, 6),
    win=_WIN, ws=0.2, lat=135, sm=6, two=("w4", "w2"), gap=24, ulead=100,
    s1f=0.75, tail=(14, 17, 20, 23, 26),
)


def _kappa(bset):
    m = np.array([_CVEC[p] for p in bset], np.float64).T
    pats = [np.array([1, 0, _D, 0]), np.array([0, 1 / _D, 0, 1])]
    return [dict(zip(bset, np.linalg.solve(m, t))) for t in pats]


def _comb7(m, link=None):
    s = m[3] + m[5]
    e = (m[3] - m[5]) + m[1]
    return [(e + m[4]) + m[7], s if link is None else link(s, e),
            (((s + m[4]) - m[7]) + m[2]) + m[6], (e - m[2]) + m[6]]


def _fwd(x):
    a1 = x[0] + x[3]
    return [a1, ((x[1] + x[2]) + a1) * 0.5, x[0] - x[1], x[0] + x[1]]


def _bexp(b):
    b1 = b[0] + b[3]
    u = b[1] + b[2]
    return {1: b1, 2: b[0] - b[1], 3: b[1] - b[3], 4: u - b1, 5: b[1] + b[3], 6: b[0] + b[1],
            7: u + b1}


def _rowcol(o, i, t):
    r = (o // 2) * 4 + (i // 2) * 2 + t // 2
    c = (o % 2) * 4 + (i % 2) * 2 + t % 2
    e = (o // 2 - o % 2) + (i // 2 - i % 2) + (t // 2 - t % 2)
    return r, c, e


def _products(cfg):
    order = []
    for p in _PH:
        ks = [q for q in range(1, 8) if (p, q) not in cfg["inner"]]
        ls = [q for q in cfg["qo"] if (p, q) in cfg["inner"]]
        kp = cfg["kpos"][p]
        order += [(p, q) for q in ls[:kp] + ks + ls[kp:]]
    tile0 = {}
    n = 0
    for pq in order:
        tile0[pq] = n
        n += 7 if pq in cfg["inner"] else 4
    return order, tile0, n


def _qsize(k):
    return (k * _BS + 7) // 4 * 4


def _bufkeys():
    keys = []
    for n, k in _NAMES:
        if n[0] == "a":
            keys.append(((n, 0), 4 * _qsize(k)))
        else:
            keys += [((n, t), _qsize(k)) for t in range(4)]
    return keys


def _schedule(L, order, cfg):
    inner, win = cfg["inner"], cfg["win"]
    prods = [(l, p, q) for l in range(L) for (p, q) in order]
    npr = len(prods)
    free = [0, 0, 0, 0]
    anchors = []
    pstart = []
    for pi, (l, p, q) in enumerate(prods):
        pstart.append(min(free))
        if (p, q) in inner:
            for j in range(7):
                mx = int(np.argmin(free))
                anchors += [(free[mx] + g * 8, pi, j, g) for g in range(_NG)]
                free[mx] += _H
        else:
            anchors += [(max(free) + g * 8, pi, 0, g) for g in range(2 * _NG)]
            free = [f + 2 * _H for f in free]
    pstart.append(max(free))
    anchors.sort()
    times = np.array([a[0] for a in anchors])

    def tpos(x):
        i = int(np.floor(x))
        return pstart[i] + (x - i) * (pstart[min(i + 1, npr)] - pstart[i])

    npos = 4 * _NG
    load = np.zeros(pstart[-1] // 8 + 1)

    def spread(t0, t1, valu, stores):
        b0, b1 = max(int(t0 // 8), 0), max(int(t1 // 8), 1)
        load[b0:b1] += (valu / 4 + stores * cfg["ws"]) / max(int(t1 // 8) - int(t0 // 8), 1)

    for pi, (l, p, q) in enumerate(prods):
        big = (p, q) in inner
        t0, t1 = pstart[pi], pstart[pi + 1]
        spread(t0 - cfg["lat"], t1 - cfg["lat"],
               (len(_MIDB[q]) - 1 + (2.875 if big else 0.5)) * npos, 0)
        extra = {5: 1, 1: 5, 2: 1, 6: 1}.get(p, 0) + (p in cfg["bp"] and q in cfg["bq"])
        spread(t0, t1 + (_H // 2 if big else 0), ((2.75 if big else 1) + extra) * npos, npos)

    kern = np.hanning(cfg["sm"] + 2)[1:-1]
    kern /= kern.sum()
    jobs = [(w, l) for l in range(L - 1) for w in ("w1", "w2", "w3", "w4", "w5")]
    jobs += [(w, L - 1) for w in ("e1", "o1", "e2", "o2", "e4", "e5", "o3", "o4", "o5")]
    sched = {}
    for jn, (w, l) in sorted(enumerate(jobs), key=lambda e: win[e[1][0]][1] - win[e[1][0]][0]):
        i0, i1, last = (l * 49 + v for v in win[w])
        prev = i0 >= npr
        if prev:
            i0, i1, last = i0 - npr, i1 - npr, last - npr
        lo, hi = int(np.ceil(tpos(i0) / 8)), int(tpos(i1) // 8)
        picks = []
        for _ in range(npos):
            sm = np.round(np.convolve(load, kern, mode="same"), 9)
            bb = lo + int(np.argmin(sm[lo + 1:hi + 1]))
            picks.append(bb)
            spread(bb * 8, bb * 8 + 16 + (cfg["gap"] if w in cfg["two"] else 8), *_TCOST[w])
        picks.sort()
        slots = []
        for bb in picks:
            ai = int(np.searchsorted(times, bb * 8))
            while anchors[ai][1] < i0:
                ai += 1
            slots.append(anchors[ai][1:])
        if w in cfg["two"]:
            slots += [anchors[int(np.searchsorted(times, bb * 8 + cfg["gap"]))][1:] for bb in picks]
        for t in range(4):
            al = slots[t * _NG:(t + 1) * _NG] + slots[npos + t * _NG:npos + (t + 1) * _NG]
            at = max(a[0] for a in al)
            assert i0 <= at <= last, (w, l, t, at)
            sched.setdefault(at, []).append((-1 if prev else 0, jn, t, w, l, al))
    where = {}
    for at, v in sched.items():
        v.sort(key=lambda e: e[:3])
        for k, e in enumerate(v):
            where[e[3], e[4], e[2]] = (at, k)
    for a, b in (("w1", "w2"), ("w2", "w4"), ("w3", "w4"), ("w4", "w5"), ("e1", "e2"),
                 ("e4", "e5"), ("o3", "o4"), ("o4", "o5")):
        for l in (range(L - 1) if a[0] == "w" else (L - 1,)):
            assert all(where[a, l, t] < where[b, l, t] for t in range(4)), (a, b, l)

    ugate = {}
    for pi in range(49):
        if prods[pi][1:] in inner and pstart[pi] >= 200:
            al = []
            for g in range(_NG):
                gt = pstart[pi] + (g // 2) * 16 - cfg["ulead"]
                ai = int(np.searchsorted(times, gt, side="right")) - 1
                while anchors[ai][1] >= pi:
                    ai -= 1
                al.append(anchors[ai][1:])
            ugate[pi] = al
    return prods, sched, ugate


def _kernel(x_hbm, w_hbm, b_hbm, o_hbm, b_ref, ring, stage, wraw, wexp, beta, fx32, fxb, fb,
            xsem, wsem, tsem, bsem, fsem, *bufs, L, nsteps, cfg):
    H, HT = _H, _TM // 2
    inner, bp, bq = cfg["inner"], cfg["bp"], cfg["bq"]
    order, tile0, _ = _products(cfg)
    tmp = bufs[:2]
    buf = dict(zip([k for k, _ in _bufkeys()], bufs[2:]))
    skew = {n: k % 4 for k, (n, _) in enumerate(_NAMES)}
    ctx = {}

    def x_copy(i):
        return pltpu.make_async_copy(
            x_hbm.at[pl.ds(pl.multiple_of(_ROFF + i * _TM, 64), _TM)], ring.at[i & 3],
            xsem.at[i & 3])

    def w_copies(l, cols=range(8)):
        return [pltpu.make_async_copy(w_hbm.at[l, :, pl.ds(c * 128, 128)], wraw.at[l, c],
                                      wsem.at[l]) for c in cols]

    def top_copy(i):
        return pltpu.make_async_copy(
            stage.at[i & 1, pl.ds(HT, HT)],
            o_hbm.at[pl.ds(pl.multiple_of(_ROFF + i * _TM, 64), HT)], tsem.at[i & 1])

    def bot_copy(i):
        return pltpu.make_async_copy(
            stage.at[i & 1, pl.ds(0, HT)],
            o_hbm.at[pl.ds(pl.multiple_of(_ROFF + i * _TM - HT, 64), HT)], bsem.at[i & 1])

    def fin(c):
        return pltpu.make_async_copy(
            x_hbm.at[pl.ds(0, _ROFF), pl.ds(c * 128, 128)], fxb.at[c], fsem.at[c])

    def fout(c):
        return pltpu.make_async_copy(
            fxb.at[(L & 1) * 8 + c], o_hbm.at[pl.ds(0, _ROFF), pl.ds(c * 128, 128)], fsem.at[c])

    def loc(n, b, t):
        if n[0] == "a":
            return buf[n, 0], (t * _qsize(4) + (skew[n] + t) % 4 + b * _BS) * 8
        return buf[n, t], ((skew[n] + t) % 4 + b * _BS) * 8

    def ld(n, b, t):
        ref, o = loc(n, b, t)
        return ref[ctx["z"], o:o + H, :]

    def st(n, b, t, v):
        ref, o = loc(n, b, t)
        ref[0, o:o + H, :] = v

    def anc(v, a):
        return v if a is None else jnp.where(ctx["never"], a, v)

    def xin(j, o, i, t):
        r, c, _ = _rowcol(o, i, t)
        return ring[ctx["slot"][j], r * H:(r + 1) * H, c * 128:(c + 1) * 128].astype(f32)

    def sname(s, l):
        return f"{s}{l - L + 4 if l >= L - 2 else l % 2}"

    def uname(p, l):
        return f"u{p}x" if (l == L - 1 and p in (2, 6)) else f"u{p}"

    def upd(l, p, s, t, a):
        m = {q: ld(uname(p, l), q - 1, t) for q in range(1, 8)}
        m[3] = anc(m[3], a)
        y = _comb7(m)
        if l > 0:
            y = [y[i] + ld(sname(s, l - 1), i, t) for i in range(4)]
        for i in range(4):
            st(sname(s, l), i, t, y[i])
        return y

    def g22(l, t, a):
        v = upd(l, 6, "V", t, a)
        return [v[i] + (ld(sname("G", l), i, t) - ld(sname("U", l), i, t)) for i in range(4)]

    def g21(l, t, a):
        return [anc(ld(sname("U", l), i, t), a[i]) + ld(sname("V", l), i, t)
                + ld(sname("H", l), i, t) for i in range(4)]

    def gate(o, g, t):
        g = [anc(g[0], ctx["a2"])] + g[1:]
        return [ld(f"x0{o}", i, t) * g[i] for i in range(4)]

    def emit(o, g, t):
        for i in range(4):
            r, c, e = _rowcol(o, i, t)
            y = xin(ctx["j"], o, i, t) * g[i]
            if e:
                y = y * (_D ** -e)
            r0 = ctx["j"] * _TM + r * H + HT
            stage[ctx["oslot"], r0:r0 + H, c * 128:(c + 1) * 128] = y.astype(bf16)

    def fresh(o, t, a):
        xs = []
        for i in range(4):
            e = _rowcol(o, i, t)[2]
            v = xin(ctx["j"] + 1, o, i, t)
            if i == 0:
                v = anc(v, a)
            st(f"x0{o}", i, t, v)
            xs.append(v * (_D ** e) if e else v)
        return xs

    def f1(l, t, x):
        for i, v in enumerate(_fwd(x)):
            st(f"fx{l % 2}", i, t, v)

    def f2(l, t, x):
        for i, v in enumerate(_fwd(x)):
            w = ld(f"fx{l % 2}", i, t)
            st("a3", i, t, v - w)
            st("a5", i, t, v + w)

    def f4(l, t, x):
        for i, v in enumerate(_fwd(x)):
            w = ld(f"fx{l % 2}", i, t)
            st("a4", i, t, w + v)
            st("a7", i, t, w - v)

    def f5(l, t, x):
        for i, v in enumerate(_fwd(x)):
            u = ld(f"fx{l % 2}", i, t) + v
            a1 = ld("a3", i, t) + ld("a4", i, t)
            st("a1", i, t, a1)
            st("a2", i, t, u + a1)
            st("a6", i, t, u - a1)

    task = {
        "w1": lambda l, t, a: f1(l, t, gate(1, upd(l, 5, "H", t, a), t)),
        "w2": lambda l, t, a: f2(l, t, gate(0, upd(l, 1, "G", t, a), t)),
        "w3": lambda l, t, a: upd(l, 2, "U", t, a),
        "w4": lambda l, t, a: f4(l, t, gate(3, g22(l, t, a), t)),
        "w5": lambda l, t, a: f5(l, t, gate(2, g21(l, t, [a, None, None, None]), t)),
        "o1": lambda l, t, a: emit(1, upd(l, 5, "H", t, a), t),
        "o2": lambda l, t, a: emit(0, upd(l, 1, "G", t, a), t),
        "o3": lambda l, t, a: upd(l, 2, "U", t, a),
        "o4": lambda l, t, a: emit(3, g22(l, t, a), t),
        "o5": lambda l, t, a: emit(2, g21(l, t, [a] * 4), t),
        "e1": lambda l, t, a: f1(l, t, fresh(1, t, a)),
        "e2": lambda l, t, a: f2(l, t, fresh(0, t, a)),
        "e4": lambda l, t, a: f4(l, t, fresh(3, t, a)),
        "e5": lambda l, t, a: f5(l, t, fresh(2, t, a)),
    }

    b_copy = pltpu.make_async_copy(b_hbm, b_ref, fsem.at[8])
    b_copy.start()
    for c in range(8):
        fin(c).start()
    for cp in w_copies(0):
        cp.start()

    for n in ("u2x", "u6x", sname("U", L - 2), sname("V", L - 2), sname("G", L - 1),
              sname("H", L - 1)):
        for t in range(4):
            buf[n, t][...] = jnp.zeros(buf[n, t].shape, f32)
    ring[3, HT:, :] = jnp.zeros((HT, ring.shape[2]), bf16)
    fx32[8:16] = jnp.ones((8, _ROFF, 128), f32)

    b_copy.wait()
    kap, kaq = _kappa(bp), _kappa(bq)
    for l in range(L):
        bl = b_ref[l:l + 1, :].astype(f32)
        for c in range(8):
            fb[l * 8 + c, 0:1, :] = bl[:, c * 128:(c + 1) * 128]
        if l == 0:
            bl = bl + 1.0
        for pi, p in enumerate(bp):
            for qi, q in enumerate(bq):
                for c3 in range(2):
                    acc = None
                    for c1 in range(2):
                        for c2 in range(2):
                            k = float(kap[c1][p] * kaq[c2][q])
                            if abs(k) < 1e-12:
                                continue
                            c = c1 * 4 + c2 * 2 + c3
                            term = bl[:, c * 128:(c + 1) * 128] * k
                            acc = term if acc is None else acc + term
                    for r3 in range(2):
                        row = l * 64 + (pi * 4 + qi) * 4 + r3 * 2 + c3
                        beta[row:row + 1, :] = acc * (_D ** (r3 - c3))
    for c in range(8):
        fin(c).wait()
    for cp in w_copies(1, range(1)):
        cp.start()
    for c in range(8):
        fx32[c] = fxb[c].astype(f32)

    def toff(p, i, t):
        return ((p - 1) * 37 + (i * 4 + t) * 2 + i) * 8

    def s1_units(l, g, dst):
        r0 = pl.multiple_of(g * 16, 16)

        def unit(i, t):
            blk = []
            for o in range(4):
                r, c, e = _rowcol(o, i, t)
                v = wraw[l, c, pl.ds(r * 128 + r0, 16), :].astype(f32)
                blk.append(v * (0.125 * _D ** e))
            ex = _bexp(blk)
            for p in _PH:
                dst[0, toff(p, i, t):toff(p, i, t) + 16, :] = ex[p]
            return [ex[7][:8]]

        return [(34, functools.partial(unit, i, t)) for i in range(4) for t in range(4)]

    def s2_units(l, g, src, zg):
        r0 = pl.multiple_of(g * 16, 16)

        def put(p, q, qs):
            f = (2.0 if p == 1 else 1.0) * (2 if q in (1, 2, 6) else 1)
            if (p, q) in inner:
                inn = _bexp([v * f for v in qs] if f != 1 else qs)
                tiles = [inn[1] + inn[1]] + [inn[r] for r in range(2, 8)]
            else:
                tiles = [v * (2 * f) for v in qs]
            for k, v in enumerate(tiles):
                wexp[l, tile0[p, q] + k, pl.ds(r0, 16), :] = v.astype(bf16)
            return tiles

        def unit(p, un, a=None):
            def tl(i):
                vs = [src[zg[1 + un], toff(p, i, t):toff(p, i, t) + 16, :] for t in range(4)]
                if a is not None and i == 1:
                    vs[1] = jnp.where(jnp.full((16, 128), zg[0], jnp.int32) != 0, a, vs[1])
                return vs

            if un == 0:
                x, y, qa, qb = tl(0), tl(1), 2, 6
            elif un == 1:
                x, y, qa, qb = tl(1), tl(3), 3, 5
            else:
                x = [u + v for u, v in zip(tl(1), tl(2))]
                y = [u + v for u, v in zip(tl(0), tl(3))]
                qa, qb = 4, 7
                put(p, 1, y)
            put(p, qa, [u - v for u, v in zip(x, y)])
            tb = put(p, qb, [u + v for u, v in zip(x, y)])
            if len(tb) == 4:
                return [v[:8] for v in tb]
            return [tb[-1][8:]]

        return [(((61, 82, 89) if p == 1 else (82, 66, 94))[un], functools.partial(unit, p, un))
                for p in _PH for un in range(3)]

    def half(l, g, ln, gn, src, dst, zg, tail):
        u2 = s2_units(l, g, src, zg)
        u1 = s1_units(ln, gn, dst)
        units = sorted([(k / len(u2), c, f) for k, (c, f) in enumerate(u2)]
                       + [((k + 0.5) / len(u1) * cfg["s1f"], c, f) for k, (c, f) in enumerate(u1)],
                       key=lambda e: e[0])
        late = [f for _, _, f in units[len(units) - len(tail):]]
        units = units[:len(units) - len(tail)]
        total = sum(c for _, c, _ in units)
        nsl = _ROFF // 16
        links = {}
        acc = 0
        for _, c, f in units:
            acc += c
            sl = min(int(np.ceil(acc / total * 2 * nsl)), 2 * nsl) - 1
            links.setdefault(sl, []).extend(f())
        fsrc = (l & 1) * 8
        fu = fxb.bitcast(jnp.uint32)
        never = jnp.full((8, 128), zg[0], jnp.int32) != 0
        cols = []
        for c in range(8):
            rows = []
            for r in range(nsl):
                v = fu[fsrc + c, r * 8:(r + 1) * 8, :]
                for a in links.get((c // 4) * nsl + r, [])[c % 4::4]:
                    v = jnp.where(never, pltpu.bitcast(a, jnp.uint32), v)
                rows.append(v)
            cols.append(pltpu.bitcast(jnp.concatenate(rows, 0), bf16))
        wg = pltpu.bitcast(wraw.bitcast(jnp.uint32)[l, g], bf16)
        y = jnp.dot(jnp.concatenate(cols, 1), wg, preferred_element_type=f32)
        gn = (y + fb[l * 8 + g, 0:1, :]) + fx32[8 + g]
        fx32[8 + g] = gn
        fxb[8 - fsrc + g] = (fx32[g] * gn).astype(bf16)
        for r, f in zip(tail, late):
            f(y[r * 8:r * 8 + 16])

    for cp in w_copies(0):
        cp.wait()
    for cp in w_copies(1, range(1, 8)):
        cp.start()
    for _, f in s1_units(0, 0, tmp[0]):
        f()

    def pair(n, carry):
        l = lax.shift_right_logical(n, 2)
        g = (n & 3) * 2

        @pl.when(jnp.logical_and(g == 6, l + 1 < L))
        def _():
            for cp in w_copies(l + 1):
                cp.wait()

        @pl.when(jnp.logical_and(g == 4, l + 2 < L))
        def _():
            for cp in w_copies(l + 2):
                cp.start()

        @pl.when(n == 4 * L - 5)
        def _():
            x_copy(0).start()
            x_copy(1).start()

        zg = [lax.shift_right_logical(n, 12 + k) for k in range(8)]
        nn = jnp.minimum(2 * n + 2, 8 * L - 1)
        half(l, g, l, g + 1, tmp[0], tmp[1], zg[:4], ())
        half(l, g + 1, lax.shift_right_logical(nn, 3), nn & 7, tmp[1], tmp[0], zg[4:], cfg["tail"])
        return carry

    lax.fori_loop(0, 4 * L, pair, 0)
    for c in range(8):
        fout(c).start()
    x_copy(0).wait()
    ctx.update(z=0, slot={0: 0}, j=-1)
    for w in ("e1", "e2"):
        for t in range(4):
            task[w](L - 1, t, None)

    prods, sched, ugate = _schedule(L, order, cfg)

    def main(step, carry):
        @pl.when(step + 1 < nsteps)
        def _():
            x_copy(step + 1).wait()

        @pl.when(step >= 2)
        def _():
            top_copy(step - 2).wait()

        @pl.when(step >= 3)
        def _():
            bot_copy(step - 2).wait()

        @pl.when(step >= 1)
        def _():
            top_copy(step - 1).start()

        @pl.when(step + 2 < nsteps)
        def _():
            x_copy(step + 2).start()

        zz = [lax.shift_right_logical(step, 12 + k) for k in range(14)]
        ctx.update(never=jnp.full((H, 128), zz[0], jnp.int32) != 0,
                   slot={-1: (step + 3) & 3, 0: step & 3, 1: (step + 1) & 3}, oslot=step & 1)
        wu = wexp.bitcast(jnp.uint32)
        subs = {}

        def wtile(l, k):
            return pltpu.bitcast(wu[l, k], bf16)

        def gather(al):
            return jnp.concatenate([subs[pi][j][g * 8:(g + 1) * 8, :] for pi, j, g in al], 0)

        ninner = 0
        for pi, (l, p, q) in enumerate(prods):
            ctx["z"] = zz[_ZQ[q]]
            qv = []
            for t in range(4):
                vs = [ld(f"a{p}", b, t) for b, _ in _MIDB[q]]
                qv.append(vs[0] if len(vs) == 1 else vs[0] - vs[1])
            k0 = tile0[p, q]
            if (p, q) in inner:
                a1 = qv[0] + qv[3]
                u = qv[1] + qv[2]
                if pi in ugate:
                    u = anc(u, gather(ugate[pi]))
                av = {1: a1, 3: qv[0] - qv[1], 5: qv[0] + qv[1], 4: qv[1] + qv[3],
                      7: qv[1] - qv[3], 2: u + a1, 6: u - a1}
                m = {r: jnp.dot(av[r].astype(bf16), wtile(l, k0 + r - 1),
                                preferred_element_type=f32) for r in _SO}
                subs[pi] = [m[r] for r in _SO]
                mq = _comb7(m, anc if ninner % 4 == 3 else None)
                ninner += 1
            else:
                a = jnp.concatenate(
                    [jnp.concatenate(qv[:2], 1), jnp.concatenate(qv[2:], 1)], 0).astype(bf16)
                wt = [wtile(l, k0 + t) for t in range(4)]
                wm = jnp.concatenate([jnp.concatenate(wt[:2], 1), jnp.concatenate(wt[2:], 1)], 0)
                mm = jnp.dot(a, wm, preferred_element_type=f32)
                subs[pi] = [mm[:, :128]]
                mq = [mm[:H, :128], mm[:H, 128:], mm[H:, :128], mm[H:, 128:]]
            if p in bp and q in bq:
                row = l * 64 + (bp.index(p) * 4 + bq.index(q)) * 4
                mq = [mq[t] + beta[row + t:row + t + 1, :] for t in range(4)]
            for t in range(4):
                v = mq[t]
                if p == 5:
                    v = v + ld("u3", q - 1, t)
                elif p == 1:
                    r3 = ld("u3", q - 1, t)
                    v = v + (((ld("u4", q - 1, t) + ld("u7", q - 1, t)) + (r3 + r3))
                             - ld("u5", q - 1, t))
                elif p == 2:
                    v = v + ld("u4", q - 1, t)
                elif p == 6:
                    v = v - ld("u7", q - 1, t)
                st(uname(p, l), q - 1, t, v)
            for j, jn, t, w, tl, al in sched.get(pi, []):
                a = gather(al)
                ctx.update(z=zz[8 + jn % 6], j=j, a2=a[H:] if len(al) > _NG else None)
                task[w](tl, t, a[:H])
            if pi == _BOT_DONE:
                @pl.when(step >= 1)
                def _():
                    bot_copy(step).start()

        return carry

    lax.fori_loop(0, nsteps, main, 0)

    top_copy(nsteps - 1).start()
    top_copy(nsteps - 2).wait()
    bot_copy(nsteps - 2).wait()
    ctx.update(z=0, slot={-1: (nsteps - 1) % 4}, j=-1, oslot=nsteps % 2)
    for w in ("o3", "o4", "o5"):
        for t in range(4):
            task[w](L - 1, t, None)
    bot_copy(nsteps).start()
    for c in range(8):
        fout(c).wait()
    top_copy(nsteps - 1).wait()
    bot_copy(nsteps - 1).wait()
    bot_copy(nsteps).wait()


def _build(**kw):
    cfg = dict(_CFG, **kw)

    def fn(x0, ws, bs):
        B, Dm = x0.shape
        L = ws.shape[0]
        assert Dm == 1024 and L == 6 and (B - _ROFF) % _TM == 0
        nsteps = (B - _ROFF) // _TM
        assert 4 <= nsteps < 4096
        ntiles = _products(cfg)[2]
        return pl.pallas_call(
            functools.partial(_kernel, L=L, nsteps=nsteps, cfg=cfg),
            in_specs=[pl.BlockSpec(memory_space=pl.ANY)] * 3,
            out_specs=pl.BlockSpec(memory_space=pl.ANY),
            out_shape=jax.ShapeDtypeStruct((B, Dm), x0.dtype),
            scratch_shapes=[
                pltpu.VMEM((L, Dm), bf16),
                pltpu.VMEM((4, _TM, Dm), bf16),
                pltpu.VMEM((2, _TM, Dm), bf16),
                pltpu.VMEM((L, 8, Dm, 128), bf16),
                pltpu.VMEM((L, ntiles, 128, 128), bf16),
                pltpu.VMEM((L * 64, 128), f32),
                pltpu.VMEM((16, _ROFF, 128), f32),
                pltpu.VMEM((16, _ROFF, 128), bf16),
                pltpu.VMEM((L * 8, 8, 128), f32),
                pltpu.SemaphoreType.DMA((4,)),
                pltpu.SemaphoreType.DMA((L,)),
                pltpu.SemaphoreType.DMA((2,)),
                pltpu.SemaphoreType.DMA((2,)),
                pltpu.SemaphoreType.DMA((9,)),
            ]
            + [pltpu.VMEM((1, 260 * 8, 128), f32)] * 2
            + [pltpu.VMEM((1, sz * 8, 128), f32) for _, sz in _bufkeys()],
            compiler_params=pltpu.CompilerParams(
                vmem_limit_bytes=126 * 1024 * 1024,
                disable_bounds_checks=True,
            ),
        )(x0, ws, bs)

    return fn


@jax.jit
def pallas_standalone__dcn_v2_cross__recsys_kernel(
    x0: jax.Array,
    ws: jax.Array,
    bs: jax.Array,
):
    return _build()(x0, ws, bs)
```

```python
import functools
import itertools

import numpy as np
import jax
import jax.numpy as jnp
from jax import lax
import jax.experimental.pallas as pl
import jax.experimental.pallas.tpu as pltpu

f32 = jnp.float32
bf16 = jnp.bfloat16

_D = float(np.sqrt(3.0))
_TM = 512
_ROFF = 512
_H = _TM // 8
_NG = _H // 8
_BS = _NG + 1 + _NG % 2
_PH = (3, 5, 4, 7, 1, 2, 6)
_SO = (5, 7, 1, 6, 2)
_ALT = (1, 2, 4, 5)
_MIDB = {1: [(0, 1)], 2: [(1, 1)], 3: [(2, 1)], 5: [(3, 1)],
         4: [(0, 1), (2, -1)], 6: [(1, 1), (0, -1)], 7: [(3, 1), (0, -1)]}
_ZQ = {1: 0, 2: 0, 3: 0, 5: 0, 4: 1, 6: 2, 7: 3}
_CVEC = {1: [1, 0, 0, 1], 2: [0, 0, 1, -1], 3: [1, 1, 1, 1], 4: [1, 0, 1, 0],
         5: [-1, 1, 1, -1], 6: [0, 0, 1, 1], 7: [1, 0, -1, 0]}

_NAMES = ([(f"u{p}", 7) for p in (3, 4, 7, 5, 1, 2, 6)]
          + [(f"a{p}", 4) for p in (3, 4, 5, 7, 2, 6, 1)]
          + [(f"{s}{k}", 4) for s in ("fx", "H", "G", "U", "V") for k in range(2)]
          + [(f"x0{o}", 4) for o in range(4)]
          + [("u2x", 7), ("u6x", 7)] + [(f"{s}{k}", 4) for s in "HGUV" for k in (2, 3)])

_WIN = {"u1": (14.7, 23, 25), "x1": (23.5, 36, 38), "u2": (35.7, 39, 40), "x2": (39.4, 47, 48),
        "u3": (45, 49, 49), "u4": (49.2, 52.3, 53), "x4": (52.7, 61, 62), "x5": (61.4, 72.5, 76),
        "v1": (14.7, 23, 25), "o1": (23.4, 35, 48), "e1": (23.5, 35, 35), "v2": (35.7, 40, 41),
        "e2": (39, 45.5, 48), "o2": (41, 48.5, 48), "e4": (49, 60.5, 62), "e5": (60.9, 72.5, 76),
        "v3": (49, 60, 85), "v4": (60, 98, 285), "o4": (98, 190, 285), "o5": (190, 290, 299)}
_BOT_DONE = 250
_STAGES = {"u1": "u", "u2": "u", "u3": "u", "u4": "u", "v1": "u", "v2": "u", "v3": "u", "v4": "u",
           "x1": "gA", "x2": "gB", "x4": "hB", "x5": "hC", "o1": "e", "o2": "e", "o4": "f",
           "o5": "f", "e1": "nA", "e2": "nB", "e4": "nB", "e5": "nC"}
_SCOST = {"u": (16, 4), "g": (17, 0), "h": (25, 0), "A": (7, 4), "B": (15, 8), "C": (23, 12),
          "e": (22, 4), "f": (30, 4), "n": (14, 4)}
_AFTER = (("u1", "x1"), ("x1", "x2"), ("u2", "x2"), ("u3", "x4"), ("u4", "x4"), ("x4", "x5"),
          ("v1", "o1"), ("e1", "e2"), ("v2", "o2"), ("e4", "e5"), ("v3", "o4"), ("v4", "o4"),
          ("v4", "o5"))
_PLAIN = (1, 1)
_QO = (3, 5, 2, 4, 7, 6, 1)
_BP, _BQ = (3, 4, 7, 1), (5, 2, 1, 6)
_CFG = dict(win=_WIN, ws=0.2, lat=135, sm=4, dur=16, ulead=76, l0=20, l1=2, s1f=0.9)


def _kappa(bset):
    m = np.array([_CVEC[p] for p in bset], np.float64).T
    pats = [np.array([1, 0, _D, 0]), np.array([0, 1 / _D, 0, 1])]
    return [dict(zip(bset, np.linalg.solve(m, t))) for t in pats]


def _comb7(m):
    s = m[3] + m[5]
    e = (m[3] - m[5]) + m[1]
    return [(e + m[4]) + m[7], s, (((s + m[4]) - m[7]) + m[2]) + m[6], (e - m[2]) + m[6]]


def _combu(m):
    s = m[3] + m[4]
    u3 = m[3] + m[5]
    return [(s + m[7]) + m[1], u3, m[4] + m[2], m[6] - m[7]]


def _bwd(u):
    h = u[1] * 0.5
    c11 = u[0] - h
    return [c11, h, (u[2] + h) + u[3], (c11 - u[2]) + u[3]]


def _fwd(x, alt=False):
    a1 = x[0] + x[3]
    return [a1, ((x[1] + x[2]) + a1) * 0.5, x[1] + x[3] if alt else x[0] - x[1], x[0] + x[1]]


def _bexp(b):
    b1 = b[0] + b[3]
    u = b[1] + b[2]
    return {1: b1, 2: b[0] - b[1], 3: b[1] - b[3], 4: u - b1, 5: b[1] + b[3], 6: b[0] + b[1],
            7: u + b1}


def _rnd(v):
    return pltpu.bitcast((pltpu.bitcast(v, jnp.int32) + 0x8000) & -0x10000, f32)


def _bexp_inner(b):
    b1 = b[0] + b[3]
    r = _rnd(b1)
    b0 = b[0] + (r - b1) * 0.5
    b2 = b0 - b[1]
    b6 = b0 + b[1]
    b7 = ((b[1] + b[2]) + r) * 0.5
    return [r, b2, b6 - r, b7 - r, r - b2, b6, b7]


def _rowcol(o, i, t):
    r = (o // 2) * 4 + (i // 2) * 2 + t // 2
    c = (o % 2) * 4 + (i % 2) * 2 + t % 2
    e = (o // 2 - o % 2) + (i // 2 - i % 2) + (t // 2 - t % 2)
    return r, c, e


def _products():
    order = [(p, q) for p in _PH for q in _QO if (p, q) != _PLAIN]
    order.insert(32, _PLAIN)
    tile0 = {}
    n = 0
    for pq in order:
        tile0[pq] = n
        n += 4 if pq == _PLAIN else 7
    return order, tile0, n


def _qsize(k):
    return (k * _BS + 7) // 4 * 4


def _bufkeys():
    keys = []
    for n, k in _NAMES:
        if n[0] == "a":
            keys.append(((n, 0), 4 * _qsize(k)))
        else:
            keys += [((n, t), _qsize(k)) for t in range(4)]
    return keys


def _schedule(L, order, cfg):
    win = cfg["win"]
    prods = [(l, p, q) for l in range(L) for (p, q) in order]
    npr = len(prods)
    free = [0, 0, 0, 0]
    anchors = []
    pstart = []
    for pi, (l, p, q) in enumerate(prods):
        pstart.append(min(free))
        if (p, q) != _PLAIN:
            for j in range(7):
                mx = int(np.argmin(free))
                anchors += [(free[mx] + g * 8, pi, j, g) for g in range(_NG)]
                free[mx] += _H
        else:
            anchors += [(max(free) + g * 8, pi, 0, g) for g in range(2 * _NG)]
            free = [f + 2 * _H for f in free]
    pstart.append(max(free))
    anchors.sort()
    times = np.array([a[0] for a in anchors])

    def tpos(x):
        i = int(np.floor(x))
        return pstart[i] + (x - i) * (pstart[min(i + 1, npr)] - pstart[i])

    npos = 4 * _NG
    load = np.zeros(pstart[-1] // 8 + 1)

    def spread(t0, t1, valu, stores):
        b0, b1 = max(int(t0 // 8), 0), max(int(t1 // 8), 1)
        load[b0:b1] += (valu / 4 + stores * cfg["ws"]) / max(int(t1 // 8) - int(t0 // 8), 1)

    for pi, (l, p, q) in enumerate(prods):
        big = (p, q) != _PLAIN
        t0, t1 = pstart[pi], pstart[pi + 1]
        spread(t0 - cfg["lat"], t1 - cfg["lat"],
               (len(_MIDB[q]) - 1 + (2.125 if big else 0.5)) * npos, 0)
        extra = {5: 1, 1: 5, 2: 1, 6: 1}.get(p, 0) + (p in _BP and q in _BQ)
        spread(t0, t1 + (_H // 2 if big else 0), ((1.5 if big else 1) + extra) * npos, npos)

    kern = np.hanning(cfg["sm"] + 2)[1:-1]
    kern /= kern.sum()
    jobs = [(w, l) for l in range(L - 1)
            for w in ("u1", "x1", "u2", "x2", "u3", "u4", "x4", "x5")]
    jobs += [(w, L - 1) for w in ("v1", "o1", "e1", "v2", "e2", "o2", "e4", "e5", "v3", "v4",
                                  "o4", "o5")]
    sched = {}
    for jn, (w, l) in sorted(enumerate(jobs), key=lambda e: win[e[1][0]][1] - win[e[1][0]][0]):
        i0, i1, last = (l * 49 + v for v in win[w])
        prev = i0 >= npr
        if prev:
            i0, i1, last = i0 - npr, i1 - npr, last - npr
        lo, hi = int(np.ceil(tpos(i0) / 8)), int(tpos(i1) // 8)
        kinds = [k for k in _STAGES[w] for _ in range(4)]
        avg = np.mean([_SCOST[k] for k in kinds], 0)
        trial = load.copy()
        picks = []
        for _ in range(len(kinds) * _NG):
            sm = np.round(np.convolve(load, kern, mode="same"), 9)
            bb = lo + int(np.argmin(sm[lo + 1:hi + 1]))
            picks.append(bb)
            spread(bb * 8, bb * 8 + cfg["dur"], *avg)
        picks.sort()
        load[:] = trial
        slots = []
        for n, bb in enumerate(picks):
            spread(bb * 8, bb * 8 + cfg["dur"], *_SCOST[kinds[n % len(kinds)]])
            ai = int(np.searchsorted(times, bb * 8))
            while anchors[ai][1] < int(i0):
                ai += 1
            slots.append(anchors[ai][1:])
        at = max(a[0] for a in slots)
        assert int(i0) <= at <= last, (w, l, at)
        sched.setdefault(at, []).append(
            (-1 if prev else 0, jn, w, l, [slots[k::len(kinds)] for k in range(len(kinds))]))
    where = {}
    for at, v in sched.items():
        v.sort(key=lambda e: e[:2])
        where.update({(e[2], e[3]): (at, k) for k, e in enumerate(v)})
    for a, b in _AFTER:
        assert all(where[a, l] < where[b, l] for w, l in jobs if w == a), (a, b)

    ugate = {}
    for pi in range(49):
        if prods[pi][1:] != _PLAIN and pstart[pi] >= 200:
            al = []
            for g in range(_NG):
                gt = pstart[pi] + (g // 2) * 16 - cfg["ulead"]
                ai = int(np.searchsorted(times, gt, side="right")) - 1
                while anchors[ai][1] >= pi:
                    ai -= 1
                al.append(anchors[ai][1:])
            ugate[pi] = al
    return prods, sched, ugate


def _kernel(x_hbm, w_hbm, b_hbm, o_hbm, b_ref, ring, stage, wraw, wexp, beta, fx32, fxb, fb,
            xsem, wsem, tsem, bsem, fsem, *bufs, L, nsteps, cfg):
    H, HT = _H, _TM // 2
    order, tile0, _ = _products()
    tmp = bufs[:2]
    buf = dict(zip([k for k, _ in _bufkeys()], bufs[2:]))
    skew = {n: k % 4 for k, (n, _) in enumerate(_NAMES)}
    ctx = {"rows": (0, H)}

    def x_copy(i):
        return pltpu.make_async_copy(
            x_hbm.at[pl.ds(pl.multiple_of(_ROFF + i * _TM, 64), _TM)], ring.at[i & 3],
            xsem.at[i & 3])

    def w_copies(l):
        return [pltpu.make_async_copy(w_hbm.at[l, :, pl.ds(c * 128, 128)], wraw.at[l & 1, c],
                                      wsem.at[l]) for c in range(8)]

    def top_copy(i):
        return pltpu.make_async_copy(
            stage.at[i & 1, pl.ds(HT, HT)],
            o_hbm.at[pl.ds(pl.multiple_of(_ROFF + i * _TM, 64), HT)], tsem.at[i & 1])

    def bot_copy(i):
        return pltpu.make_async_copy(
            stage.at[i & 1, pl.ds(0, HT)],
            o_hbm.at[pl.ds(pl.multiple_of(_ROFF + i * _TM - HT, 64), HT)], bsem.at[i & 1])

    def fin(c):
        return pltpu.make_async_copy(
            x_hbm.at[pl.ds(0, _ROFF), pl.ds(c * 128, 128)], fxb.at[c], fsem.at[c])

    def fout(c):
        return pltpu.make_async_copy(
            fxb.at[(L & 1) * 8 + c], o_hbm.at[pl.ds(0, _ROFF), pl.ds(c * 128, 128)], fsem.at[c])

    def loc(n, b, t):
        if n[0] == "a":
            return buf[n, 0], (t * _qsize(4) + (skew[n] + t) % 4 + b * _BS) * 8
        return buf[n, t], ((skew[n] + t) % 4 + b * _BS) * 8

    def ld(n, b, t):
        ref, o = loc(n, b, t)
        r, k = ctx["rows"]
        return ref[ctx["z"], o + r:o + r + k, :]

    def st(n, b, t, v):
        ref, o = loc(n, b, t)
        r, k = ctx["rows"]
        ref[0, o + r:o + r + k, :] = v

    def anc(v, a):
        return v if a is None else jnp.where(ctx["never"], a, v)

    def xin(j, o, i, t):
        r, c, _ = _rowcol(o, i, t)
        r0, k = r * H + ctx["rows"][0], ctx["rows"][1]
        return ring[ctx["slot"][j], r0:r0 + k, c * 128:(c + 1) * 128].astype(f32)

    def sname(s, l):
        return f"{s}{l - L + 4 if l >= L - 2 else l % 2}"

    def uname(p, l):
        return f"u{p}x" if (l == L - 1 and p in (2, 6)) else f"u{p}"

    def upd(l, p, s, a):
        for j in range(4):
            m = {q: ld(uname(p, l), q - 1, j) for q in range(1, 8)}
            m[3] = anc(m[3], next(a))
            v = _comb7(m)
            if l > 0:
                v = [v[i] + ld(sname(s, l - 1), i, j) for i in range(4)]
            for i in range(4):
                st(sname(s, l), i, j, v[i])

    def gval(o, l):
        def g(i):
            s = lambda n, j: ld(sname(n, l), i, j)
            return [s("GH"[o], j) if o < 2 else
                    (s("U", j) + s("V", j)) + s("H", j) if o == 2 else
                    (s("G", j) - s("U", j)) + s("V", j) for j in range(4)]
        return g

    def blocks(g, i, a):
        u = g(i)
        u[1] = anc(u[1], next(a))
        return _bwd(u)

    def gate(o, l, a):
        g = gval(o, l)
        return [_fwd([ld(f"x0{o}", i, t) * v for t, v in enumerate(blocks(g, i, a))],
                     l + 1 in _ALT) for i in range(4)]

    def emit(o, g, a):
        for i in range(4):
            for t, v in enumerate(blocks(g, i, a)):
                r, c, e = _rowcol(o, i, t)
                y = xin(ctx["j"], o, i, t) * v
                if e:
                    y = y * (_D ** -e)
                r0 = ctx["j"] * _TM + r * H + HT + ctx["rows"][0]
                stage[ctx["oslot"], r0:r0 + ctx["rows"][1], c * 128:(c + 1) * 128] = y.astype(bf16)

    def fresh(o, a):
        out = []
        for i in range(4):
            xs = []
            for t in range(4):
                e = _rowcol(o, i, t)[2]
                v = xin(ctx["j"] + 1, o, i, t)
                if t == 0:
                    v = anc(v, next(a))
                st(f"x0{o}", i, t, v)
                xs.append(v * (_D ** e) if e else v)
            out.append(_fwd(xs, 0 in _ALT))
        return out

    def mid(x, a):
        for j in range(4):
            for i, v in enumerate(_fwd([anc(x[0][j], next(a))] + [x[i][j] for i in (1, 2, 3)])):
                yield i, j, v

    def f1(l, x, a):
        for i, j, v in mid(x, a):
            st(f"fx{l % 2}", i, j, v)

    def f2(l, x, a):
        for i, j, v in mid(x, a):
            w = ld(f"fx{l % 2}", i, j)
            st("a3", i, j, v - w)
            st("a5", i, j, v + w)

    def f4(l, x, a):
        for i, j, v in mid(x, a):
            w = ld(f"fx{l % 2}", i, j)
            st("a4", i, j, w + v)
            st("a7", i, j, w - v)

    def f5(l, x, a):
        for i, j, v in mid(x, a):
            u = ld(f"fx{l % 2}", i, j) + v
            a1 = ld("a3", i, j) + ld("a4", i, j)
            st("a1", i, j, a1)
            st("a2", i, j, u + a1)
            st("a6", i, j, u - a1)

    task = {
        "u1": lambda l, a: upd(l, 5, "H", a),
        "u2": lambda l, a: upd(l, 1, "G", a),
        "u3": lambda l, a: upd(l, 2, "U", a),
        "u4": lambda l, a: upd(l, 6, "V", a),
        "x1": lambda l, a: f1(l, gate(1, l, a), a),
        "x2": lambda l, a: f2(l, gate(0, l, a), a),
        "x4": lambda l, a: f4(l, gate(3, l, a), a),
        "x5": lambda l, a: f5(l, gate(2, l, a), a),
        "o1": lambda l, a: emit(1, gval(1, l), a),
        "o2": lambda l, a: emit(0, gval(0, l), a),
        "o4": lambda l, a: emit(3, gval(3, l), a),
        "o5": lambda l, a: emit(2, gval(2, l), a),
        "e1": lambda l, a: f1(l, fresh(1, a), a),
        "e2": lambda l, a: f2(l, fresh(0, a), a),
        "e4": lambda l, a: f4(l, fresh(3, a), a),
        "e5": lambda l, a: f5(l, fresh(2, a), a),
    }
    for k in "1234":
        task["v" + k] = task["u" + k]

    def run_plain(names):
        for g in range(_NG):
            ctx["rows"] = (g * 8, 8)
            for w in names:
                task[w](L - 1, itertools.repeat(None))
        ctx["rows"] = (0, H)

    b_copy = pltpu.make_async_copy(b_hbm, b_ref, fsem.at[8])
    b_copy.start()
    for c in range(8):
        fin(c).start()
    for cp in w_copies(0):
        cp.start()

    for n in ("u2x", "u6x", sname("U", L - 2), sname("V", L - 2), sname("G", L - 1),
              sname("H", L - 1)):
        for t in range(4):
            buf[n, t][...] = jnp.zeros(buf[n, t].shape, f32)
    ring[3, HT:, :] = jnp.zeros((HT, ring.shape[2]), bf16)
    fx32[8:16] = jnp.ones((8, _ROFF, 128), f32)

    b_copy.wait()
    kap, kaq = _kappa(_BP), _kappa(_BQ)
    for l in range(L):
        bl = b_ref[l:l + 1, :].astype(f32)
        for c in range(8):
            fb[l * 8 + c, 0:1, :] = bl[:, c * 128:(c + 1) * 128]
        if l == 0:
            bl = bl + 1.0
        for pi, p in enumerate(_BP):
            for qi, q in enumerate(_BQ):
                col = []
                for c3 in range(2):
                    acc = None
                    for c1 in range(2):
                        for c2 in range(2):
                            k = float(kap[c1][p] * kaq[c2][q])
                            if abs(k) < 1e-12:
                                continue
                            c = c1 * 4 + c2 * 2 + c3
                            term = bl[:, c * 128:(c + 1) * 128] * k
                            acc = term if acc is None else acc + term
                    col.append(acc)
                us = [col[0] + col[1] * (1 / _D), col[1] * (2 / _D),
                      col[0] * ((_D + 1) / 2) - col[1] * ((1 + 1 / _D) / 2),
                      col[0] * ((_D - 1) / 2) + col[1] * ((1 - 1 / _D) / 2)]
                row = l * 64 + (pi * 4 + qi) * 4
                for j in range(4):
                    beta[row + j:row + j + 1, :] = us[j]
    for c in range(8):
        fin(c).wait()
    for c in range(8):
        fx32[c] = fxb[c].astype(f32)

    def toff(p, i, t):
        return ((p - 1) * 37 + (i * 4 + t) * 2 + i) * 8

    def s1_units(l, g, dst):
        r0 = g * 16

        def unit(mids, t, a):
            blk = {}
            for i in mids:
                for o in range(4):
                    r, c, e = _rowcol(o, i, t)
                    v = wraw[l & 1, c, r * 128 + r0:r * 128 + r0 + 16, :].astype(f32)
                    blk[o, i] = v * (0.25 * _D ** e)
            if len(mids) == 2:
                blk[0, 0] = anc(blk[0, 0], a(0))
                sm = (blk[0, 0] + blk[3, 0]) + (blk[0, 3] + blk[3, 3])
                dl = (_rnd(sm) - sm) * 0.25
                for k in ((0, 0), (3, 0), (0, 3), (3, 3)):
                    blk[k] = blk[k] + dl
            else:
                blk[1, mids[0]] = anc(blk[1, mids[0]], a(0))
            out = []
            for i in mids:
                ex = _bexp([blk[o, i] for o in range(4)])
                for p in _PH:
                    dst[0, toff(p, i, t):toff(p, i, t) + 16, :] = ex[p]
                out.append(ex[7][:8])
            return out

        return [(34 if len(m) == 1 else 90, functools.partial(unit, m, t))
                for t in range(4) for m in ((0, 3), (1,), (2,))]

    def s2_units(l, g, src, zg):
        r0 = g * 16

        def put(p, q, qs, a=None):
            qs = [qs[0], anc(qs[1], a), qs[2], qs[3]]
            if (p, q) != _PLAIN:
                f = (2.0 if p == 1 else 1.0) * (2 if q in (1, 2, 6) else 1)
                qs = _bexp_inner([v * f for v in qs] if f != 1 else qs)
            for k, v in enumerate(qs):
                wexp[l, tile0[p, q] + k, r0:r0 + 16, :] = v.astype(bf16)

        def unit(p, un, a):
            def tl(i):
                vs = [src[zg[un], toff(p, i, t):toff(p, i, t) + 16, :] for t in range(4)]
                if i == (0 if un == 2 else 1):
                    vs[1] = anc(vs[1], a(0))
                return vs

            if un == 0:
                x, y, qa, qb = tl(0), tl(1), 2, 6
            elif un == 1:
                x, y, qa, qb = tl(1), tl(3), 3, 5
            else:
                x = [u + v for u, v in zip(tl(1), tl(2))]
                y = [u + v for u, v in zip(tl(0), tl(3))]
                qa, qb = 4, 7
                put(p, 1, y)
            put(p, qa, [u - v for u, v in zip(x, y)], a(2) if un == 2 else None)
            put(p, qb, [u + v for u, v in zip(x, y)], a(4 if un == 2 else 2))

        return [((102, 86, 145)[un], functools.partial(unit, p, un))
                for p in _PH for un in range(3)]

    def layer(l, carry):
        for cp in w_copies(l):
            cp.wait()

        @pl.when(l + 1 < L)
        def _():
            for cp in w_copies(l + 1):
                cp.start()

        @pl.when(l == L - 2)
        def _():
            x_copy(0).start()
            x_copy(1).start()

        zg = [lax.shift_right_logical(l, 8 + k) for k in range(4)]
        ctx["never"] = jnp.full((16, 128), zg[0], jnp.int32) != 0
        head = [v for _, f in s1_units(l, 0, tmp[0]) for v in f(lambda d: None)]
        units = []
        for g in range(8):
            u2 = s2_units(l, g, tmp[g % 2], zg[1:])
            units += [(g + k / len(u2), c, f) for k, (c, f) in enumerate(u2)]
            if g < 7:
                u1 = s1_units(l, g + 1, tmp[(g + 1) % 2])
                units += [(g + (k + 0.5) / len(u1) * cfg["s1f"], c, f)
                          for k, (c, f) in enumerate(u1)]
        units.sort(key=lambda e: e[0])
        total = sum(c for _, c, _ in units)
        nr = _ROFF // 8
        acc = 0
        todo = {}
        for _, c, f in units:
            sl = cfg["l0"] + int(acc / total * (16 * nr - cfg["l0"] - cfg["l1"]))
            todo.setdefault(sl // nr, []).append((sl % nr, f))
            acc += c
        fsrc = (l & 1) * 8
        fu = fxb.bitcast(jnp.uint32)
        wu = wraw.bitcast(jnp.uint32)
        for g in range(8):
            for h in range(2):
                cols = [fu[fsrc + 4 * h + c] for c in range(4)]
                if g == 0 and h == 0:
                    pace = jnp.concatenate([pltpu.bitcast(v, jnp.uint32) for v in head], 0)
                    nv = jnp.full((128, 128), zg[0], jnp.int32) != 0
                    cols[0] = jnp.concatenate(
                        [cols[0][:16], jnp.where(nv, pace, cols[0][16:144]), cols[0][144:]], 0)
                xa = jnp.concatenate([pltpu.bitcast(v, bf16) for v in cols], 1)
                y = jnp.dot(xa, pltpu.bitcast(wu[l & 1, g, h * 256:(h + 1) * 256, :], bf16),
                            preferred_element_type=f32)
                if h == 0:
                    fx32[8 + g] = (y + fb[l * 8 + g, 0:1, :]) + fx32[8 + g]
                else:
                    gn = y + fx32[8 + g]
                    fx32[8 + g] = gn
                    fxb[8 - fsrc + g] = (fx32[g] * gn).astype(bf16)
                for r, f in todo.get(2 * g + h, []):
                    f(lambda d: y[min(r + d, nr - 2) * 8:min(r + d, nr - 2) * 8 + 16])
        return carry

    lax.fori_loop(0, L, layer, 0)
    for c in range(8):
        fout(c).start()
    x_copy(0).wait()
    ctx.update(z=0, slot={0: 0}, j=-1)
    run_plain(("e1", "e2"))

    prods, sched, ugate = _schedule(L, order, cfg)

    def main(step, carry):
        @pl.when(step + 1 < nsteps)
        def _():
            x_copy(step + 1).wait()

        @pl.when(step >= 2)
        def _():
            top_copy(step - 2).wait()

        @pl.when(step >= 3)
        def _():
            bot_copy(step - 2).wait()

        @pl.when(step >= 1)
        def _():
            top_copy(step - 1).start()

        @pl.when(step + 2 < nsteps)
        def _():
            x_copy(step + 2).start()

        zz = [lax.shift_right_logical(step, 12 + k) for k in range(14)]
        ctx.update(never=jnp.full((H, 128), zz[0], jnp.int32) != 0,
                   slot={-1: (step + 3) & 3, 0: step & 3, 1: (step + 1) & 3}, oslot=step & 1)
        wu = wexp.bitcast(jnp.uint32)
        subs = {}

        def wtile(l, k):
            return pltpu.bitcast(wu[l, k], bf16)

        def gather(al):
            return jnp.concatenate([subs[pi][j][g * 8:(g + 1) * 8, :] for pi, j, g in al], 0)

        for pi, (l, p, q) in enumerate(prods):
            ctx["z"] = zz[_ZQ[q]]
            qv = []
            for t in range(4):
                vs = [ld(f"a{p}", b, t) for b, _ in _MIDB[q]]
                qv.append(vs[0] if len(vs) == 1 else vs[0] - vs[1])
                if t == 1 and pi in ugate:
                    qv[t] = anc(qv[t], gather(ugate[pi]))
            k0 = tile0[p, q]
            if (p, q) != _PLAIN:
                a1 = _rnd(qv[0])
                r3, r4 = (4, 3) if l in _ALT else (3, 4)
                av = {1: a1, 2: qv[1], r3: qv[2], 5: qv[3], r4: a1 - qv[2], 6: qv[1] - a1,
                      7: qv[3] - a1}
                so = (r3, r4) + _SO
                m = {r: jnp.dot(av[r].astype(bf16), wtile(l, k0 + r - 1),
                                preferred_element_type=f32) for r in so}
                subs[pi] = [m[r] for r in so]
                mq = _combu(m)
            else:
                if l in _ALT:
                    qv[2] = qv[0] - qv[2]
                d1 = qv[0] + qv[0]
                y11, y12 = qv[2] + qv[3], qv[3] - qv[2]
                qv = [y11, y12, (qv[1] * 4.0 - d1) - y12, d1 - y11]
                a = jnp.concatenate(
                    [jnp.concatenate(qv[:2], 1), jnp.concatenate(qv[2:], 1)], 0).astype(bf16)
                wt = [wtile(l, k0 + t) for t in range(4)]
                wm = jnp.concatenate([jnp.concatenate(wt[:2], 1), jnp.concatenate(wt[2:], 1)], 0)
                mm = jnp.dot(a, wm, preferred_element_type=f32)
                subs[pi] = [mm[:, :128]]
                c11, c12, c21, c22 = mm[:H, :128], mm[:H, 128:], mm[H:, :128], mm[H:, 128:]
                sm = c11 + c12
                mq = [sm + sm, c12 * 4.0, (c21 - c22) + (c11 - c12), (c21 + c22) - sm]
            if p in _BP and q in _BQ:
                row = l * 64 + (_BP.index(p) * 4 + _BQ.index(q)) * 4
                mq = [mq[t] + beta[row + t:row + t + 1, :] for t in range(4)]
            for t in range(4):
                v = mq[t]
                if p == 5:
                    v = v + ld("u3", q - 1, t)
                elif p == 1:
                    r3 = ld("u3", q - 1, t)
                    v = v + (((ld("u4", q - 1, t) + ld("u7", q - 1, t)) + (r3 + r3))
                             - ld("u5", q - 1, t))
                elif p == 2:
                    v = v + ld("u4", q - 1, t)
                elif p == 6:
                    v = v - ld("u7", q - 1, t)
                st(uname(p, l), q - 1, t, v)
            for j, jn, w, tl, als in sched.get(pi, []):
                ctx.update(z=zz[4 + jn % 10], j=j)
                task[w](tl, iter([gather(al) for al in als]))
            if pi == _BOT_DONE:
                @pl.when(step >= 1)
                def _():
                    bot_copy(step).start()

        return carry

    lax.fori_loop(0, nsteps, main, 0)

    top_copy(nsteps - 1).start()
    top_copy(nsteps - 2).wait()
    bot_copy(nsteps - 2).wait()
    ctx.update(z=0, slot={-1: (nsteps - 1) % 4}, j=-1, oslot=nsteps % 2)
    run_plain(("v3", "v4", "o4", "o5"))
    bot_copy(nsteps).start()
    for c in range(8):
        fout(c).wait()
    top_copy(nsteps - 1).wait()
    bot_copy(nsteps - 1).wait()
    bot_copy(nsteps).wait()


def _build(**kw):
    cfg = dict(_CFG, **kw)

    def fn(x0, ws, bs):
        B, Dm = x0.shape
        L = ws.shape[0]
        assert Dm == 1024 and L == 6 and (B - _ROFF) % _TM == 0
        nsteps = (B - _ROFF) // _TM
        assert 4 <= nsteps < 4096
        ntiles = _products()[2]
        return pl.pallas_call(
            functools.partial(_kernel, L=L, nsteps=nsteps, cfg=cfg),
            in_specs=[pl.BlockSpec(memory_space=pl.ANY)] * 3,
            out_specs=pl.BlockSpec(memory_space=pl.ANY),
            out_shape=jax.ShapeDtypeStruct((B, Dm), x0.dtype),
            scratch_shapes=[
                pltpu.VMEM((L, Dm), bf16),
                pltpu.VMEM((4, _TM, Dm), bf16),
                pltpu.VMEM((2, _TM, Dm), bf16),
                pltpu.VMEM((2, 8, Dm, 128), bf16),
                pltpu.VMEM((L, ntiles, 128, 128), bf16),
                pltpu.VMEM((L * 64, 128), f32),
                pltpu.VMEM((16, _ROFF, 128), f32),
                pltpu.VMEM((16, _ROFF, 128), bf16),
                pltpu.VMEM((L * 8, 8, 128), f32),
                pltpu.SemaphoreType.DMA((4,)),
                pltpu.SemaphoreType.DMA((L,)),
                pltpu.SemaphoreType.DMA((2,)),
                pltpu.SemaphoreType.DMA((2,)),
                pltpu.SemaphoreType.DMA((9,)),
            ]
            + [pltpu.VMEM((1, 260 * 8, 128), f32)] * 2
            + [pltpu.VMEM((1, sz * 8, 128), f32) for _, sz in _bufkeys()],
            compiler_params=pltpu.CompilerParams(
                vmem_limit_bytes=126 * 1024 * 1024,
                disable_bounds_checks=True,
            ),
        )(x0, ws, bs)

    return fn


@jax.jit
def pallas_standalone__dcn_v2_cross__recsys_kernel(
    x0: jax.Array,
    ws: jax.Array,
    bs: jax.Array,
):
    return _build()(x0, ws, bs)
```

```python
import functools
import itertools

import numpy as np
import jax
import jax.numpy as jnp
from jax import lax
import jax.experimental.pallas as pl
import jax.experimental.pallas.tpu as pltpu

f32 = jnp.float32
bf16 = jnp.bfloat16

_D = float(np.sqrt(3.0))
_TM = 512
_ROFF = 512
_H = _TM // 8
_NG = _H // 8
_BS = _NG + 1 + _NG % 2
_PH = (3, 5, 4, 7, 1, 2, 6)
_SO = (5, 7, 1, 6, 2)
_ALT = (1, 2, 4, 5)
_MIDB = {1: [(0, 1)], 2: [(1, 1)], 3: [(2, 1)], 5: [(3, 1)],
         4: [(0, 1), (2, -1)], 6: [(1, 1), (0, -1)], 7: [(3, 1), (0, -1)]}
_ZQ = {1: 0, 2: 0, 3: 0, 5: 0, 4: 1, 6: 2, 7: 3}
_CVEC = {1: [1, 0, 0, 1], 2: [0, 0, 1, -1], 3: [1, 1, 1, 1], 4: [1, 0, 1, 0],
         5: [-1, 1, 1, -1], 6: [0, 0, 1, 1], 7: [1, 0, -1, 0]}

_NAMES = ([(f"u{p}", 7) for p in (3, 4, 7, 5, 1, 2, 6)]
          + [(f"a{p}", 4) for p in (3, 4, 5, 7, 2, 6, 1)]
          + [(f"{s}{k}", 4) for s in ("fx", "H", "G", "U", "V") for k in range(2)]
          + [(f"x0{o}", 4) for o in range(4)]
          + [("u2x", 7), ("u6x", 7)] + [(f"{s}{k}", 4) for s in "HGUV" for k in (2, 3)])

_WIN = {"u1": (14.7, 23, 25), "x1": (23.5, 36, 38), "u2": (35.7, 39, 40), "x2": (39.4, 47, 48),
        "u3": (45, 49, 49), "u4": (49.2, 52.3, 53), "x4": (52.7, 61, 62), "x5": (61.4, 72.5, 76),
        "v1": (14.7, 23, 25), "o1": (23.4, 35, 48), "e1": (23.5, 35, 35), "v2": (35.7, 40, 41),
        "e2": (39, 45.5, 48), "o2": (41, 48.5, 48), "e4": (49, 60.5, 62), "e5": (60.9, 72.5, 76),
        "v3": (49, 72, 85), "v4": (72, 110, 285), "o4": (110.5, 200, 285), "o5": (200, 292, 299)}
_BOT_DONE = 250
_STAGES = {"u1": "u", "u2": "u", "u3": "u", "u4": "u", "v1": "u", "v2": "u", "v3": "u", "v4": "u",
           "x1": "gA", "x2": "gB", "x4": "hB", "x5": "hC", "o1": "e", "o2": "e", "o4": "f",
           "o5": "f", "e1": "nA", "e2": "nB", "e4": "nB", "e5": "nC"}
_SCOST = {"u": (16, 4), "g": (17, 0), "h": (25, 0), "A": (7, 4), "B": (15, 8), "C": (23, 12),
          "e": (22, 4), "f": (30, 4), "n": (14, 4)}
_AFTER = (("u1", "x1"), ("x1", "x2"), ("u2", "x2"), ("u3", "x4"), ("u4", "x4"), ("x4", "x5"),
          ("v1", "o1"), ("e1", "e2"), ("v2", "o2"), ("e4", "e5"), ("v3", "o4"), ("v4", "o4"),
          ("v4", "o5"))
_PLAIN = (1, 1)
_QO = (3, 5, 2, 4, 7, 6, 1)
_BP, _BQ = (3, 4, 7, 1), (5, 2, 1, 6)
_CFG = dict(win=_WIN, ws=0.2, lat=135, sm=4, dur=16, ulead=76, l0=20, l1=2, s1f=0.9)


def _kappa(bset):
    m = np.array([_CVEC[p] for p in bset], np.float64).T
    pats = [np.array([1, 0, _D, 0]), np.array([0, 1 / _D, 0, 1])]
    return [dict(zip(bset, np.linalg.solve(m, t))) for t in pats]


def _comb7(m):
    s = m[3] + m[5]
    e = (m[3] - m[5]) + m[1]
    return [(e + m[4]) + m[7], s, (((s + m[4]) - m[7]) + m[2]) + m[6], (e - m[2]) + m[6]]


def _combu(m):
    s = m[3] + m[4]
    u3 = m[3] + m[5]
    return [(s + m[7]) + m[1], u3, m[4] + m[2], m[6] - m[7]]


def _bwd(u):
    h = u[1] * 0.5
    c11 = u[0] - h
    return [c11, h, (u[2] + h) + u[3], (c11 - u[2]) + u[3]]


def _fwd(x, alt=False):
    a1 = x[0] + x[3]
    return [a1, ((x[1] + x[2]) + a1) * 0.5, x[1] + x[3] if alt else x[0] - x[1], x[0] + x[1]]


def _bexp(b):
    b1 = b[0] + b[3]
    u = b[1] + b[2]
    return {1: b1, 2: b[0] - b[1], 3: b[1] - b[3], 4: u - b1, 5: b[1] + b[3], 6: b[0] + b[1],
            7: u + b1}


def _rnd(v):
    return pltpu.bitcast((pltpu.bitcast(v, jnp.int32) + 0x8000) & -0x10000, f32)


def _bexp_inner(b):
    b1 = b[0] + b[3]
    r = _rnd(b1)
    b0 = b[0] + (r - b1) * 0.5
    b2 = b0 - b[1]
    b6 = b0 + b[1]
    b7 = ((b[1] + b[2]) + r) * 0.5
    return [r, b2, b6 - r, b7 - r, r - b2, b6, b7]


def _rowcol(o, i, t):
    r = (o // 2) * 4 + (i // 2) * 2 + t // 2
    c = (o % 2) * 4 + (i % 2) * 2 + t % 2
    e = (o // 2 - o % 2) + (i // 2 - i % 2) + (t // 2 - t % 2)
    return r, c, e


def _products():
    order = [(p, q) for p in _PH for q in _QO if (p, q) != _PLAIN]
    order.insert(32, _PLAIN)
    tile0 = {}
    n = 0
    for pq in order:
        tile0[pq] = n
        n += 4 if pq == _PLAIN else 7
    return order, tile0, n


def _qsize(k):
    return (k * _BS + 7) // 4 * 4


def _bufkeys():
    keys = []
    for n, k in _NAMES:
        if n[0] == "a":
            keys.append(((n, 0), 4 * _qsize(k)))
        else:
            keys += [((n, t), _qsize(k)) for t in range(4)]
    return keys


def _schedule(L, order, cfg):
    win = cfg["win"]
    prods = [(l, p, q) for l in range(L) for (p, q) in order]
    npr = len(prods)
    free = [0, 0, 0, 0]
    anchors = []
    pstart = []
    for pi, (l, p, q) in enumerate(prods):
        pstart.append(min(free))
        if (p, q) != _PLAIN:
            for j in range(7):
                mx = int(np.argmin(free))
                anchors += [(free[mx] + g * 8, pi, j, g) for g in range(_NG)]
                free[mx] += _H
        else:
            anchors += [(max(free) + g * 8, pi, 0, g) for g in range(2 * _NG)]
            free = [f + 2 * _H for f in free]
    pstart.append(max(free))
    anchors.sort()
    times = np.array([a[0] for a in anchors])

    def tpos(x):
        i = int(np.floor(x))
        return pstart[i] + (x - i) * (pstart[min(i + 1, npr)] - pstart[i])

    npos = 4 * _NG
    load = np.zeros(pstart[-1] // 8 + 1)

    def spread(t0, t1, valu, stores):
        b0, b1 = max(int(t0 // 8), 0), max(int(t1 // 8), 1)
        load[b0:b1] += (valu / 4 + stores * cfg["ws"]) / max(int(t1 // 8) - int(t0 // 8), 1)

    for pi, (l, p, q) in enumerate(prods):
        big = (p, q) != _PLAIN
        t0, t1 = pstart[pi], pstart[pi + 1]
        spread(t0 - cfg["lat"], t1 - cfg["lat"],
               (len(_MIDB[q]) - 1 + (2.125 if big else 0.5)) * npos, 0)
        extra = {5: 1, 1: 5, 2: 1, 6: 1}.get(p, 0) + (p in _BP and q in _BQ)
        spread(t0, t1 + (_H // 2 if big else 0), ((1.5 if big else 1) + extra) * npos, npos)

    kern = np.hanning(cfg["sm"] + 2)[1:-1]
    kern /= kern.sum()
    jobs = [(w, l) for l in range(L - 1)
            for w in ("u1", "x1", "u2", "x2", "u3", "u4", "x4", "x5")]
    jobs += [(w, L - 1) for w in ("v1", "o1", "e1", "v2", "e2", "o2", "e4", "e5", "v3", "v4",
                                  "o4", "o5")]
    sched = {}
    for jn, (w, l) in sorted(enumerate(jobs), key=lambda e: win[e[1][0]][1] - win[e[1][0]][0]):
        i0, i1, last = (l * 49 + v for v in win[w])
        prev = i0 >= npr
        if prev:
            i0, i1, last = i0 - npr, i1 - npr, last - npr
        lo, hi = int(np.ceil(tpos(i0) / 8)), int(tpos(i1) // 8)
        kinds = [k for k in _STAGES[w] for _ in range(4)]
        avg = np.mean([_SCOST[k] for k in kinds], 0)
        trial = load.copy()
        picks = []
        for _ in range(len(kinds) * _NG):
            sm = np.round(np.convolve(load, kern, mode="same"), 9)
            bb = lo + int(np.argmin(sm[lo + 1:hi + 1]))
            picks.append(bb)
            spread(bb * 8, bb * 8 + cfg["dur"], *avg)
        picks.sort()
        load[:] = trial
        slots = []
        for n, bb in enumerate(picks):
            spread(bb * 8, bb * 8 + cfg["dur"], *_SCOST[kinds[n % len(kinds)]])
            ai = int(np.searchsorted(times, bb * 8))
            while anchors[ai][1] < int(i0):
                ai += 1
            slots.append(anchors[ai][1:])
        at = max(a[0] for a in slots)
        assert int(i0) <= at <= last, (w, l, at)
        sched.setdefault(at, []).append(
            (-1 if prev else 0, jn, w, l, [slots[k::len(kinds)] for k in range(len(kinds))]))
    where = {}
    for at, v in sched.items():
        v.sort(key=lambda e: e[:2])
        where.update({(e[2], e[3]): (at, k) for k, e in enumerate(v)})
    for a, b in _AFTER:
        assert all(where[a, l] < where[b, l] for w, l in jobs if w == a), (a, b)

    ugate = {}
    for pi in range(49):
        if prods[pi][1:] != _PLAIN and pstart[pi] >= 200:
            al = []
            for g in range(_NG):
                gt = pstart[pi] + (g // 2) * 16 - cfg["ulead"]
                ai = int(np.searchsorted(times, gt, side="right")) - 1
                while anchors[ai][1] >= pi:
                    ai -= 1
                al.append(anchors[ai][1:])
            ugate[pi] = al
    return prods, sched, ugate


def _kernel(x_hbm, w_hbm, b_hbm, o_hbm, b_ref, ring, stage, wraw, wexp, beta, fx32, fxb, fb,
            xsem, wsem, tsem, bsem, fsem, *bufs, L, nsteps, cfg):
    H, HT = _H, _TM // 2
    order, tile0, _ = _products()
    tmp = bufs[:2]
    buf = dict(zip([k for k, _ in _bufkeys()], bufs[2:]))
    skew = {n: k % 4 for k, (n, _) in enumerate(_NAMES)}
    ctx = {"rows": (0, H)}

    def x_copy(i):
        return pltpu.make_async_copy(
            x_hbm.at[pl.ds(pl.multiple_of(_ROFF + i * _TM, 64), _TM)], ring.at[i & 3],
            xsem.at[i & 3])

    def w_copies(l):
        return [pltpu.make_async_copy(w_hbm.at[l, :, pl.ds(c * 128, 128)], wraw.at[l & 1, c],
                                      wsem.at[l]) for c in range(8)]

    def top_copy(i):
        return pltpu.make_async_copy(
            stage.at[i & 1, pl.ds(HT, HT)],
            o_hbm.at[pl.ds(pl.multiple_of(_ROFF + i * _TM, 64), HT)], tsem.at[i & 1])

    def bot_copy(i):
        return pltpu.make_async_copy(
            stage.at[i & 1, pl.ds(0, HT)],
            o_hbm.at[pl.ds(pl.multiple_of(_ROFF + i * _TM - HT, 64), HT)], bsem.at[i & 1])

    def fin(c):
        return pltpu.make_async_copy(
            x_hbm.at[pl.ds(0, _ROFF), pl.ds(c * 128, 128)], fxb.at[c], fsem.at[c])

    def fout(c):
        return pltpu.make_async_copy(
            fxb.at[(L & 1) * 8 + c], o_hbm.at[pl.ds(0, _ROFF), pl.ds(c * 128, 128)], fsem.at[c])

    def loc(n, b, t):
        if n[0] == "a":
            return buf[n, 0], (t * _qsize(4) + (skew[n] + t) % 4 + b * _BS) * 8
        return buf[n, t], ((skew[n] + t) % 4 + b * _BS) * 8

    def ld(n, b, t):
        ref, o = loc(n, b, t)
        r, k = ctx["rows"]
        return ref[ctx["z"], o + r:o + r + k, :]

    def st(n, b, t, v):
        ref, o = loc(n, b, t)
        r, k = ctx["rows"]
        ref[0, o + r:o + r + k, :] = v

    def anc(v, a):
        return v if a is None else jnp.where(ctx["never"], a, v)

    def xin(j, o, i, t):
        r, c, _ = _rowcol(o, i, t)
        r0, k = r * H + ctx["rows"][0], ctx["rows"][1]
        return ring[ctx["slot"][j], r0:r0 + k, c * 128:(c + 1) * 128].astype(f32)

    def sname(s, l):
        return f"{s}{l - L + 4 if l >= L - 2 else l % 2}"

    def uname(p, l):
        return f"u{p}x" if (l == L - 1 and p in (2, 6)) else f"u{p}"

    def upd(l, p, s, a):
        for j in range(4):
            m = {q: ld(uname(p, l), q - 1, j) for q in range(1, 8)}
            m[3] = anc(m[3], next(a))
            v = _comb7(m)
            if l > 0:
                v = [v[i] + ld(sname(s, l - 1), i, j) for i in range(4)]
            for i in range(4):
                st(sname(s, l), i, j, v[i])

    def gval(o, l):
        def g(i):
            s = lambda n, j: ld(sname(n, l), i, j)
            return [s("GH"[o], j) if o < 2 else
                    (s("U", j) + s("V", j)) + s("H", j) if o == 2 else
                    (s("G", j) - s("U", j)) + s("V", j) for j in range(4)]
        return g

    def blocks(g, i, a):
        u = g(i)
        u[1] = anc(u[1], next(a))
        return _bwd(u)

    def gate(o, l, a):
        g = gval(o, l)
        return [_fwd([ld(f"x0{o}", i, t) * v for t, v in enumerate(blocks(g, i, a))],
                     l + 1 in _ALT) for i in range(4)]

    def emit(o, g, a):
        for i in range(4):
            for t, v in enumerate(blocks(g, i, a)):
                r, c, e = _rowcol(o, i, t)
                y = xin(ctx["j"], o, i, t) * v
                if e:
                    y = y * (_D ** -e)
                r0 = ctx["j"] * _TM + r * H + HT + ctx["rows"][0]
                stage[ctx["oslot"], r0:r0 + ctx["rows"][1], c * 128:(c + 1) * 128] = y.astype(bf16)

    def fresh(o, a):
        out = []
        for i in range(4):
            xs = []
            for t in range(4):
                e = _rowcol(o, i, t)[2]
                v = xin(ctx["j"] + 1, o, i, t)
                if t == 0:
                    v = anc(v, next(a))
                st(f"x0{o}", i, t, v)
                xs.append(v * (_D ** e) if e else v)
            out.append(_fwd(xs, 0 in _ALT))
        return out

    def mid(x, a):
        for j in range(4):
            for i, v in enumerate(_fwd([anc(x[0][j], next(a))] + [x[i][j] for i in (1, 2, 3)])):
                yield i, j, v

    def f1(l, x, a):
        for i, j, v in mid(x, a):
            st(f"fx{l % 2}", i, j, v)

    def f2(l, x, a):
        for i, j, v in mid(x, a):
            w = ld(f"fx{l % 2}", i, j)
            st("a3", i, j, v - w)
            st("a5", i, j, v + w)

    def f4(l, x, a):
        for i, j, v in mid(x, a):
            w = ld(f"fx{l % 2}", i, j)
            st("a4", i, j, w + v)
            st("a7", i, j, w - v)

    def f5(l, x, a):
        for i, j, v in mid(x, a):
            u = ld(f"fx{l % 2}", i, j) + v
            a1 = ld("a3", i, j) + ld("a4", i, j)
            st("a1", i, j, a1)
            st("a2", i, j, u + a1)
            st("a6", i, j, u - a1)

    task = {
        "u1": lambda l, a: upd(l, 5, "H", a),
        "u2": lambda l, a: upd(l, 1, "G", a),
        "u3": lambda l, a: upd(l, 2, "U", a),
        "u4": lambda l, a: upd(l, 6, "V", a),
        "x1": lambda l, a: f1(l, gate(1, l, a), a),
        "x2": lambda l, a: f2(l, gate(0, l, a), a),
        "x4": lambda l, a: f4(l, gate(3, l, a), a),
        "x5": lambda l, a: f5(l, gate(2, l, a), a),
        "o1": lambda l, a: emit(1, gval(1, l), a),
        "o2": lambda l, a: emit(0, gval(0, l), a),
        "o4": lambda l, a: emit(3, gval(3, l), a),
        "o5": lambda l, a: emit(2, gval(2, l), a),
        "e1": lambda l, a: f1(l, fresh(1, a), a),
        "e2": lambda l, a: f2(l, fresh(0, a), a),
        "e4": lambda l, a: f4(l, fresh(3, a), a),
        "e5": lambda l, a: f5(l, fresh(2, a), a),
    }
    for k in "1234":
        task["v" + k] = task["u" + k]

    def run_plain(names):
        for g in range(_NG):
            ctx["rows"] = (g * 8, 8)
            for w in names:
                task[w](L - 1, itertools.repeat(None))
        ctx["rows"] = (0, H)

    b_copy = pltpu.make_async_copy(b_hbm, b_ref, fsem.at[8])
    b_copy.start()
    for c in range(8):
        fin(c).start()
    for cp in w_copies(0):
        cp.start()

    for n in ("u2x", "u6x", sname("U", L - 2), sname("V", L - 2), sname("G", L - 1),
              sname("H", L - 1)):
        for t in range(4):
            buf[n, t][...] = jnp.zeros(buf[n, t].shape, f32)
    ring[3, HT:, :] = jnp.zeros((HT, ring.shape[2]), bf16)
    fx32[8:16] = jnp.ones((8, _ROFF, 128), f32)

    b_copy.wait()
    kap, kaq = _kappa(_BP), _kappa(_BQ)
    for l in range(L):
        bl = b_ref[l:l + 1, :].astype(f32)
        for c in range(8):
            fb[l * 8 + c, 0:1, :] = bl[:, c * 128:(c + 1) * 128]
        if l == 0:
            bl = bl + 1.0
        for pi, p in enumerate(_BP):
            for qi, q in enumerate(_BQ):
                col = []
                for c3 in range(2):
                    acc = None
                    for c1 in range(2):
                        for c2 in range(2):
                            k = float(kap[c1][p] * kaq[c2][q])
                            if abs(k) < 1e-12:
                                continue
                            c = c1 * 4 + c2 * 2 + c3
                            term = bl[:, c * 128:(c + 1) * 128] * k
                            acc = term if acc is None else acc + term
                    col.append(acc)
                us = [col[0] + col[1] * (1 / _D), col[1] * (2 / _D),
                      col[0] * ((_D + 1) / 2) - col[1] * ((1 + 1 / _D) / 2),
                      col[0] * ((_D - 1) / 2) + col[1] * ((1 - 1 / _D) / 2)]
                row = l * 64 + (pi * 4 + qi) * 4
                for j in range(4):
                    beta[row + j:row + j + 1, :] = us[j]
    for c in range(8):
        fin(c).wait()
    for c in range(8):
        fx32[c] = fxb[c].astype(f32)

    def toff(p, i, t):
        return ((p - 1) * 37 + (i * 4 + t) * 2 + i) * 8

    def s1_units(l, g, dst):
        r0 = g * 16

        def unit(mids, t, a):
            blk = {}
            for i in mids:
                for o in range(4):
                    r, c, e = _rowcol(o, i, t)
                    v = wraw[l & 1, c, r * 128 + r0:r * 128 + r0 + 16, :].astype(f32)
                    blk[o, i] = v * (0.25 * _D ** e)
            if len(mids) == 2:
                blk[0, 0] = anc(blk[0, 0], a(0))
                sm = (blk[0, 0] + blk[3, 0]) + (blk[0, 3] + blk[3, 3])
                dl = (_rnd(sm) - sm) * 0.25
                for k in ((0, 0), (3, 0), (0, 3), (3, 3)):
                    blk[k] = blk[k] + dl
            else:
                blk[1, mids[0]] = anc(blk[1, mids[0]], a(0))
            out = []
            for i in mids:
                ex = _bexp([blk[o, i] for o in range(4)])
                for p in _PH:
                    dst[0, toff(p, i, t):toff(p, i, t) + 16, :] = ex[p]
                out.append(ex[7][:8])
            return out

        return [(34 if len(m) == 1 else 90, functools.partial(unit, m, t))
                for t in range(4) for m in ((0, 3), (1,), (2,))]

    def s2_units(l, g, src, zg):
        r0 = g * 16

        def put(p, q, qs, a=None):
            qs = [qs[0], anc(qs[1], a), qs[2], qs[3]]
            if (p, q) != _PLAIN:
                f = (2.0 if p == 1 else 1.0) * (2 if q in (1, 2, 6) else 1)
                qs = _bexp_inner([v * f for v in qs] if f != 1 else qs)
            for k, v in enumerate(qs):
                wexp[l, tile0[p, q] + k, r0:r0 + 16, :] = v.astype(bf16)

        def unit(p, un, a):
            def tl(i):
                vs = [src[zg[un], toff(p, i, t):toff(p, i, t) + 16, :] for t in range(4)]
                if i == (0 if un == 2 else 1):
                    vs[1] = anc(vs[1], a(0))
                return vs

            if un == 0:
                x, y, qa, qb = tl(0), tl(1), 2, 6
            elif un == 1:
                x, y, qa, qb = tl(1), tl(3), 3, 5
            else:
                x = [u + v for u, v in zip(tl(1), tl(2))]
                y = [u + v for u, v in zip(tl(0), tl(3))]
                qa, qb = 4, 7
                put(p, 1, y)
            put(p, qa, [u - v for u, v in zip(x, y)], a(2) if un == 2 else None)
            put(p, qb, [u + v for u, v in zip(x, y)], a(4 if un == 2 else 2))

        return [((102, 86, 145)[un], functools.partial(unit, p, un))
                for p in _PH for un in range(3)]

    def layer(l, carry):
        for cp in w_copies(l):
            cp.wait()

        @pl.when(l + 1 < L)
        def _():
            for cp in w_copies(l + 1):
                cp.start()

        @pl.when(l == L - 2)
        def _():
            x_copy(0).start()
            x_copy(1).start()

        zg = [lax.shift_right_logical(l, 8 + k) for k in range(4)]
        ctx["never"] = jnp.full((16, 128), zg[0], jnp.int32) != 0
        head = [v for _, f in s1_units(l, 0, tmp[0]) for v in f(lambda d: None)]
        units = []
        for g in range(8):
            u2 = s2_units(l, g, tmp[g % 2], zg[1:])
            units += [(g + k / len(u2), c, f) for k, (c, f) in enumerate(u2)]
            if g < 7:
                u1 = s1_units(l, g + 1, tmp[(g + 1) % 2])
                units += [(g + (k + 0.5) / len(u1) * cfg["s1f"], c, f)
                          for k, (c, f) in enumerate(u1)]
        units.sort(key=lambda e: e[0])
        total = sum(c for _, c, _ in units)
        nr = _ROFF // 8
        acc = 0
        todo = {}
        for _, c, f in units:
            sl = cfg["l0"] + int(acc / total * (16 * nr - cfg["l0"] - cfg["l1"]))
            todo.setdefault(sl // nr, []).append((sl % nr, f))
            acc += c
        fsrc = (l & 1) * 8
        fu = fxb.bitcast(jnp.uint32)
        wu = wraw.bitcast(jnp.uint32)
        for g in range(8):
            for h in range(2):
                cols = [fu[fsrc + 4 * h + c] for c in range(4)]
                if g == 0 and h == 0:
                    pace = jnp.concatenate([pltpu.bitcast(v, jnp.uint32) for v in head], 0)
                    nv = jnp.full((128, 128), zg[0], jnp.int32) != 0
                    cols[0] = jnp.concatenate(
                        [cols[0][:16], jnp.where(nv, pace, cols[0][16:144]), cols[0][144:]], 0)
                xa = jnp.concatenate([pltpu.bitcast(v, bf16) for v in cols], 1)
                y = jnp.dot(xa, pltpu.bitcast(wu[l & 1, g, h * 256:(h + 1) * 256, :], bf16),
                            preferred_element_type=f32)
                if h == 0:
                    fx32[8 + g] = (y + fb[l * 8 + g, 0:1, :]) + fx32[8 + g]
                else:
                    gn = y + fx32[8 + g]
                    fx32[8 + g] = gn
                    fxb[8 - fsrc + g] = (fx32[g] * gn).astype(bf16)
                for r, f in todo.get(2 * g + h, []):
                    f(lambda d: y[min(r + d, nr - 2) * 8:min(r + d, nr - 2) * 8 + 16])
        return carry

    lax.fori_loop(0, L, layer, 0)
    for c in range(8):
        fout(c).start()
    x_copy(0).wait()
    ctx.update(z=0, slot={0: 0}, j=-1)
    run_plain(("e1", "e2"))

    prods, sched, ugate = _schedule(L, order, cfg)

    def main(step, carry):
        @pl.when(step + 1 < nsteps)
        def _():
            x_copy(step + 1).wait()

        @pl.when(step >= 2)
        def _():
            top_copy(step - 2).wait()

        @pl.when(step >= 3)
        def _():
            bot_copy(step - 2).wait()

        @pl.when(step >= 1)
        def _():
            top_copy(step - 1).start()

        @pl.when(step + 2 < nsteps)
        def _():
            x_copy(step + 2).start()

        zz = [lax.shift_right_logical(step, 12 + k) for k in range(15)]
        ctx.update(never=jnp.full((H, 128), zz[0], jnp.int32) != 0,
                   slot={-1: (step + 3) & 3, 0: step & 3, 1: (step + 1) & 3}, oslot=step & 1)
        wu = wexp.bitcast(jnp.uint32)
        subs = {}

        def wtile(l, k):
            return pltpu.bitcast(wu[l, k], bf16)

        def gather(al):
            return jnp.concatenate([subs[pi][j][g * 8:(g + 1) * 8, :] for pi, j, g in al], 0)

        nin = 0
        for pi, (l, p, q) in enumerate(prods):
            ctx["z"] = zz[_ZQ[q]]
            qv = []
            for t in range(4):
                vs = [ld(f"a{p}", b, t) for b, _ in _MIDB[q]]
                qv.append(vs[0] if len(vs) == 1 else vs[0] - vs[1])
                if t == 1 and pi in ugate:
                    qv[t] = anc(qv[t], gather(ugate[pi]))
            k0 = tile0[p, q]
            if (p, q) != _PLAIN:
                a1 = _rnd(qv[0])
                r3, r4 = (4, 3) if l in _ALT else (3, 4)
                dv = list(qv)
                t = (0, 2, 1, 3)[nin % 4]
                if t and len(_MIDB[q]) == 1 and not (t == 1 and pi in ugate):
                    ctx["z"] = zz[14]
                    dv[t] = ld(f"a{p}", _MIDB[q][0][0], t)
                    ctx["z"] = zz[_ZQ[q]]
                nin += 1
                av = {1: a1, 2: dv[1], r3: dv[2], 5: dv[3], r4: a1 - qv[2], 6: qv[1] - a1,
                      7: qv[3] - a1}
                so = (r3, r4) + _SO
                m = {r: jnp.dot(av[r].astype(bf16), wtile(l, k0 + r - 1),
                                preferred_element_type=f32) for r in so}
                subs[pi] = [m[r] for r in so]
                mq = _combu(m)
            else:
                if l in _ALT:
                    qv[2] = qv[0] - qv[2]
                d1 = qv[0] + qv[0]
                y11, y12 = qv[2] + qv[3], qv[3] - qv[2]
                qv = [y11, y12, (qv[1] * 4.0 - d1) - y12, d1 - y11]
                a = jnp.concatenate(
                    [jnp.concatenate(qv[:2], 1), jnp.concatenate(qv[2:], 1)], 0).astype(bf16)
                wt = [wtile(l, k0 + t) for t in range(4)]
                wm = jnp.concatenate([jnp.concatenate(wt[:2], 1), jnp.concatenate(wt[2:], 1)], 0)
                mm = jnp.dot(a, wm, preferred_element_type=f32)
                subs[pi] = [mm[:, :128]]
                c11, c12, c21, c22 = mm[:H, :128], mm[:H, 128:], mm[H:, :128], mm[H:, 128:]
                sm = c11 + c12
                mq = [sm + sm, c12 * 4.0, (c21 - c22) + (c11 - c12), (c21 + c22) - sm]
            if p in _BP and q in _BQ:
                row = l * 64 + (_BP.index(p) * 4 + _BQ.index(q)) * 4
                mq = [mq[t] + beta[row + t:row + t + 1, :] for t in range(4)]
            for t in range(4):
                v = mq[t]
                if p == 5:
                    v = v + ld("u3", q - 1, t)
                elif p == 1:
                    r3 = ld("u3", q - 1, t)
                    v = v + (((ld("u4", q - 1, t) + ld("u7", q - 1, t)) + (r3 + r3))
                             - ld("u5", q - 1, t))
                elif p == 2:
                    v = v + ld("u4", q - 1, t)
                elif p == 6:
                    v = v - ld("u7", q - 1, t)
                st(uname(p, l), q - 1, t, v)
            for j, jn, w, tl, als in sched.get(pi, []):
                ctx.update(z=zz[4 + jn % 10], j=j)
                task[w](tl, iter([gather(al) for al in als]))
            if pi == _BOT_DONE:
                @pl.when(step >= 1)
                def _():
                    bot_copy(step).start()

        return carry

    lax.fori_loop(0, nsteps, main, 0)

    top_copy(nsteps - 1).start()
    top_copy(nsteps - 2).wait()
    bot_copy(nsteps - 2).wait()
    ctx.update(z=0, slot={-1: (nsteps - 1) % 4}, j=-1, oslot=nsteps % 2)
    run_plain(("v3", "v4", "o4", "o5"))
    bot_copy(nsteps).start()
    for c in range(8):
        fout(c).wait()
    top_copy(nsteps - 1).wait()
    bot_copy(nsteps - 1).wait()
    bot_copy(nsteps).wait()


def _build(**kw):
    cfg = dict(_CFG, **kw)

    def fn(x0, ws, bs):
        B, Dm = x0.shape
        L = ws.shape[0]
        assert Dm == 1024 and L == 6 and (B - _ROFF) % _TM == 0
        nsteps = (B - _ROFF) // _TM
        assert 4 <= nsteps < 4096
        ntiles = _products()[2]
        return pl.pallas_call(
            functools.partial(_kernel, L=L, nsteps=nsteps, cfg=cfg),
            in_specs=[pl.BlockSpec(memory_space=pl.ANY)] * 3,
            out_specs=pl.BlockSpec(memory_space=pl.ANY),
            out_shape=jax.ShapeDtypeStruct((B, Dm), x0.dtype),
            scratch_shapes=[
                pltpu.VMEM((L, Dm), bf16),
                pltpu.VMEM((4, _TM, Dm), bf16),
                pltpu.VMEM((2, _TM, Dm), bf16),
                pltpu.VMEM((2, 8, Dm, 128), bf16),
                pltpu.VMEM((L, ntiles, 128, 128), bf16),
                pltpu.VMEM((L * 64, 128), f32),
                pltpu.VMEM((16, _ROFF, 128), f32),
                pltpu.VMEM((16, _ROFF, 128), bf16),
                pltpu.VMEM((L * 8, 8, 128), f32),
                pltpu.SemaphoreType.DMA((4,)),
                pltpu.SemaphoreType.DMA((L,)),
                pltpu.SemaphoreType.DMA((2,)),
                pltpu.SemaphoreType.DMA((2,)),
                pltpu.SemaphoreType.DMA((9,)),
            ]
            + [pltpu.VMEM((1, 260 * 8, 128), f32)] * 2
            + [pltpu.VMEM((1, sz * 8, 128), f32) for _, sz in _bufkeys()],
            compiler_params=pltpu.CompilerParams(
                vmem_limit_bytes=126 * 1024 * 1024,
                disable_bounds_checks=True,
            ),
        )(x0, ws, bs)

    return fn


@jax.jit
def pallas_standalone__dcn_v2_cross__recsys_kernel(
    x0: jax.Array,
    ws: jax.Array,
    bs: jax.Array,
):
    return _build()(x0, ws, bs)
```
